```python
import jax
import jax.numpy as jnp

def _softmax(x, axis=-1):
    return jax.nn.softmax(x, axis=axis)

def _gelu(x):
    return jax.nn.gelu(x, approximate=True)

def _silu(x):
    return jax.nn.silu(x)

def _sigmoid(x):
    return jax.nn.sigmoid(x)

def _layernorm(x, axis=-1, eps=1e-05):
    m = jnp.mean(x, axis=axis, keepdims=True)
    v = jnp.var(x, axis=axis, keepdims=True)
    return (x - m) / jnp.sqrt(v + eps)

def _scatter_add(tgt, idx, src, axis=0):
    return tgt.at[idx].add(src)

def _segment_sum(src, seg, n):
    return jax.ops.segment_sum(src, seg, n)

class _Rng:

    def __init__(self, key):
        self._k = key

    def _next(self):
        self._k, sub = jax.random.split(self._k)
        return sub

    def normal(self, shape):
        return jax.random.normal(self._next(), shape, dtype=jnp.bfloat16)

    def randint(self, lo, hi, shape):
        return jax.random.randint(self._next(), shape, lo, hi, dtype=jnp.int32)

    def uniform(self, shape, lo=0.0, hi=1.0):
        return jax.random.uniform(self._next(), shape, jnp.bfloat16, lo, hi)

    def permutation(self, n):
        return jax.random.permutation(self._next(), n)
kernel_name = 'interleave_layers__memory_aug_recurrent_mem_tr__spectral_gfnet__prompt'

def setup_inputs():
    _rng = _Rng(jax.random.key(int.from_bytes(__import__("os").urandom(4), "little")))
    _w = lambda a: (lambda t: t.astype(jnp.bfloat16) if jnp.issubdtype(t.dtype, jnp.floating) else t)(jnp.asarray(a))

    def _A_setup():
        B, S, Dm = (1, 2048, 640)
        H, Dh = (32, 128)
        M, seg = (8, 32)
        seg = min(seg, S)
        S = S // seg * seg
        return {'x': _w((lambda *s: _rng.normal(s) * 0.05)(B, S, Dm)), 'mem0': _w((lambda *s: _rng.normal(s) * 0.05)(B, M, Dm)), 'Wq': _w((lambda *s: _rng.normal(s) * 0.05)(Dm, H, Dh) * Dm ** (-0.5)), 'Wk': _w((lambda *s: _rng.normal(s) * 0.05)(Dm, H, Dh) * Dm ** (-0.5)), 'Wv': _w((lambda *s: _rng.normal(s) * 0.05)(Dm, H, Dh) * Dm ** (-0.5)), 'Wo': _w((lambda *s: _rng.normal(s) * 0.05)(H, Dh, Dm) * (H * Dh) ** (-0.5)), 'seg_len': seg}
    _A_in = _A_setup()

    def _B_setup():
        B, S, D = (1, 2048, 640)
        Df = D // 2 + 1
        return {'x': _w((lambda *s: _rng.normal(s) * 0.05)(B, S, D)), 'w_r': _w((lambda *s: _rng.normal(s) * 0.05)(S, Df) * 0.02), 'w_i': _w((lambda *s: _rng.normal(s) * 0.05)(S, Df) * 0.02)}
    _B_in = _B_setup()
    return {'A_x': _A_in['x'], 'A_mem0': _A_in['mem0'], 'A_Wq': _A_in['Wq'], 'A_Wk': _A_in['Wk'], 'A_Wv': _A_in['Wv'], 'A_Wo': _A_in['Wo'], 'A_seg_len': _A_in['seg_len'], 'B_x': _B_in['x'], 'B_w_r': _B_in['w_r'], 'B_w_i': _B_in['w_i']}

def reference(A_x, A_mem0, A_Wq, A_Wk, A_Wv, A_Wo, A_seg_len, B_x, B_w_r, B_w_i):

    def _A_ref(x, mem0, Wq, Wk, Wv, Wo, seg_len):
        B, S, Dm = x.shape
        H, Dh = (Wq.shape[1], Wq.shape[2])
        M = mem0.shape[1]
        scale = Dh ** (-0.5)
        n_seg = S // seg_len
        L = M + seg_len
        idx = jnp.arange(L)
        mask = (idx[:, None] < M) | (idx[:, None] >= idx[None, :])
        mem = mem0
        outs = []
        for s in range(n_seg):
            xs = x[:, s * seg_len:(s + 1) * seg_len, :].copy()
            h = jnp.concatenate([mem, xs], axis=1)
            q = jnp.einsum('btd,dhe->bhte', h, Wq)
            k = jnp.einsum('btd,dhe->bhte', h, Wk)
            v = jnp.einsum('btd,dhe->bhte', h, Wv)
            scores = jnp.einsum('bhqe,bhke->bhqk', q, k) * scale
            scores = jnp.where(mask[None, None], scores, -1000000000.0)
            p = _softmax(scores, axis=-1)
            o = jnp.einsum('bhqk,bhke->bhqe', p, v)
            o = jnp.einsum('bhte,hed->btd', o, Wo)
            mem = o[:, :M, :].copy()
            outs.append(o[:, M:, :])
        return jnp.concatenate(outs, axis=1)

    def _B_ref(x, w_r, w_i):
        B, S, D = x.shape
        X = (lambda x, axes=(-2, -1): jnp.fft.rfft2(x.astype(jnp.float32), axes=axes))(x, axes=(-2, -1))
        W = w_r + 1j * w_i
        X = X * W
        y = (lambda x, s, axes=(-2, -1): jnp.fft.irfft2(x, s=s, axes=axes).astype(jnp.bfloat16))(X, (S, D), axes=(-2, -1))
        return y
    x = A_x
    x = x + _A_ref(_layernorm(x, axis=-1), A_mem0, A_Wq, A_Wk, A_Wv, A_Wo, A_seg_len)
    x = x + _B_ref(_layernorm(x, axis=-1), B_w_r, B_w_i)
    x = x + _A_ref(_layernorm(x, axis=-1), A_mem0, A_Wq, A_Wk, A_Wv, A_Wo, A_seg_len)
    x = x + _B_ref(_layernorm(x, axis=-1), B_w_r, B_w_i)
    return x
```

```python
import functools
import math

import jax
import jax.numpy as jnp
import numpy as np
import jax.experimental.pallas as pl
import jax.experimental.pallas.tpu as pltpu

S, DM, H, DH, M, SEG = 2048, 640, 32, 128, 8, 32
L = M + SEG
DF = DM // 2 + 1
R16 = 16
NB = S // R16
F32, BF16, U32 = jnp.float32, jnp.bfloat16, jnp.uint32
_NN = (((1,), (0,)), ((), ()))
_NT = (((1,), (1,)), ((), ()))


def _dot(a, b, dims=_NN):
    return jax.lax.dot_general(a, b, dims, preferred_element_type=F32)


def _rnd(v):
    return v.astype(BF16).astype(F32)


def _constants():
    b = np.arange(128)[:, None].astype(np.float64)
    j = np.arange(128)
    fd = np.zeros((5 * 128, 256))
    perm = np.zeros((DF, 384))
    cscale = np.zeros((1, 384))
    th = 2 * np.pi * b * (5 * j[None, :65]) / DM
    fd[:128, :65] = np.cos(th)
    fd[:128, 128:128 + 65] = -np.sin(th)
    fd[:128, 128] = 0.0
    fd[:128, 128 + 64] = 0.0
    perm[5 * j[:65], j[:65]] = 1.0
    cscale[0, :65] = 2.0
    cscale[0, 0] = cscale[0, 64] = 1.0
    for r in (1, 2):
        fp = np.where(j < 64, r + 5 * j, (5 - r) + 5 * (j - 64))
        f = np.where(j < 64, fp, DM - fp)
        sg = np.where(j < 64, 1.0, -1.0)[None, :]
        th = 2 * np.pi * b * f[None, :] / DM
        o = 128 + (r - 1) * 256
        fd[o:o + 128, :128] = np.cos(th)
        fd[o:o + 128, 128:] = -sg * np.sin(th)
        fd[o + 128:o + 256, :128] = np.sin(th)
        fd[o + 128:o + 256, 128:] = sg * np.cos(th)
        perm[fp, r * 128 + j] = 1.0
        cscale[0, r * 128:(r + 1) * 128] = 2.0
    cscale /= float(S * DM)
    fs = np.zeros((R16, 256, 256))
    g = np.arange(128)[:, None].astype(np.float64)
    bb = np.arange(128)[None, :].astype(np.float64)
    for r in range(R16):
        th = 2 * np.pi * ((r + R16 * g) * bb % S) / S
        c, s = np.cos(th), np.sin(th)
        fs[r] = np.block([[c, s], [-s, c]])
    bf = lambda a: np.asarray(a, dtype=BF16)
    return (bf(fd), bf(fd.T), bf(fs), bf(fs.transpose(0, 2, 1)), bf(perm), cscale.astype(np.float32))


def _fft4(x, sgn):
    (ar, ai), (br, bi), (cr, ci), (dr, di) = x
    s0r, s0i, d0r, d0i = ar + cr, ai + ci, ar - cr, ai - ci
    s1r, s1i, d1r, d1i = br + dr, bi + di, br - dr, bi - di
    p = (d0r + d1i, d0i - d1r)
    q = (d0r - d1i, d0i + d1r)
    y1, y3 = (p, q) if sgn < 0 else (q, p)
    return [(s0r + s1r, s0i + s1i), y1, (s0r - s1r, s0i - s1i), y3]


def _twiddle(v, e, sgn):
    if e == 0:
        return v
    vr, vi = v
    if e == 4:
        return (-vi, vr) if sgn > 0 else (vi, -vr)
    c, s = math.cos(2 * math.pi * e / 16), sgn * math.sin(2 * math.pi * e / 16)
    if e in (2, 6):
        if c * s > 0:
            return ((vr - vi) * c, (vr + vi) * c)
        return ((vr + vi) * c, (vi - vr) * c)
    return (vr * c - vi * s, vr * s + vi * c)


def _fft16(x, sgn):
    t = [_fft4([x[n2 + 4 * n1] for n1 in range(4)], sgn) for n2 in range(4)]
    y = [None] * 16
    for k1 in range(4):
        o = _fft4([_twiddle(t[n2][k1], n2 * k1, sgn) for n2 in range(4)], sgn)
        for k2 in range(4):
            y[k1 + 4 * k2] = o[k2]
    return y


_C1, _C2 = math.cos(2 * math.pi / 5), math.cos(4 * math.pi / 5)
_S1, _S2 = math.sin(2 * math.pi / 5), math.sin(4 * math.pi / 5)


def _rfft5(u):
    x = [u[:, a * 128:(a + 1) * 128] for a in range(5)]
    s1, s2, d1, d2 = x[1] + x[4], x[2] + x[3], x[4] - x[1], x[3] - x[2]
    return jnp.concatenate([
        x[0] + s1 + s2,
        x[0] + _C1 * s1 + _C2 * s2, _S1 * d1 + _S2 * d2,
        x[0] + _C2 * s1 + _C1 * s2, _S2 * d1 - _S1 * d2], axis=1)


def _irfft5(q):
    q0, q1r, q1i, q2r, q2i = [q[:, a * 128:(a + 1) * 128] for a in range(5)]
    e1, e2 = q0 + _C1 * q1r + _C2 * q2r, q0 + _C2 * q1r + _C1 * q2r
    o1, o2 = _S1 * q1i + _S2 * q2i, _S2 * q1i - _S1 * q2i
    return jnp.concatenate([q0 + q1r + q2r, e1 - o1, e2 - o2, e2 + o2, e1 + o1], axis=1)


def _layernorm(x):
    mu = jnp.mean(x, axis=1, keepdims=True)
    d = x - mu
    var = jnp.mean(d * d, axis=1, keepdims=True)
    return _rnd(d * jax.lax.rsqrt(var + 1e-5))


NCH = 5
WROWS = DM * H // NCH


def _kernel(x_hbm, mem_hbm, wq_hbm, wk_hbm, wv_hbm, wo_hbm, wr_hbm, wi_hbm,
            fd_hbm, fdt_hbm, fs_hbm, fst_hbm, perm_hbm, cs_hbm,
            o_ref,
            memb, stage, t32, wqkv, wostage, wo, wrb, wib, wp,
            fd, fdt, fs, fst, perm, cs,
            xs, us, u_buf, t_buf, v_buf, q_buf, sems):
    cnt = [0]

    def copy(src, dst):
        c = pltpu.make_async_copy(src, dst, sems.at[cnt[0]])
        cnt[0] += 1
        c.start()
        return c

    c_small = [copy(perm_hbm, perm), copy(cs_hbm, cs), copy(wr_hbm, wrb), copy(wi_hbm, wib)]
    c_x = [copy(x_hbm, o_ref), copy(mem_hbm, memb)]
    c_w = [[copy(w.at[pl.ds(c * WROWS, WROWS)], stage.at[i * NCH + c]) for c in range(NCH)]
           for i, w in enumerate((wq_hbm, wk_hbm, wv_hbm))]
    c_wo = [copy(wo_hbm.at[pl.ds(c * 1024, 1024)], wostage.at[pl.ds(c * 1024, 1024)]) for c in range(4)]
    c_b = [copy(fd_hbm, fd), copy(fs_hbm, fs), copy(fst_hbm, fst), copy(fdt_hbm, fdt)]

    for c in c_small:
        c.wait()
    pr = jax.lax.broadcasted_iota(jnp.int32, (256, 256), 0)
    pc = jax.lax.broadcasted_iota(jnp.int32, (256, 256), 1)
    shuffle = jnp.where(pc == (pr >> 4) + ((pr & 15) << 4), 1.0, 0.0).astype(BF16)

    def perm_filter(i, _):
        rows = pl.ds(pl.multiple_of(i * 256, 256), 256)
        for part, src in enumerate((wrb, wib)):
            w = _dot(shuffle, _dot(src[rows, :], perm[...]).astype(BF16)) * cs[...]
            for r in range(R16):
                wp[r, pl.ds(pl.multiple_of(i * 16, 16), 16), part * 384:(part + 1) * 384] = w[r * 16:(r + 1) * 16]
    jax.lax.fori_loop(0, S // 256, perm_filter, None)

    for c in c_x:
        c.wait()

    def first_ln(i, _):
        rows = pl.ds(pl.multiple_of(i * 64, 64), 64)
        x = o_ref[rows, :].astype(F32)
        xs[rows, :] = x
        us[rows, :] = _layernorm(x)
    jax.lax.fori_loop(0, S // 64, first_ln, None)

    for i in range(3):
        for c in range(NCH):
            c_w[i][c].wait()

            def widen(j, _):
                t32[pl.ds(pl.multiple_of(j * 256, 256), 256), :] = pltpu.bitcast(
                    stage[i * NCH + c, pl.ds(pl.multiple_of(j * 512, 512), 512), :], U32)
            jax.lax.fori_loop(0, WROWS // 512, widen, None)

            def split(j, _):
                v = t32[pl.ds(j, 128, stride=H // 2), :]
                lo = pltpu.bitcast(v << 16, F32).astype(BF16)
                hi = pltpu.bitcast(v & np.uint32(0xFFFF0000), F32).astype(BF16)
                wqkv[2 * j, c * 128:(c + 1) * 128, i * 128:(i + 1) * 128] = lo
                wqkv[2 * j + 1, c * 128:(c + 1) * 128, i * 128:(i + 1) * 128] = hi
            jax.lax.fori_loop(0, H // 2, split, None, unroll=4)
    for c in range(4):
        c_wo[c].wait()

        def retile(j, _):
            rows = pl.ds(pl.multiple_of(c * 1024 + j * 128, 128), 128)
            wo[rows, :] = wostage[rows, :]
        jax.lax.fori_loop(0, 8, retile, None)

    row = jax.lax.broadcasted_iota(jnp.int32, (L, L), 0)
    col = jax.lax.broadcasted_iota(jnp.int32, (L, L), 1)
    mask = (row < M) | (row >= col)
    scale = DH ** -0.5
    G = 4

    def a_step(s, mem):
        rows = pl.ds(pl.multiple_of(s * SEG, SEG), SEG)
        hh = jnp.concatenate([mem, us[rows, :]], axis=0)
        qkv, sc, pp, oo = {}, {}, {}, {}
        acc = None
        for t in range(H + H // G):
            if t < H:
                qkv[t] = _dot(hh, wqkv[t])
            else:
                g = t - H
                o = jnp.concatenate([oo[g * G + i] for i in range(G)], axis=1)
                r = _dot(o, wo[g * G * DH:(g + 1) * G * DH, :])
                acc = r if acc is None else acc + r
            h = t - 2
            if 0 <= h < H:
                sc[h] = _dot(qkv[h][:, :128], qkv[h][:, 128:256].astype(BF16), _NT)
            h = t - 3
            if 0 <= h < H:
                z = jnp.where(mask, sc[h] * scale, -1e9)
                e = jnp.exp(z - jnp.max(z, axis=1, keepdims=True))
                pp[h] = e * (1.0 / jnp.sum(e, axis=1, keepdims=True))
            h = t - 5
            if 0 <= h < H:
                oo[h] = _dot(pp[h], qkv[h][:, 256:].astype(BF16))
        acc = _rnd(acc)
        xs[rows, :] = _rnd(xs[rows, :] + acc[M:])
        return acc[:M]

    def b_fwd(i, _):
        base = i * 16
        for a in range(R16):
            x = xs[pl.ds(pl.multiple_of(base + a * NB, 16), 16), :]
            v_buf[a * 16:(a + 1) * 16, :DM] = _rfft5(_layernorm(x)).astype(BF16)
        for r in range(3):
            k0, k1 = (0, 128) if r == 0 else (r * 256 - 128, r * 256 + 128)
            q_buf[:, r * 256:(r + 1) * 256] = _dot(v_buf[:, k0:k1], fd[k0:k1, :])
        for r in range(3):
            y = _fft16([(q_buf[a * 16:(a + 1) * 16, r * 256:r * 256 + 128],
                         q_buf[a * 16:(a + 1) * 16, r * 256 + 128:(r + 1) * 256])
                        for a in range(R16)], -1)
            for k in range(R16):
                t_buf[k, pl.ds(pl.multiple_of(base, 16), 16), r * 128:(r + 1) * 128] = y[k][0].astype(BF16)
                t_buf[k, pl.ds(pl.multiple_of(base + NB, 16), 16), r * 128:(r + 1) * 128] = y[k][1].astype(BF16)

    def b_mid(k, _):
        x = _dot(fs[k], t_buf[k])
        xr, xi = x[:NB], x[NB:]
        wr, wi = wp[k, :, :384], wp[k, :, 384:]
        y = jnp.concatenate([xr * wr - xi * wi, xr * wi + xi * wr], axis=0).astype(BF16)
        z = _dot(fst[k], y)
        rows = pl.ds(pl.multiple_of(k * NB, NB), NB)
        u_buf[rows, :384] = z[:NB]
        u_buf[rows, 384:] = z[NB:]

    def b_inv(i, _):
        base = i * 16
        for r in range(3):
            y = _fft16([(u_buf[pl.ds(pl.multiple_of(base + k * NB, 16), 16), r * 128:(r + 1) * 128],
                         u_buf[pl.ds(pl.multiple_of(base + k * NB, 16), 16), 384 + r * 128:384 + (r + 1) * 128])
                        for k in range(R16)], +1)
            for a in range(R16):
                v_buf[a * 16:(a + 1) * 16, r * 256:r * 256 + 128] = y[a][0].astype(BF16)
                v_buf[a * 16:(a + 1) * 16, r * 256 + 128:(r + 1) * 256] = y[a][1].astype(BF16)
        for r in range(3):
            k0, k1 = (0, 128) if r == 0 else (r * 256 - 128, r * 256 + 128)
            q_buf[:, k0:k1] = _dot(v_buf[:, r * 256:(r + 1) * 256], fdt[:, k0:k1])
        for a in range(R16):
            rows = pl.ds(pl.multiple_of(base + a * NB, 16), 16)
            x = (xs[rows, :] + _rnd(_irfft5(q_buf[a * 16:(a + 1) * 16, :DM]))).astype(BF16)
            o_ref[rows, :] = x
            x = x.astype(F32)
            xs[rows, :] = x
            us[rows, :] = _layernorm(x)

    def layer(l, _):
        jax.lax.fori_loop(0, S // SEG, a_step, memb[...].astype(F32))

        @pl.when(l == 0)
        def _():
            for c in c_b:
                c.wait()
        jax.lax.fori_loop(0, NB // 16, b_fwd, None)
        jax.lax.fori_loop(0, R16, b_mid, None, unroll=2)
        jax.lax.fori_loop(0, NB // 16, b_inv, None)
    jax.lax.fori_loop(0, 2, layer, None)


@functools.partial(jax.jit, static_argnames=("A_seg_len",))
def pallas_interleave_layers__memory_aug_recurrent_mem_tr__spectral_gfnet__prompt_kernel(
    A_x, A_mem0, A_Wq, A_Wk, A_Wv, A_Wo, A_seg_len, B_x, B_w_r, B_w_i,
):
    del B_x
    assert A_x.shape == (1, S, DM) and A_Wq.shape == (DM, H, DH) and int(A_seg_len) == SEG
    consts = _constants()
    vm = pltpu.VMEM
    out = pl.pallas_call(
        _kernel,
        out_shape=jax.ShapeDtypeStruct((S, DM), BF16),
        in_specs=[pl.BlockSpec(memory_space=pl.ANY)] * 14,
        out_specs=pl.BlockSpec(memory_space=pltpu.VMEM),
        scratch_shapes=[
            vm((M, DM), BF16),
            vm((3 * NCH, WROWS, DH), BF16),
            vm((WROWS // 2, DH), U32),
            vm((H, DM, 3 * DH), BF16),
            vm((H * DH, DM), BF16),
            vm((H * DH, DM), BF16),
            vm((S, DF), BF16), vm((S, DF), BF16),
            vm((R16, NB, 768), F32),
            vm((DM, 256), BF16), vm((256, DM), BF16),
            vm((R16, 256, 256), BF16), vm((R16, 256, 256), BF16),
            vm((DF, 384), BF16), vm((1, 384), F32),
            vm((S, DM), F32), vm((S, DM), F32),
            vm((S, 768), F32),
            vm((R16, 256, 384), BF16),
            vm((256, 768), BF16),
            vm((256, 768), F32),
            pltpu.SemaphoreType.DMA((32,)),
        ],
        compiler_params=pltpu.CompilerParams(vmem_limit_bytes=110 * 2**20),
        name="rmt_gfnet",
    )(A_x.reshape(S, DM), A_mem0.reshape(M, DM),
      A_Wq.reshape(DM * H, DH), A_Wk.reshape(DM * H, DH), A_Wv.reshape(DM * H, DH),
      A_Wo.reshape(H * DH, DM), B_w_r, B_w_i, *consts)
    return out.reshape(1, S, DM)
```

```python
import functools
import math

import jax
import jax.numpy as jnp
import numpy as np
import jax.experimental.pallas as pl
import jax.experimental.pallas.tpu as pltpu

S, DM, H, DH, M, SEG = 2048, 640, 32, 128, 8, 32
L = M + SEG
DF = DM // 2 + 1
R16 = 16
NB = S // R16
F32, BF16, U32 = jnp.float32, jnp.bfloat16, jnp.uint32
_NN = (((1,), (0,)), ((), ()))
_NT = (((1,), (1,)), ((), ()))


def _dot(a, b, dims=_NN):
    return jax.lax.dot_general(a, b, dims, preferred_element_type=F32)


def _rnd(v):
    return v.astype(BF16).astype(F32)


def _constants():
    b = np.arange(128)[:, None].astype(np.float64)
    j = np.arange(128)
    fd = np.zeros((5 * 128, 256))
    perm = np.zeros((DF, 384))
    cscale = np.zeros((1, 384))
    th = 2 * np.pi * b * (5 * j[None, :65]) / DM
    fd[:128, :65] = np.cos(th)
    fd[:128, 128:128 + 65] = -np.sin(th)
    fd[:128, 128] = 0.0
    fd[:128, 128 + 64] = 0.0
    perm[5 * j[:65], j[:65]] = 1.0
    cscale[0, :65] = 2.0
    cscale[0, 0] = cscale[0, 64] = 1.0
    for r in (1, 2):
        fp = np.where(j < 64, r + 5 * j, (5 - r) + 5 * (j - 64))
        f = np.where(j < 64, fp, DM - fp)
        sg = np.where(j < 64, 1.0, -1.0)[None, :]
        th = 2 * np.pi * b * f[None, :] / DM
        o = 128 + (r - 1) * 256
        fd[o:o + 128, :128] = np.cos(th)
        fd[o:o + 128, 128:] = -sg * np.sin(th)
        fd[o + 128:o + 256, :128] = np.sin(th)
        fd[o + 128:o + 256, 128:] = sg * np.cos(th)
        perm[fp, r * 128 + j] = 1.0
        cscale[0, r * 128:(r + 1) * 128] = 2.0
    cscale /= float(S * DM)
    fs = np.zeros((R16, 256, 256))
    g = np.arange(128)[:, None].astype(np.float64)
    bb = np.arange(128)[None, :].astype(np.float64)
    for r in range(R16):
        th = 2 * np.pi * ((r + R16 * g) * bb % S) / S
        c, s = np.cos(th), np.sin(th)
        fs[r] = np.block([[c, s], [-s, c]])
    bf = lambda a: np.asarray(a, dtype=BF16)
    return (bf(fd), bf(fd.T), bf(fs), bf(fs.transpose(0, 2, 1)), bf(perm.T), cscale.astype(np.float32))


def _fft4(x, sgn):
    (ar, ai), (br, bi), (cr, ci), (dr, di) = x
    s0r, s0i, d0r, d0i = ar + cr, ai + ci, ar - cr, ai - ci
    s1r, s1i, d1r, d1i = br + dr, bi + di, br - dr, bi - di
    p = (d0r + d1i, d0i - d1r)
    q = (d0r - d1i, d0i + d1r)
    y1, y3 = (p, q) if sgn < 0 else (q, p)
    return [(s0r + s1r, s0i + s1i), y1, (s0r - s1r, s0i - s1i), y3]


def _twiddle(v, e, sgn):
    if e == 0:
        return v
    vr, vi = v
    if e == 4:
        return (-vi, vr) if sgn > 0 else (vi, -vr)
    c, s = math.cos(2 * math.pi * e / 16), sgn * math.sin(2 * math.pi * e / 16)
    if e in (2, 6):
        if c * s > 0:
            return ((vr - vi) * c, (vr + vi) * c)
        return ((vr + vi) * c, (vi - vr) * c)
    return (vr * c - vi * s, vr * s + vi * c)


def _fft16(x, sgn):
    t = [_fft4([x[n2 + 4 * n1] for n1 in range(4)], sgn) for n2 in range(4)]
    y = [None] * 16
    for k1 in range(4):
        o = _fft4([_twiddle(t[n2][k1], n2 * k1, sgn) for n2 in range(4)], sgn)
        for k2 in range(4):
            y[k1 + 4 * k2] = o[k2]
    return y


_C1, _C2 = math.cos(2 * math.pi / 5), math.cos(4 * math.pi / 5)
_S1, _S2 = math.sin(2 * math.pi / 5), math.sin(4 * math.pi / 5)


def _rfft5(u):
    x = [u[:, a * 128:(a + 1) * 128] for a in range(5)]
    s1, s2, d1, d2 = x[1] + x[4], x[2] + x[3], x[4] - x[1], x[3] - x[2]
    return jnp.concatenate([
        x[0] + s1 + s2,
        x[0] + _C1 * s1 + _C2 * s2, _S1 * d1 + _S2 * d2,
        x[0] + _C2 * s1 + _C1 * s2, _S2 * d1 - _S1 * d2], axis=1)


def _irfft5(q):
    q0, q1r, q1i, q2r, q2i = [q[:, a * 128:(a + 1) * 128] for a in range(5)]
    e1, e2 = q0 + _C1 * q1r + _C2 * q2r, q0 + _C2 * q1r + _C1 * q2r
    o1, o2 = _S1 * q1i + _S2 * q2i, _S2 * q1i - _S1 * q2i
    return jnp.concatenate([q0 + q1r + q2r, e1 - o1, e2 - o2, e2 + o2, e1 + o1], axis=1)


def _layernorm(x):
    mu = jnp.mean(x, axis=1, keepdims=True)
    d = x - mu
    var = jnp.mean(d * d, axis=1, keepdims=True)
    return _rnd(d * jax.lax.rsqrt(var + 1e-5))


NCH = 5
WROWS = DM * H // NCH


def _kernel(x_hbm, mem_hbm, wq_hbm, wk_hbm, wv_hbm, wo_hbm, wr_hbm, wi_hbm,
            fd_hbm, fdt_hbm, fs_hbm, fst_hbm, perm_hbm, cs_hbm,
            o_ref,
            memb, stage, t32, wqkv, wostage, wo, wrb, wib, wp,
            fd, fdt, fs, fst, perm, cs,
            xs, us, u_buf, t_buf, v_buf, q_buf, sems):
    cnt = [0]

    def copy(src, dst):
        c = pltpu.make_async_copy(src, dst, sems.at[cnt[0]])
        cnt[0] += 1
        c.start()
        return c

    c_small = [copy(perm_hbm, perm), copy(cs_hbm, cs), copy(wr_hbm, wrb), copy(wi_hbm, wib)]
    c_x = [copy(x_hbm, o_ref), copy(mem_hbm, memb)]
    c_w = [[copy(w.at[pl.ds(c * WROWS, WROWS)], stage.at[i * NCH + c]) for c in range(NCH)]
           for i, w in enumerate((wq_hbm, wk_hbm, wv_hbm))]
    c_wo = [copy(wo_hbm.at[pl.ds(c * 1024, 1024)], wostage.at[pl.ds(c * 1024, 1024)]) for c in range(4)]
    c_b = [copy(fd_hbm, fd), copy(fs_hbm, fs), copy(fst_hbm, fst), copy(fdt_hbm, fdt)]

    for c in c_small:
        c.wait()
    pr = jax.lax.broadcasted_iota(jnp.int32, (256, 256), 0)
    pc = jax.lax.broadcasted_iota(jnp.int32, (256, 256), 1)
    shuffle = jnp.where(pc == (pr >> 4) + ((pr & 15) << 4), 1.0, 0.0).astype(BF16)

    def perm_filter(i, _):
        rows = pl.ds(pl.multiple_of(i * 256, 256), 256)
        for part, src in enumerate((wrb, wib)):
            w = _dot(shuffle, _dot(perm[...], src[:, rows]).astype(BF16), _NT) * cs[...]
            for r in range(R16):
                wp[r, pl.ds(pl.multiple_of(i * 16, 16), 16), part * 384:(part + 1) * 384] = w[r * 16:(r + 1) * 16]
    jax.lax.fori_loop(0, S // 256, perm_filter, None)

    for c in c_x:
        c.wait()

    def first_ln(i, _):
        rows = pl.ds(pl.multiple_of(i * 64, 64), 64)
        x = o_ref[rows, :].astype(F32)
        xs[rows, :] = x
        us[rows, :] = _layernorm(x)
    jax.lax.fori_loop(0, S // 64, first_ln, None)

    for i in range(3):
        for c in range(NCH):
            c_w[i][c].wait()

            def widen(j, _):
                t32[pl.ds(pl.multiple_of(j * 256, 256), 256), :] = pltpu.bitcast(
                    stage[i * NCH + c, pl.ds(pl.multiple_of(j * 512, 512), 512), :], U32)
            jax.lax.fori_loop(0, WROWS // 512, widen, None)

            def split(j, _):
                v = t32[pl.ds(j, 128, stride=H // 2), :]
                lo = pltpu.bitcast(v << 16, F32).astype(BF16)
                hi = pltpu.bitcast(v & np.uint32(0xFFFF0000), F32).astype(BF16)
                wqkv[2 * j, c * 64:(c + 1) * 64, i * 128:(i + 1) * 128] = pltpu.bitcast(lo, U32)
                wqkv[2 * j + 1, c * 64:(c + 1) * 64, i * 128:(i + 1) * 128] = pltpu.bitcast(hi, U32)
            jax.lax.fori_loop(0, H // 2, split, None, unroll=4)
    for c in range(4):
        c_wo[c].wait()

        def retile(j, _):
            rows = pl.ds(pl.multiple_of(c * 1024 + j * 128, 128), 128)
            wo[pl.ds(pl.multiple_of(c * 512 + j * 64, 64), 64), :] = pltpu.bitcast(wostage[rows, :], U32)
        jax.lax.fori_loop(0, 8, retile, None)

    row = jax.lax.broadcasted_iota(jnp.int32, (L, L), 0)
    col = jax.lax.broadcasted_iota(jnp.int32, (L, L), 1)
    mask = (row < M) | (row >= col)
    scale = DH ** -0.5
    G = 4

    def a_step(s, mem):
        rows = pl.ds(pl.multiple_of(s * SEG, SEG), SEG)
        hh = jnp.concatenate([mem, us[rows, :]], axis=0)
        qkv, sc, pp, oo = {}, {}, {}, {}
        acc = None
        for t in range(H + H // G):
            if t < H:
                qkv[t] = _dot(hh, pltpu.bitcast(wqkv[t], BF16))
            else:
                g = t - H
                o = jnp.concatenate([oo[g * G + i] for i in range(G)], axis=1)
                r = _dot(o, pltpu.bitcast(wo[g * G * 64:(g + 1) * G * 64, :], BF16))
                acc = r if acc is None else acc + r
            h = t - 2
            if 0 <= h < H:
                sc[h] = _dot(qkv[h][:, :128], qkv[h][:, 128:256].astype(BF16), _NT)
            h = t - 3
            if 0 <= h < H:
                z = jnp.where(mask, sc[h] * scale, -1e9)
                e = jnp.exp(z - jnp.max(z, axis=1, keepdims=True))
                pp[h] = e * (1.0 / jnp.sum(e, axis=1, keepdims=True))
            h = t - 5
            if 0 <= h < H:
                oo[h] = _dot(pp[h], qkv[h][:, 256:].astype(BF16))
        acc = _rnd(acc)
        xs[rows, :] = _rnd(xs[rows, :] + acc[M:])
        return acc[:M]

    def b_fwd(i, _):
        base = i * 16
        for a in range(R16):
            x = xs[pl.ds(pl.multiple_of(base + a * NB, 16), 16), :]
            v_buf[a * 16:(a + 1) * 16, :DM] = _rfft5(_layernorm(x)).astype(BF16)
        for r in range(3):
            k0, k1 = (0, 128) if r == 0 else (r * 256 - 128, r * 256 + 128)
            q_buf[:, r * 256:(r + 1) * 256] = _dot(v_buf[:, k0:k1], fd[k0:k1, :])
        for r in range(3):
            y = _fft16([(q_buf[a * 16:(a + 1) * 16, r * 256:r * 256 + 128],
                         q_buf[a * 16:(a + 1) * 16, r * 256 + 128:(r + 1) * 256])
                        for a in range(R16)], -1)
            for k in range(R16):
                t_buf[k, pl.ds(pl.multiple_of(base, 16), 16), r * 128:(r + 1) * 128] = y[k][0].astype(BF16)
                t_buf[k, pl.ds(pl.multiple_of(base + NB, 16), 16), r * 128:(r + 1) * 128] = y[k][1].astype(BF16)

    def b_mid(k, _):
        x = _dot(fs[k], t_buf[k])
        xr, xi = x[:NB], x[NB:]
        wr, wi = wp[k, :, :384], wp[k, :, 384:]
        y = jnp.concatenate([xr * wr - xi * wi, xr * wi + xi * wr], axis=0).astype(BF16)
        z = _dot(fst[k], y)
        rows = pl.ds(pl.multiple_of(k * NB, NB), NB)
        u_buf[rows, :384] = z[:NB]
        u_buf[rows, 384:] = z[NB:]

    def b_inv(i, _):
        base = i * 16
        for r in range(3):
            y = _fft16([(u_buf[pl.ds(pl.multiple_of(base + k * NB, 16), 16), r * 128:(r + 1) * 128],
                         u_buf[pl.ds(pl.multiple_of(base + k * NB, 16), 16), 384 + r * 128:384 + (r + 1) * 128])
                        for k in range(R16)], +1)
            for a in range(R16):
                v_buf[a * 16:(a + 1) * 16, r * 256:r * 256 + 128] = y[a][0].astype(BF16)
                v_buf[a * 16:(a + 1) * 16, r * 256 + 128:(r + 1) * 256] = y[a][1].astype(BF16)
        for r in range(3):
            k0, k1 = (0, 128) if r == 0 else (r * 256 - 128, r * 256 + 128)
            q_buf[:, k0:k1] = _dot(v_buf[:, r * 256:(r + 1) * 256], fdt[:, k0:k1])
        for a in range(R16):
            rows = pl.ds(pl.multiple_of(base + a * NB, 16), 16)
            x = (xs[rows, :] + _rnd(_irfft5(q_buf[a * 16:(a + 1) * 16, :DM]))).astype(BF16)
            o_ref[rows, :] = x
            x = x.astype(F32)
            xs[rows, :] = x
            us[rows, :] = _layernorm(x)

    def layer(l, _):
        jax.lax.fori_loop(0, S // SEG, a_step, memb[...].astype(F32))

        @pl.when(l == 0)
        def _():
            for c in c_b:
                c.wait()
        jax.lax.fori_loop(0, NB // 16, b_fwd, None)
        jax.lax.fori_loop(0, R16, b_mid, None, unroll=2)
        jax.lax.fori_loop(0, NB // 16, b_inv, None)
    jax.lax.fori_loop(0, 2, layer, None)


@functools.partial(jax.jit, static_argnames=("A_seg_len",))
def pallas_interleave_layers__memory_aug_recurrent_mem_tr__spectral_gfnet__prompt_kernel(
    A_x, A_mem0, A_Wq, A_Wk, A_Wv, A_Wo, A_seg_len, B_x, B_w_r, B_w_i,
):
    del B_x
    assert A_x.shape == (1, S, DM) and A_Wq.shape == (DM, H, DH) and int(A_seg_len) == SEG
    consts = _constants()
    vm = pltpu.VMEM
    out = pl.pallas_call(
        _kernel,
        out_shape=jax.ShapeDtypeStruct((S, DM), BF16),
        in_specs=[pl.BlockSpec(memory_space=pltpu.HBM)] * 14,
        out_specs=pl.BlockSpec(memory_space=pltpu.VMEM),
        scratch_shapes=[
            vm((M, DM), BF16),
            vm((3 * NCH, WROWS, DH), BF16),
            vm((WROWS // 2, DH), U32),
            vm((H, DM // 2, 3 * DH), U32),
            vm((H * DH, DM), BF16),
            vm((H * DH // 2, DM), U32),
            vm((DF, S), BF16), vm((DF, S), BF16),
            vm((R16, NB, 768), F32),
            vm((DM, 256), BF16), vm((256, DM), BF16),
            vm((R16, 256, 256), BF16), vm((R16, 256, 256), BF16),
            vm((384, DF), BF16), vm((1, 384), F32),
            vm((S, DM), F32), vm((S, DM), F32),
            vm((S, 768), F32),
            vm((R16, 256, 384), BF16),
            vm((256, 768), BF16),
            vm((256, 768), F32),
            pltpu.SemaphoreType.DMA((32,)),
        ],
        compiler_params=pltpu.CompilerParams(vmem_limit_bytes=110 * 2**20),
        name="rmt_gfnet",
    )(A_x.reshape(S, DM), A_mem0.reshape(M, DM),
      A_Wq.reshape(DM * H, DH), A_Wk.reshape(DM * H, DH), A_Wv.reshape(DM * H, DH),
      A_Wo.reshape(H * DH, DM), B_w_r.T, B_w_i.T, *consts)
    return out.reshape(1, S, DM)
```

```python
import functools
import math

import jax
import jax.numpy as jnp
import numpy as np
import jax.experimental.pallas as pl
import jax.experimental.pallas.tpu as pltpu

S, DM, H, DH, M, SEG = 2048, 640, 32, 128, 8, 32
L = M + SEG
DF = DM // 2 + 1
R16 = 16
NB = S // R16
F32, BF16, U32 = jnp.float32, jnp.bfloat16, jnp.uint32
_NN = (((1,), (0,)), ((), ()))
_NT = (((1,), (1,)), ((), ()))


def _dot(a, b, dims=_NN):
    return jax.lax.dot_general(a, b, dims, preferred_element_type=F32)


def _rnd(v):
    return v.astype(BF16).astype(F32)


def _constants():
    b = np.arange(128)[:, None].astype(np.float64)
    j = np.arange(128)
    fd = np.zeros((5 * 128, 256))
    perm = np.zeros((DF, 384))
    cscale = np.zeros((1, 384))
    th = 2 * np.pi * b * (5 * j[None, :65]) / DM
    fd[:128, :65] = np.cos(th)
    fd[:128, 128:128 + 65] = -np.sin(th)
    fd[:128, 128] = 0.0
    fd[:128, 128 + 64] = 0.0
    perm[5 * j[:65], j[:65]] = 1.0
    cscale[0, :65] = 2.0
    cscale[0, 0] = cscale[0, 64] = 1.0
    for r in (1, 2):
        fp = np.where(j < 64, r + 5 * j, (5 - r) + 5 * (j - 64))
        f = np.where(j < 64, fp, DM - fp)
        sg = np.where(j < 64, 1.0, -1.0)[None, :]
        th = 2 * np.pi * b * f[None, :] / DM
        o = 128 + (r - 1) * 256
        fd[o:o + 128, :128] = np.cos(th)
        fd[o:o + 128, 128:] = -sg * np.sin(th)
        fd[o + 128:o + 256, :128] = np.sin(th)
        fd[o + 128:o + 256, 128:] = sg * np.cos(th)
        perm[fp, r * 128 + j] = 1.0
        cscale[0, r * 128:(r + 1) * 128] = 2.0
    cscale /= float(S * DM)
    fs = np.zeros((R16, 256, 256))
    g = np.arange(128)[:, None].astype(np.float64)
    bb = np.arange(128)[None, :].astype(np.float64)
    for r in range(R16):
        th = 2 * np.pi * ((r + R16 * g) * bb % S) / S
        c, s = np.cos(th), np.sin(th)
        fs[r] = np.block([[c, s], [-s, c]])
    bf = lambda a: np.asarray(a, dtype=BF16)

    def pk(a):
        w = np.ascontiguousarray(bf(a)).view(np.uint16).astype(np.uint32)
        return w[..., 0::2, :] | (w[..., 1::2, :] << 16)
    return (pk(fd), pk(fd.T), pk(fs), pk(fs.transpose(0, 2, 1)), bf(perm.T), cscale.astype(np.float32))


def _fft4(x, sgn):
    (ar, ai), (br, bi), (cr, ci), (dr, di) = x
    s0r, s0i, d0r, d0i = ar + cr, ai + ci, ar - cr, ai - ci
    s1r, s1i, d1r, d1i = br + dr, bi + di, br - dr, bi - di
    p = (d0r + d1i, d0i - d1r)
    q = (d0r - d1i, d0i + d1r)
    y1, y3 = (p, q) if sgn < 0 else (q, p)
    return [(s0r + s1r, s0i + s1i), y1, (s0r - s1r, s0i - s1i), y3]


def _twiddle(v, e, sgn):
    if e == 0:
        return v
    vr, vi = v
    if e == 4:
        return (-vi, vr) if sgn > 0 else (vi, -vr)
    c, s = math.cos(2 * math.pi * e / 16), sgn * math.sin(2 * math.pi * e / 16)
    if e in (2, 6):
        if c * s > 0:
            return ((vr - vi) * c, (vr + vi) * c)
        return ((vr + vi) * c, (vi - vr) * c)
    return (vr * c - vi * s, vr * s + vi * c)


def _fft16(x, sgn):
    t = [_fft4([x[n2 + 4 * n1] for n1 in range(4)], sgn) for n2 in range(4)]
    y = [None] * 16
    for k1 in range(4):
        o = _fft4([_twiddle(t[n2][k1], n2 * k1, sgn) for n2 in range(4)], sgn)
        for k2 in range(4):
            y[k1 + 4 * k2] = o[k2]
    return y


_C1, _C2 = math.cos(2 * math.pi / 5), math.cos(4 * math.pi / 5)
_S1, _S2 = math.sin(2 * math.pi / 5), math.sin(4 * math.pi / 5)


def _rfft5(u):
    x = [u[:, a * 128:(a + 1) * 128] for a in range(5)]
    s1, s2, d1, d2 = x[1] + x[4], x[2] + x[3], x[4] - x[1], x[3] - x[2]
    return jnp.concatenate([
        x[0] + s1 + s2,
        x[0] + _C1 * s1 + _C2 * s2, _S1 * d1 + _S2 * d2,
        x[0] + _C2 * s1 + _C1 * s2, _S2 * d1 - _S1 * d2], axis=1)


def _irfft5(q):
    q0, q1r, q1i, q2r, q2i = [q[:, a * 128:(a + 1) * 128] for a in range(5)]
    e1, e2 = q0 + _C1 * q1r + _C2 * q2r, q0 + _C2 * q1r + _C1 * q2r
    o1, o2 = _S1 * q1i + _S2 * q2i, _S2 * q1i - _S1 * q2i
    return jnp.concatenate([q0 + q1r + q2r, e1 - o1, e2 - o2, e2 + o2, e1 + o1], axis=1)


def _layernorm(x):
    mu = jnp.mean(x, axis=1, keepdims=True)
    d = x - mu
    var = jnp.mean(d * d, axis=1, keepdims=True)
    return _rnd(d * jax.lax.rsqrt(var + 1e-5))


NCH = 5
WROWS = DM * H // NCH


NSEG = S // SEG
_KR = ((0, 128), (128, 384), (384, 640))


def _pack(v):
    return pltpu.bitcast(v.astype(BF16), U32)


def _unpack(v):
    return pltpu.bitcast(v, BF16)


def _rows(i, n):
    return pl.ds(i * n, n) if isinstance(i, int) else pl.ds(pl.multiple_of(i * n, n), n)


def _kernel(x_hbm, mem_hbm, wq_hbm, wk_hbm, wv_hbm, wo_hbm, wr_hbm, wi_hbm,
            fd_hbm, fdt_hbm, fs_hbm, fst_hbm, perm_hbm, cs_hbm,
            o_hbm,
            xio, memb, stage, t32, wqkv, wostage, wo, wrb, wib, wp,
            fd, fdt, fs, fst, perm, cs,
            xs, us, u_buf, t_buf, z_buf, sems):
    cnt = [0]

    def copy(src, dst):
        c = pltpu.make_async_copy(src, dst, sems.at[cnt[0]])
        cnt[0] += 1
        c.start()
        return c

    c_small = [copy(perm_hbm, perm), copy(cs_hbm, cs), copy(wr_hbm, wrb), copy(wi_hbm, wib)]
    c_w = [[copy(w.at[pl.ds(c * WROWS, WROWS)], stage.at[i * NCH + c]) for c in range(NCH)]
           for i, w in enumerate((wq_hbm, wk_hbm, wv_hbm))]
    c_wo = [copy(wo_hbm.at[pl.ds(c * 1024, 1024)], wostage.at[pl.ds(c * 1024, 1024)]) for c in range(4)]
    c_x = [copy(x_hbm, xio), copy(mem_hbm, memb), copy(fd_hbm, fd)]
    c_b = [copy(fs_hbm, fs), copy(fst_hbm, fst), copy(fdt_hbm, fdt)]

    for c in c_small:
        c.wait()
    pr = jax.lax.broadcasted_iota(jnp.int32, (256, 256), 0)
    pc = jax.lax.broadcasted_iota(jnp.int32, (256, 256), 1)
    shuffle = jnp.where(pc == (pr >> 4) + ((pr & 15) << 4), 1.0, 0.0).astype(BF16)

    def perm_filter(i, _):
        for part, src in enumerate((wrb, wib)):
            w = _dot(shuffle, _dot(perm[...], src[:, _rows(i, 256)]).astype(BF16), _NT) * cs[...]
            for r in range(R16):
                wp[r, _rows(i, 16), part * 384:(part + 1) * 384] = w[r * 16:(r + 1) * 16]
    jax.lax.fori_loop(0, S // 256, perm_filter, None)

    for i in range(3):
        for c in range(NCH):
            c_w[i][c].wait()

            def widen(j, _):
                t32[_rows(j, 256), :] = pltpu.bitcast(stage[i * NCH + c, _rows(j, 512), :], U32)
            jax.lax.fori_loop(0, WROWS // 512, widen, None)

            def split(j, _):
                v = t32[pl.ds(j, 128, stride=H // 2), :]
                wqkv[2 * j, c * 64:(c + 1) * 64, i * 128:(i + 1) * 128] = _pack(pltpu.bitcast(v << 16, F32))
                wqkv[2 * j + 1, c * 64:(c + 1) * 64, i * 128:(i + 1) * 128] = _pack(
                    pltpu.bitcast(v & np.uint32(0xFFFF0000), F32))
            jax.lax.fori_loop(0, H // 2, split, None, unroll=4)
    for c in range(4):
        c_wo[c].wait()

        def retile(j, _):
            wo[_rows(c * 8 + j, 64), :] = pltpu.bitcast(wostage[_rows(c * 8 + j, 128), :], U32)
        jax.lax.fori_loop(0, 8, retile, None)
    for c in c_x:
        c.wait()

    def fwd_vpu(i, n=SEG):
        return _rfft5(_layernorm(xs[_rows(i, n), :])).astype(BF16)

    def fwd_mxu(i, v, n=SEG):
        for r, (k0, k1) in enumerate(_KR):
            u = _dot(v[:, k0:k1], _unpack(fd[k0 // 2:k1 // 2, :]))
            u_buf[r, _rows(i, n), :] = u[:, :128]
            u_buf[3 + r, _rows(i, n), :] = u[:, 128:]

    def inv_mxu(i, n=SEG):
        return jnp.concatenate(
            [_dot(_unpack(z_buf[r, _rows(i, n // 2), :]), _unpack(fdt[:, k0:k1])) for r, (k0, k1) in enumerate(_KR)],
            axis=1)

    def inv_vpu(i, q, n=SEG):
        return (xs[_rows(i, n), :] + _rnd(_irfft5(q))).astype(BF16)

    def set_input(i, x):
        x = x.astype(F32)
        xs[_rows(i, SEG), :] = x
        us[_rows(i, SEG), :] = _layernorm(x)

    row = jax.lax.broadcasted_iota(jnp.int32, (L, L), 0)
    col = jax.lax.broadcasted_iota(jnp.int32, (L, L), 1)
    mask = (row < M) | (row >= col)
    scale = DH ** -0.5
    G = 4

    def a_step(s, mem, after_b):
        prv, nxt = jnp.maximum(s - 1, 0), jnp.minimum(s + 1, NSEG - 1)
        hh = jnp.concatenate([mem, us[_rows(s, SEG), :]], axis=0)
        qkv, sc, pp, oo = {}, {}, {}, {}
        acc = None
        for t in range(H + H // G):
            if t < H:
                qkv[t] = _dot(hh, _unpack(wqkv[t]))
            else:
                g = t - H
                o = jnp.concatenate([oo[g * G + i] for i in range(G)], axis=1)
                r = _dot(o, _unpack(wo[g * G * 64:(g + 1) * G * 64, :]))
                acc = r if acc is None else acc + r
            h = t - 2
            if 0 <= h < H:
                sc[h] = _dot(qkv[h][:, :128], qkv[h][:, 128:256].astype(BF16), _NT)
            h = t - 3
            if 0 <= h < H:
                z = jnp.where(mask, sc[h] * scale, -1e9)
                e = jnp.exp(z - jnp.max(z, axis=1, keepdims=True))
                pp[h] = e * (1.0 / jnp.sum(e, axis=1, keepdims=True))
            h = t - 5
            if 0 <= h < H:
                oo[h] = _dot(pp[h], qkv[h][:, 256:].astype(BF16))
            if t == 0 and after_b:
                q = inv_mxu(nxt)
            if t == 2:
                set_input(s + 1, inv_vpu(nxt, q) if after_b else xio[_rows(nxt, SEG), :])
            if t == H + 4:
                v = fwd_vpu(prv)
        fwd_mxu(prv, v)
        acc = _rnd(acc)
        xs[_rows(s, SEG), :] = _rnd(xs[_rows(s, SEG), :] + acc[M:])
        return acc[:M]

    def radix_fwd(r, j):
        y = _fft16([(u_buf[r, a * NB + j * 16:a * NB + (j + 1) * 16, :],
                     u_buf[3 + r, a * NB + j * 16:a * NB + (j + 1) * 16, :]) for a in range(R16)], -1)
        for k in range(R16):
            t_buf[r, k, j * 8:(j + 1) * 8, :] = _pack(y[k][0])
            t_buf[r, k, 64 + j * 8:64 + (j + 1) * 8, :] = _pack(y[k][1])

    def radix_inv(r, j):
        y = _fft16([(u_buf[r, k * NB + j * 16:k * NB + (j + 1) * 16, :],
                     u_buf[3 + r, k * NB + j * 16:k * NB + (j + 1) * 16, :]) for k in range(R16)], +1)
        for a in range(R16):
            z_buf[r, a * 64 + j * 8:a * 64 + (j + 1) * 8, :128] = _pack(y[a][0])
            z_buf[r, a * 64 + j * 8:a * 64 + (j + 1) * 8, 128:] = _pack(y[a][1])

    def dft_fwd(r, k):
        return _dot(_unpack(fs[k]), _unpack(t_buf[r, k]))

    def filt(r, k, x):
        xr, xi = x[:NB], x[NB:]
        wr, wi = wp[k, :, r * 128:(r + 1) * 128], wp[k, :, 384 + r * 128:384 + (r + 1) * 128]
        return jnp.concatenate([xr * wr - xi * wi, xr * wi + xi * wr], axis=0).astype(BF16)

    def dft_inv(r, k, y):
        z = _dot(_unpack(fst[k]), y)
        u_buf[r, k * NB:(k + 1) * NB, :] = z[:NB]
        u_buf[3 + r, k * NB:(k + 1) * NB, :] = z[NB:]

    def b_mid():
        ys = {}
        for t in range(-8, 33):
            if 0 <= t < 24:
                r, j = divmod(t, 8)
                xf = [dft_fwd(r, 2 * j + i) for i in range(2)]
            if 0 <= t - 1 < 24:
                r, j = divmod(t - 1, 8)
                for i in range(2):
                    dft_inv(r, 2 * j + i, ys.pop((r, 2 * j + i)))
            if 0 <= t < 24:
                r, j = divmod(t, 8)
                for i in range(2):
                    ys[r, 2 * j + i] = filt(r, 2 * j + i, xf[i])
            if 0 <= t + 8 < 24:
                radix_fwd(*divmod(t + 8, 8))
            if 0 <= t - 9 < 24:
                radix_inv(*divmod(t - 9, 8))

    mem0 = memb[...].astype(F32)
    set_input(0, xio[:SEG, :])
    a_first = functools.partial(a_step, after_b=False)
    a_second = functools.partial(a_step, after_b=True)
    jax.lax.fori_loop(0, NSEG, a_first, mem0)
    for c in c_b:
        c.wait()

    def layer(l, _):
        fwd_mxu(NSEG - 1, fwd_vpu(NSEG - 1))
        b_mid()

        @pl.when(l == 0)
        def _():
            set_input(0, inv_vpu(0, inv_mxu(0)))
            jax.lax.fori_loop(0, NSEG, a_second, mem0)
    jax.lax.fori_loop(0, 2, layer, None)

    c_out = []
    for i in range(S // 256):
        xio[_rows(i, 256), :] = inv_vpu(i, inv_mxu(i, 256), 256)
        c_out.append(copy(xio.at[_rows(i, 256)], o_hbm.at[_rows(i, 256)]))
    for c in c_out:
        c.wait()


@functools.partial(jax.jit, static_argnames=("A_seg_len",))
def pallas_interleave_layers__memory_aug_recurrent_mem_tr__spectral_gfnet__prompt_kernel(
    A_x, A_mem0, A_Wq, A_Wk, A_Wv, A_Wo, A_seg_len, B_x, B_w_r, B_w_i,
):
    del B_x
    assert A_x.shape == (1, S, DM) and A_Wq.shape == (DM, H, DH) and int(A_seg_len) == SEG
    consts = _constants()
    vm = pltpu.VMEM
    out = pl.pallas_call(
        _kernel,
        out_shape=jax.ShapeDtypeStruct((S, DM), BF16),
        in_specs=[pl.BlockSpec(memory_space=pltpu.HBM)] * 14,
        out_specs=pl.BlockSpec(memory_space=pltpu.HBM),
        scratch_shapes=[
            vm((S, DM), BF16),
            vm((M, DM), BF16),
            vm((3 * NCH, WROWS, DH), BF16),
            vm((WROWS // 2, DH), U32),
            vm((H, DM // 2, 3 * DH), U32),
            vm((H * DH, DM), BF16),
            vm((H * DH // 2, DM), U32),
            vm((DF, S), BF16), vm((DF, S), BF16),
            vm((R16, NB, 768), F32),
            vm((DM // 2, 256), U32), vm((128, DM), U32),
            vm((R16, 128, 256), U32), vm((R16, 128, 256), U32),
            vm((384, DF), BF16), vm((1, 384), F32),
            vm((S + SEG, DM), F32), vm((S + SEG, DM), F32),
            vm((6, S, 128), F32),
            vm((3, R16, 128, 128), U32),
            vm((3, S // 2, 256), U32),
            pltpu.SemaphoreType.DMA((37,)),
        ],
        compiler_params=pltpu.CompilerParams(vmem_limit_bytes=110 * 2**20),
        name="rmt_gfnet",
    )(A_x.reshape(S, DM), A_mem0.reshape(M, DM),
      A_Wq.reshape(DM * H, DH), A_Wk.reshape(DM * H, DH), A_Wv.reshape(DM * H, DH),
      A_Wo.reshape(H * DH, DM), B_w_r.T, B_w_i.T, *consts)
    return out.reshape(1, S, DM)
```

```python
import functools
import math

import jax
import jax.numpy as jnp
import numpy as np
import jax.experimental.pallas as pl
import jax.experimental.pallas.tpu as pltpu

S, DM, H, DH, M, SEG = 2048, 640, 32, 128, 8, 32
L = M + SEG
DF = DM // 2 + 1
R16 = 16
NB = S // R16
F32, BF16, U32 = jnp.float32, jnp.bfloat16, jnp.uint32
_NN = (((1,), (0,)), ((), ()))
_NT = (((1,), (1,)), ((), ()))


def _dot(a, b, dims=_NN):
    return jax.lax.dot_general(a, b, dims, preferred_element_type=F32)


def _rnd(v):
    return v.astype(BF16).astype(F32)


def _constants():
    b = np.arange(128)[:, None].astype(np.float64)
    j = np.arange(128)
    fd = np.zeros((5 * 128, 256))
    perm = np.zeros((DF, 384))
    cscale = np.zeros((1, 384))
    th = 2 * np.pi * b * (5 * j[None, :65]) / DM
    fd[:128, :65] = np.cos(th)
    fd[:128, 128:128 + 65] = -np.sin(th)
    fd[:128, 128] = 0.0
    fd[:128, 128 + 64] = 0.0
    perm[5 * j[:65], j[:65]] = 1.0
    cscale[0, :65] = 2.0
    cscale[0, 0] = cscale[0, 64] = 1.0
    for r in (1, 2):
        fp = np.where(j < 64, r + 5 * j, (5 - r) + 5 * (j - 64))
        f = np.where(j < 64, fp, DM - fp)
        sg = np.where(j < 64, 1.0, -1.0)[None, :]
        th = 2 * np.pi * b * f[None, :] / DM
        o = 128 + (r - 1) * 256
        fd[o:o + 128, :128] = np.cos(th)
        fd[o:o + 128, 128:] = -sg * np.sin(th)
        fd[o + 128:o + 256, :128] = np.sin(th)
        fd[o + 128:o + 256, 128:] = sg * np.cos(th)
        perm[fp, r * 128 + j] = 1.0
        cscale[0, r * 128:(r + 1) * 128] = 2.0
    cscale /= float(S * DM)
    fs = np.zeros((R16, 256, 256))
    g = np.arange(128)[:, None].astype(np.float64)
    bb = np.arange(128)[None, :].astype(np.float64)
    for r in range(R16):
        th = 2 * np.pi * ((r + R16 * g) * bb % S) / S
        c, s = np.cos(th), np.sin(th)
        fs[r] = np.block([[c, s], [-s, c]])
    bf = lambda a: np.asarray(a, dtype=BF16)

    il = np.arange(256) // 2 + 128 * (np.arange(256) % 2)

    def pk(a):
        w = np.ascontiguousarray(bf(a)).view(np.uint16).astype(np.uint32)
        return w[..., 0::2, :] | (w[..., 1::2, :] << 16)
    return (pk(fd), pk(fd.T), pk(fs[:, :, il]), pk(fs.transpose(0, 2, 1)[:, :, il]), bf(perm.T), cscale.astype(np.float32))


def _fft4(x, sgn):
    (ar, ai), (br, bi), (cr, ci), (dr, di) = x
    s0r, s0i, d0r, d0i = ar + cr, ai + ci, ar - cr, ai - ci
    s1r, s1i, d1r, d1i = br + dr, bi + di, br - dr, bi - di
    p = (d0r + d1i, d0i - d1r)
    q = (d0r - d1i, d0i + d1r)
    y1, y3 = (p, q) if sgn < 0 else (q, p)
    return [(s0r + s1r, s0i + s1i), y1, (s0r - s1r, s0i - s1i), y3]


def _twiddle(v, e, sgn):
    if e == 0:
        return v
    vr, vi = v
    if e == 4:
        return (-vi, vr) if sgn > 0 else (vi, -vr)
    c, s = math.cos(2 * math.pi * e / 16), sgn * math.sin(2 * math.pi * e / 16)
    if e in (2, 6):
        if c * s > 0:
            return ((vr - vi) * c, (vr + vi) * c)
        return ((vr + vi) * c, (vi - vr) * c)
    return (vr * c - vi * s, vr * s + vi * c)


def _fft16(x, sgn):
    t = [_fft4([x[n2 + 4 * n1] for n1 in range(4)], sgn) for n2 in range(4)]
    y = [None] * 16
    for k1 in range(4):
        o = _fft4([_twiddle(t[n2][k1], n2 * k1, sgn) for n2 in range(4)], sgn)
        for k2 in range(4):
            y[k1 + 4 * k2] = o[k2]
    return y


_C1, _C2 = math.cos(2 * math.pi / 5), math.cos(4 * math.pi / 5)
_S1, _S2 = math.sin(2 * math.pi / 5), math.sin(4 * math.pi / 5)


def _rfft5(u):
    x = [u[:, a * 128:(a + 1) * 128] for a in range(5)]
    s1, s2, d1, d2 = x[1] + x[4], x[2] + x[3], x[4] - x[1], x[3] - x[2]
    return jnp.concatenate([
        x[0] + s1 + s2,
        x[0] + _C1 * s1 + _C2 * s2, _S1 * d1 + _S2 * d2,
        x[0] + _C2 * s1 + _C1 * s2, _S2 * d1 - _S1 * d2], axis=1)


def _irfft5(q):
    q0, q1r, q1i, q2r, q2i = [q[:, a * 128:(a + 1) * 128] for a in range(5)]
    e1, e2 = q0 + _C1 * q1r + _C2 * q2r, q0 + _C2 * q1r + _C1 * q2r
    o1, o2 = _S1 * q1i + _S2 * q2i, _S2 * q1i - _S1 * q2i
    return jnp.concatenate([q0 + q1r + q2r, e1 - o1, e2 - o2, e2 + o2, e1 + o1], axis=1)


def _layernorm(x):
    mu = jnp.mean(x, axis=1, keepdims=True)
    d = x - mu
    var = jnp.mean(d * d, axis=1, keepdims=True)
    return _rnd(d * jax.lax.rsqrt(var + 1e-5))


NCH = 5
WROWS = DM * H // NCH


NSEG = S // SEG
_KR = ((0, 128), (128, 384), (384, 640))


def _pack(v):
    return pltpu.bitcast(v.astype(BF16), U32)


def _pack_complex(re, im):
    return pltpu.bitcast(pltpu.pack_elementwise([re, im], packed_dtype=BF16), U32)


def _unpack(v):
    return pltpu.bitcast(v, BF16)


def _rows(i, n):
    return pl.ds(i * n, n) if isinstance(i, int) else pl.ds(pl.multiple_of(i * n, n), n)


def _kernel(x_hbm, mem_hbm, wq_hbm, wk_hbm, wv_hbm, wo_hbm, wr_hbm, wi_hbm,
            fd_hbm, fdt_hbm, fs_hbm, fst_hbm, perm_hbm, cs_hbm,
            o_hbm,
            xio, memb, stage, t32, wqkv, wostage, wo, wrb, wib, wp,
            fd, fdt, fs, fst, perm, cs,
            xs, us, u_buf, t_buf, z_buf, zero, sems):
    cnt = [0]

    def copy(src, dst):
        c = pltpu.make_async_copy(src, dst, sems.at[cnt[0]])
        cnt[0] += 1
        c.start()
        return c

    c_small = [copy(perm_hbm, perm), copy(cs_hbm, cs), copy(wr_hbm, wrb), copy(wi_hbm, wib)]
    c_w = [[copy(w.at[pl.ds(c * WROWS, WROWS)], stage.at[i * NCH + c]) for c in range(NCH)]
           for i, w in enumerate((wq_hbm, wk_hbm, wv_hbm))]
    c_wo = [copy(wo_hbm.at[pl.ds(c * 1024, 1024)], wostage.at[pl.ds(c * 1024, 1024)]) for c in range(4)]
    c_x = [copy(x_hbm, xio), copy(mem_hbm, memb), copy(fd_hbm, fd)]
    c_b = [copy(fs_hbm, fs), copy(fst_hbm, fst), copy(fdt_hbm, fdt)]

    for c in c_small:
        c.wait()
    pr = jax.lax.broadcasted_iota(jnp.int32, (256, 256), 0)
    pc = jax.lax.broadcasted_iota(jnp.int32, (256, 256), 1)
    shuffle = jnp.where(pc == (pr >> 4) + ((pr & 15) << 4), 1.0, 0.0).astype(BF16)

    def perm_filter(i, _):
        for part, src in enumerate((wrb, wib)):
            w = _dot(shuffle, _dot(perm[...], src[:, _rows(i, 256)]).astype(BF16), _NT) * cs[...]
            for r in range(R16):
                for c in range(3):
                    wp[part * 3 + c, r, _rows(i, 16), :] = w[r * 16:(r + 1) * 16, c * 128:(c + 1) * 128]
    jax.lax.fori_loop(0, S // 256, perm_filter, None)

    for i in range(3):
        for c in range(NCH):
            c_w[i][c].wait()

            def widen(j, _):
                t32[_rows(j, 256), :] = pltpu.bitcast(stage[i * NCH + c, _rows(j, 512), :], U32)
            jax.lax.fori_loop(0, WROWS // 512, widen, None)

            def split(j, _):
                v = t32[pl.ds(j, 128, stride=H // 2), :]
                wqkv[2 * j, c * 64:(c + 1) * 64, i * 128:(i + 1) * 128] = _pack(pltpu.bitcast(v << 16, F32))
                wqkv[2 * j + 1, c * 64:(c + 1) * 64, i * 128:(i + 1) * 128] = _pack(
                    pltpu.bitcast(v & np.uint32(0xFFFF0000), F32))
            jax.lax.fori_loop(0, H // 2, split, None, unroll=4)
    for c in range(4):
        c_wo[c].wait()

        def retile(j, _):
            wo[_rows(c * 8 + j, 64), :] = pltpu.bitcast(wostage[_rows(c * 8 + j, 128), :], U32)
        jax.lax.fori_loop(0, 8, retile, None)
    for c in c_x:
        c.wait()

    def fwd_vpu(i, n=SEG):
        return _rfft5(_layernorm(xs[_rows(i, n), :]))

    def fwd_mxu(i, v, n=SEG):
        for r, (k0, k1) in enumerate(_KR):
            u_buf[r, _rows(i, n), :] = _dot(v[:, k0:k1], _unpack(fd[k0 // 2:k1 // 2, :]))

    def inv_mxu(i, n=SEG):
        return jnp.concatenate(
            [_dot(z_buf[r, _rows(i, n), :], _unpack(fdt[:, k0:k1])) for r, (k0, k1) in enumerate(_KR)],
            axis=1)

    def inv_vpu(i, q, n=SEG):
        return (xs[_rows(i, n), :] + _rnd(_irfft5(q))).astype(BF16)

    def set_input(i, x):
        x = x.astype(F32)
        xs[_rows(i, SEG), :] = x
        us[_rows(i, SEG), :] = _layernorm(x)

    row = jax.lax.broadcasted_iota(jnp.int32, (L, L), 0)
    col = jax.lax.broadcasted_iota(jnp.int32, (L, L), 1)
    mask = (row < M) | (row >= col)
    scale = DH ** -0.5
    G = 4

    def a_step(s, mem, after_b):
        prv, nxt = jnp.maximum(s - 1, 0), jnp.minimum(s + 1, NSEG - 1)
        hh = jnp.concatenate([mem, us[_rows(s, SEG), :]], axis=0)
        qkv, sc, pp, oo = {}, {}, {}, {}
        acc = None
        for t in range(H + H // G):
            if t < H:
                qkv[t] = _dot(hh, _unpack(wqkv[t]))
            else:
                g = t - H
                o = jnp.concatenate([oo[g * G + i] for i in range(G)], axis=1)
                r = _dot(o, _unpack(wo[g * G * 64:(g + 1) * G * 64, :]))
                acc = r if acc is None else acc + r
            h = t - 2
            if 0 <= h < H:
                sc[h] = _dot(qkv[h][:, :128], qkv[h][:, 128:256].astype(BF16), _NT)
            h = t - 3
            if 0 <= h < H:
                z = jnp.where(mask, sc[h] * scale, -1e9)
                e = jnp.exp(z - jnp.max(z, axis=1, keepdims=True))
                pp[h] = e * (1.0 / jnp.sum(e, axis=1, keepdims=True))
            h = t - 5
            if 0 <= h < H:
                oo[h] = _dot(pp[h], qkv[h][:, 256:].astype(BF16))
            if t == 0 and after_b:
                q = inv_mxu(nxt)
            if t == 2:
                set_input(s + 1, inv_vpu(nxt, q) if after_b else xio[_rows(nxt, SEG), :])
            if t == H + 4:
                v = fwd_vpu(prv)
        fwd_mxu(prv, v)
        xs[_rows(s, SEG), :] = _rnd(xs[_rows(s, SEG), :] + _rnd(acc[M:]))
        return acc[:M]

    def radix_fwd(r, j):
        y = _fft16([(u_buf[r, _rows(a * 16 + j, 8), :128], u_buf[r, _rows(a * 16 + j, 8), 128:])
                    for a in range(R16)], -1)
        for k in range(R16):
            t_buf[r, k, _rows(j, 8), :] = _pack_complex(*y[k])

    def radix_inv(r, j):
        y = _fft16([(z_buf[r, _rows(k * 16 + j, 8), :128], z_buf[r, _rows(k * 16 + j, 8), 128:])
                    for k in range(R16)], +1)
        for a in range(R16):
            z_buf[r, _rows(a * 16 + j, 8), :128] = y[a][0]
            z_buf[r, _rows(a * 16 + j, 8), 128:] = y[a][1]

    def dft_fwd(r, k):
        return _dot(_unpack(fs[k]), _unpack(t_buf[r, k]))

    def filt(r, k, x):
        xr, xi = x[:NB], x[NB:]
        wr, wi = wp[r, k], wp[3 + r, k]
        return _unpack(_pack_complex(xr * wr - xi * wi, xr * wi + xi * wr))

    def dft_inv(r, k, y):
        z = _dot(_unpack(fst[k]), y)
        z_buf[r, _rows(k, NB), :128] = z[:NB]
        z_buf[r, _rows(k, NB), 128:] = z[NB:]

    def b_mid():
        z0, z1, z2, z3 = zero[0], zero[1], zero[2], zero[3]
        ys = {}
        for t in range(-8, 33):
            if 0 <= t < 24:
                r, j = divmod(t, 8)
                xf = [dft_fwd(r + z0, 2 * j + i) for i in range(2)]
            for i in range(2):
                if 0 <= t - 9 < 24:
                    r, j = divmod(2 * (t - 9) + i, 16)
                    radix_inv(r + z1, j)
            if 0 <= t - 1 < 24:
                r, j = divmod(t - 1, 8)
                for i in range(2):
                    dft_inv(r + z2, 2 * j + i, ys.pop((r, 2 * j + i)))
            if 0 <= t < 24:
                r, j = divmod(t, 8)
                for i in range(2):
                    ys[r, 2 * j + i] = filt(r, 2 * j + i, xf[i])
            for i in range(2):
                if 0 <= t + 8 < 24:
                    r, j = divmod(2 * (t + 8) + i, 16)
                    radix_fwd(r + z3, j)

    for i in range(4):
        zero[i] = 0
    mem0 = memb[...].astype(F32)
    set_input(0, xio[:SEG, :])
    a_first = functools.partial(a_step, after_b=False)
    a_second = functools.partial(a_step, after_b=True)
    jax.lax.fori_loop(0, NSEG, a_first, mem0)
    for c in c_b:
        c.wait()

    def layer(l, _):
        fwd_mxu(NSEG - 1, fwd_vpu(NSEG - 1))
        b_mid()

        @pl.when(l == 0)
        def _():
            set_input(0, inv_vpu(0, inv_mxu(0)))
            jax.lax.fori_loop(0, NSEG, a_second, mem0)
    jax.lax.fori_loop(0, 2, layer, None)

    c_out = []
    for i in range(S // 256):
        xio[_rows(i, 256), :] = inv_vpu(i, inv_mxu(i, 256), 256)
        c_out.append(copy(xio.at[_rows(i, 256)], o_hbm.at[_rows(i, 256)]))
    for c in c_out:
        c.wait()


@functools.partial(jax.jit, static_argnames=("A_seg_len",))
def pallas_interleave_layers__memory_aug_recurrent_mem_tr__spectral_gfnet__prompt_kernel(
    A_x, A_mem0, A_Wq, A_Wk, A_Wv, A_Wo, A_seg_len, B_x, B_w_r, B_w_i,
):
    del B_x
    assert A_x.shape == (1, S, DM) and A_Wq.shape == (DM, H, DH) and int(A_seg_len) == SEG
    consts = _constants()
    vm = pltpu.VMEM
    out = pl.pallas_call(
        _kernel,
        out_shape=jax.ShapeDtypeStruct((S, DM), BF16),
        in_specs=[pl.BlockSpec(memory_space=pltpu.HBM)] * 14,
        out_specs=pl.BlockSpec(memory_space=pltpu.HBM),
        scratch_shapes=[
            vm((S, DM), BF16),
            vm((M, DM), BF16),
            vm((3 * NCH, WROWS, DH), BF16),
            vm((WROWS // 2, DH), U32),
            vm((H, DM // 2, 3 * DH), U32),
            vm((H * DH, DM), BF16),
            vm((H * DH // 2, DM), U32),
            vm((DF, S), BF16), vm((DF, S), BF16),
            vm((6, R16, NB, 128), F32),
            vm((DM // 2, 256), U32), vm((128, DM), U32),
            vm((R16, 128, 256), U32), vm((R16, 128, 256), U32),
            vm((384, DF), BF16), vm((1, 384), F32),
            vm((S + SEG, DM), F32), vm((S + SEG, DM), F32),
            vm((3, S, 256), F32),
            vm((3, R16, 128, 128), U32),
            vm((3, S, 256), F32),
            pltpu.SMEM((4,), jnp.int32),
            pltpu.SemaphoreType.DMA((37,)),
        ],
        compiler_params=pltpu.CompilerParams(vmem_limit_bytes=110 * 2**20),
        name="rmt_gfnet",
    )(A_x.reshape(S, DM), A_mem0.reshape(M, DM),
      A_Wq.reshape(DM * H, DH), A_Wk.reshape(DM * H, DH), A_Wv.reshape(DM * H, DH),
      A_Wo.reshape(H * DH, DM), B_w_r.T, B_w_i.T, *consts)
    return out.reshape(1, S, DM)
```

```python
import functools
import math

import jax
import jax.numpy as jnp
import numpy as np
import jax.experimental.pallas as pl
import jax.experimental.pallas.tpu as pltpu

S, DM, H, DH, M, SEG = 2048, 640, 32, 128, 8, 32
L = M + SEG
DF = DM // 2 + 1
R16 = 16
NB = S // R16
F32, BF16, U32 = jnp.float32, jnp.bfloat16, jnp.uint32
_NN = (((1,), (0,)), ((), ()))
_NT = (((1,), (1,)), ((), ()))


def _dot(a, b, dims=_NN):
    return jax.lax.dot_general(a, b, dims, preferred_element_type=F32)


def _rnd(v):
    return v.astype(BF16).astype(F32)


def _constants():
    b = np.arange(128)[:, None].astype(np.float64)
    j = np.arange(128)
    fd = np.zeros((5 * 128, 256))
    perm = np.zeros((DF, 384))
    cscale = np.zeros((1, 384))
    th = 2 * np.pi * b * (5 * j[None, :65]) / DM
    fd[:128, :65] = np.cos(th)
    fd[:128, 128:128 + 65] = -np.sin(th)
    fd[:128, 128] = 0.0
    fd[:128, 128 + 64] = 0.0
    perm[5 * j[:65], j[:65]] = 1.0
    cscale[0, :65] = 2.0
    cscale[0, 0] = cscale[0, 64] = 1.0
    for r in (1, 2):
        fp = np.where(j < 64, r + 5 * j, (5 - r) + 5 * (j - 64))
        f = np.where(j < 64, fp, DM - fp)
        sg = np.where(j < 64, 1.0, -1.0)[None, :]
        th = 2 * np.pi * b * f[None, :] / DM
        o = 128 + (r - 1) * 256
        fd[o:o + 128, :128] = np.cos(th)
        fd[o:o + 128, 128:] = -sg * np.sin(th)
        fd[o + 128:o + 256, :128] = np.sin(th)
        fd[o + 128:o + 256, 128:] = sg * np.cos(th)
        perm[fp, r * 128 + j] = 1.0
        cscale[0, r * 128:(r + 1) * 128] = 2.0
    cscale /= float(S * DM)
    fs = np.zeros((R16, 256, 256))
    g = np.arange(128)[:, None].astype(np.float64)
    bb = np.arange(128)[None, :].astype(np.float64)
    for r in range(R16):
        th = 2 * np.pi * ((r + R16 * g) * bb % S) / S
        c, s = np.cos(th), np.sin(th)
        fs[r] = np.block([[c, s], [-s, c]])
    bf = lambda a: np.asarray(a, dtype=BF16)

    il = np.arange(256) // 2 + 128 * (np.arange(256) % 2)

    def pk(a):
        w = np.ascontiguousarray(bf(a)).view(np.uint16).astype(np.uint32)
        return w[..., 0::2, :] | (w[..., 1::2, :] << 16)
    return (pk(fd), pk(fd.T), pk(fs[:, :, il]), pk(fs.transpose(0, 2, 1)[:, :, il]), bf(perm.T), cscale.astype(np.float32))


def _fft4(x, sgn):
    (ar, ai), (br, bi), (cr, ci), (dr, di) = x
    s0r, s0i, d0r, d0i = ar + cr, ai + ci, ar - cr, ai - ci
    s1r, s1i, d1r, d1i = br + dr, bi + di, br - dr, bi - di
    p = (d0r + d1i, d0i - d1r)
    q = (d0r - d1i, d0i + d1r)
    y1, y3 = (p, q) if sgn < 0 else (q, p)
    return [(s0r + s1r, s0i + s1i), y1, (s0r - s1r, s0i - s1i), y3]


def _twiddle(v, e, sgn):
    if e == 0:
        return v
    vr, vi = v
    if e == 4:
        return (-vi, vr) if sgn > 0 else (vi, -vr)
    c, s = math.cos(2 * math.pi * e / 16), sgn * math.sin(2 * math.pi * e / 16)
    if e in (2, 6):
        if c * s > 0:
            return ((vr - vi) * c, (vr + vi) * c)
        return ((vr + vi) * c, (vi - vr) * c)
    return (vr * c - vi * s, vr * s + vi * c)


def _fft16(x, sgn):
    t = [_fft4([x[n2 + 4 * n1] for n1 in range(4)], sgn) for n2 in range(4)]
    y = [None] * 16
    for k1 in range(4):
        o = _fft4([_twiddle(t[n2][k1], n2 * k1, sgn) for n2 in range(4)], sgn)
        for k2 in range(4):
            y[k1 + 4 * k2] = o[k2]
    return y


_C1, _C2 = math.cos(2 * math.pi / 5), math.cos(4 * math.pi / 5)
_S1, _S2 = math.sin(2 * math.pi / 5), math.sin(4 * math.pi / 5)


def _rfft5(u):
    x = [u[:, a * 128:(a + 1) * 128] for a in range(5)]
    s1, s2, d1, d2 = x[1] + x[4], x[2] + x[3], x[4] - x[1], x[3] - x[2]
    return jnp.concatenate([
        x[0] + s1 + s2,
        x[0] + _C1 * s1 + _C2 * s2, _S1 * d1 + _S2 * d2,
        x[0] + _C2 * s1 + _C1 * s2, _S2 * d1 - _S1 * d2], axis=1)


def _irfft5(q):
    q0, q1r, q1i, q2r, q2i = [q[:, a * 128:(a + 1) * 128] for a in range(5)]
    e1, e2 = q0 + _C1 * q1r + _C2 * q2r, q0 + _C2 * q1r + _C1 * q2r
    o1, o2 = _S1 * q1i + _S2 * q2i, _S2 * q1i - _S1 * q2i
    return jnp.concatenate([q0 + q1r + q2r, e1 - o1, e2 - o2, e2 + o2, e1 + o1], axis=1)


def _layernorm(x):
    mu = jnp.mean(x, axis=1, keepdims=True)
    d = x - mu
    var = jnp.mean(d * d, axis=1, keepdims=True)
    return _rnd(d * jax.lax.rsqrt(var + 1e-5))


NCH = 5
WROWS = DM * H // NCH


NSEG = S // SEG
LAG = (2, 3, 5)
UNROLL = 2
_KR = ((0, 128), (128, 384), (384, 640))


def _pack(v):
    return pltpu.bitcast(v.astype(BF16), U32)


def _pack_complex(re, im):
    return pltpu.bitcast(pltpu.pack_elementwise([re, im], packed_dtype=BF16), U32)


def _unpack(v):
    return pltpu.bitcast(v, BF16)


def _rows(i, n):
    return pl.ds(i * n, n) if isinstance(i, int) else pl.ds(pl.multiple_of(i * n, n), n)


def _kernel(x_hbm, mem_hbm, wq_hbm, wk_hbm, wv_hbm, wo_hbm, wr_hbm, wi_hbm,
            fd_hbm, fdt_hbm, fs_hbm, fst_hbm, perm_hbm, cs_hbm,
            o_hbm,
            xio, memb, stage, t32, wqkv, wostage, wo, wrb, wib, wp,
            fd, fdt, fs, fst, perm, cs,
            xs, us, u_buf, t_buf, z_buf, zero, sems):
    cnt = [0]

    def copy(src, dst):
        c = pltpu.make_async_copy(src, dst, sems.at[cnt[0]])
        cnt[0] += 1
        c.start()
        return c

    c_small = [copy(perm_hbm, perm), copy(cs_hbm, cs), copy(wr_hbm, wrb), copy(wi_hbm, wib)]
    c_w = [[copy(w.at[pl.ds(c * WROWS, WROWS)], stage.at[i * NCH + c]) for c in range(NCH)]
           for i, w in enumerate((wq_hbm, wk_hbm, wv_hbm))]
    c_wo = [copy(wo_hbm.at[pl.ds(c * 1024, 1024)], wostage.at[pl.ds(c * 1024, 1024)]) for c in range(4)]
    c_x = [copy(x_hbm, xio), copy(mem_hbm, memb), copy(fd_hbm, fd)]
    c_b = [copy(fs_hbm, fs), copy(fst_hbm, fst), copy(fdt_hbm, fdt)]

    for c in c_small:
        c.wait()
    pr = jax.lax.broadcasted_iota(jnp.int32, (256, 256), 0)
    pc = jax.lax.broadcasted_iota(jnp.int32, (256, 256), 1)
    shuffle = jnp.where(pc == (pr >> 4) + ((pr & 15) << 4), 1.0, 0.0).astype(BF16)

    def perm_filter(i, _):
        for part, src in enumerate((wrb, wib)):
            w = _dot(shuffle, _dot(perm[...], src[:, _rows(i, 256)]).astype(BF16), _NT) * cs[...]
            for r in range(R16):
                for c in range(3):
                    wp[part * 3 + c, r, _rows(i, 16), :] = w[r * 16:(r + 1) * 16, c * 128:(c + 1) * 128]
    jax.lax.fori_loop(0, S // 256, perm_filter, None)

    for i in range(3):
        for c in range(NCH):
            c_w[i][c].wait()

            def widen(j, _):
                t32[_rows(j, 256), :] = pltpu.bitcast(stage[i * NCH + c, _rows(j, 512), :], U32)
            jax.lax.fori_loop(0, WROWS // 512, widen, None)

            def split(j, _):
                v = t32[pl.ds(j, 128, stride=H // 2), :]
                wqkv[2 * j, c * 64:(c + 1) * 64, i * 128:(i + 1) * 128] = _pack(pltpu.bitcast(v << 16, F32))
                wqkv[2 * j + 1, c * 64:(c + 1) * 64, i * 128:(i + 1) * 128] = _pack(
                    pltpu.bitcast(v & np.uint32(0xFFFF0000), F32))
            jax.lax.fori_loop(0, H // 2, split, None, unroll=4)
    for c in range(4):
        c_wo[c].wait()

        def retile(j, _):
            wo[_rows(c * 8 + j, 64), :] = pltpu.bitcast(wostage[_rows(c * 8 + j, 128), :], U32)
        jax.lax.fori_loop(0, 8, retile, None)
    for c in c_x:
        c.wait()

    def fwd_vpu(i, n=SEG):
        return _rfft5(_layernorm(xs[_rows(i, n), :]))

    def fwd_mxu(i, v, n=SEG):
        for r, (k0, k1) in enumerate(_KR):
            u_buf[r, _rows(i, n), :] = _dot(v[:, k0:k1], _unpack(fd[k0 // 2:k1 // 2, :]))

    def inv_mxu(i, n=SEG):
        return jnp.concatenate(
            [_dot(z_buf[r, _rows(i, n), :], _unpack(fdt[:, k0:k1])) for r, (k0, k1) in enumerate(_KR)],
            axis=1)

    def inv_vpu(i, q, n=SEG):
        return (xs[_rows(i, n), :] + _rnd(_irfft5(q))).astype(BF16)

    def set_input(i, x):
        x = x.astype(F32)
        xs[_rows(i, SEG), :] = x
        us[_rows(i, SEG), :] = _layernorm(x)

    row = jax.lax.broadcasted_iota(jnp.int32, (L, L), 0)
    col = jax.lax.broadcasted_iota(jnp.int32, (L, L), 1)
    mask = (row >= SEG) | (col >= SEG) | (row >= col)
    scale = DH ** -0.5
    G = 4

    def a_step(s, mem, after_b):
        prv, nxt = jnp.maximum(s - 1, 0), jnp.minimum(s + 1, NSEG - 1)
        hh = jnp.concatenate([us[_rows(s, SEG), :], mem], axis=0)
        if after_b:
            q = inv_mxu(nxt)
        qkv, sc, pp, oo = {}, {}, {}, {}
        acc = None
        for t in range(H + H // G):
            if t < H:
                qkv[t] = _dot(hh, _unpack(wqkv[t]))
            else:
                g = t - H
                o = jnp.concatenate([oo[g * G + i] for i in range(G)], axis=1)
                o = jnp.concatenate([o[SEG:], o[:SEG]], axis=0)
                r = _dot(o, _unpack(wo[g * G * 64:(g + 1) * G * 64, :]))
                acc = r if acc is None else acc + r
            h = t - LAG[0]
            if 0 <= h < H:
                sc[h] = _dot(qkv[h][:, :128], qkv[h][:, 128:256].astype(BF16), _NT)
            h = t - LAG[1]
            if 0 <= h < H:
                z = jnp.where(mask, sc[h] * scale, -1e9)
                e = jnp.exp(z - jnp.max(z, axis=1, keepdims=True))
                pp[h] = e * (1.0 / jnp.sum(e, axis=1, keepdims=True))
            h = t - LAG[2]
            if 0 <= h < H:
                oo[h] = _dot(pp[h], qkv[h][:, 256:].astype(BF16))
            if t == 2:
                set_input(s + 1, inv_vpu(nxt, q) if after_b else xio[_rows(nxt, SEG), :])
            if t == H + 4:
                v = fwd_vpu(prv)
        fwd_mxu(prv, v)
        xs[_rows(s, SEG), :] = _rnd(xs[_rows(s, SEG), :] + _rnd(acc[M:]))
        return acc[:M]

    def radix_fwd(r, j):
        y = _fft16([(u_buf[r, _rows(a * 16 + j, 8), :128], u_buf[r, _rows(a * 16 + j, 8), 128:])
                    for a in range(R16)], -1)
        for k in range(R16):
            t_buf[r, k, _rows(j, 8), :] = _pack_complex(*y[k])

    def radix_inv(r, j):
        y = _fft16([(z_buf[r, _rows(k * 16 + j, 8), :128], z_buf[r, _rows(k * 16 + j, 8), 128:])
                    for k in range(R16)], +1)
        for a in range(R16):
            z_buf[r, _rows(a * 16 + j, 8), :128] = y[a][0]
            z_buf[r, _rows(a * 16 + j, 8), 128:] = y[a][1]

    def dft_fwd(r, k):
        return _dot(_unpack(fs[k]), _unpack(t_buf[r, k]))

    def filt(r, k, x):
        xr, xi = x[:NB], x[NB:]
        wr, wi = wp[r, k], wp[3 + r, k]
        return _unpack(_pack_complex(xr * wr - xi * wi, xr * wi + xi * wr))

    def dft_inv(r, k, y):
        z = _dot(_unpack(fst[k]), y)
        z_buf[r, _rows(k, NB), :128] = z[:NB]
        z_buf[r, _rows(k, NB), 128:] = z[NB:]

    def b_mid():
        z0, z1, z2, z3 = zero[0], zero[1], zero[2], zero[3]
        ys = {}
        for t in range(-8, 33):
            if 0 <= t < 24:
                r, j = divmod(t, 8)
                xf = [dft_fwd(r + z0, 2 * j + i) for i in range(2)]
            for i in range(2):
                if 0 <= t - 9 < 24:
                    r, j = divmod(2 * (t - 9) + i, 16)
                    radix_inv(r + z1, j)
            if 0 <= t - 1 < 24:
                r, j = divmod(t - 1, 8)
                for i in range(2):
                    dft_inv(r + z2, 2 * j + i, ys.pop((r, 2 * j + i)))
            if 0 <= t < 24:
                r, j = divmod(t, 8)
                for i in range(2):
                    ys[r, 2 * j + i] = filt(r, 2 * j + i, xf[i])
            for i in range(2):
                if 0 <= t + 8 < 24:
                    r, j = divmod(2 * (t + 8) + i, 16)
                    radix_fwd(r + z3, j)

    for i in range(4):
        zero[i] = 0
    mem0 = memb[...].astype(F32)
    set_input(0, xio[:SEG, :])

    def a_steps(i, mem, after_b):
        for u in range(UNROLL):
            mem = a_step(i * UNROLL + u, mem, after_b)
        return mem
    a_first = functools.partial(a_steps, after_b=False)
    a_second = functools.partial(a_steps, after_b=True)
    jax.lax.fori_loop(0, NSEG // UNROLL, a_first, mem0)
    for c in c_b:
        c.wait()

    def layer(l, _):
        fwd_mxu(NSEG - 1, fwd_vpu(NSEG - 1))
        b_mid()

        @pl.when(l == 0)
        def _():
            set_input(0, inv_vpu(0, inv_mxu(0)))
            jax.lax.fori_loop(0, NSEG // UNROLL, a_second, mem0)
    jax.lax.fori_loop(0, 2, layer, None)

    c_out = []
    for i in range(S // 256):
        xio[_rows(i, 256), :] = inv_vpu(i, inv_mxu(i, 256), 256)
        c_out.append(copy(xio.at[_rows(i, 256)], o_hbm.at[_rows(i, 256)]))
    for c in c_out:
        c.wait()


@functools.partial(jax.jit, static_argnames=("A_seg_len",))
def pallas_interleave_layers__memory_aug_recurrent_mem_tr__spectral_gfnet__prompt_kernel(
    A_x, A_mem0, A_Wq, A_Wk, A_Wv, A_Wo, A_seg_len, B_x, B_w_r, B_w_i,
):
    del B_x
    assert A_x.shape == (1, S, DM) and A_Wq.shape == (DM, H, DH) and int(A_seg_len) == SEG
    consts = _constants()
    vm = pltpu.VMEM
    out = pl.pallas_call(
        _kernel,
        out_shape=jax.ShapeDtypeStruct((S, DM), BF16),
        in_specs=[pl.BlockSpec(memory_space=pltpu.HBM)] * 14,
        out_specs=pl.BlockSpec(memory_space=pltpu.HBM),
        scratch_shapes=[
            vm((S, DM), BF16),
            vm((M, DM), BF16),
            vm((3 * NCH, WROWS, DH), BF16),
            vm((WROWS // 2, DH), U32),
            vm((H, DM // 2, 3 * DH), U32),
            vm((H * DH, DM), BF16),
            vm((H * DH // 2, DM), U32),
            vm((DF, S), BF16), vm((DF, S), BF16),
            vm((6, R16, NB, 128), F32),
            vm((DM // 2, 256), U32), vm((128, DM), U32),
            vm((R16, 128, 256), U32), vm((R16, 128, 256), U32),
            vm((384, DF), BF16), vm((1, 384), F32),
            vm((S + SEG, DM), F32), vm((S + SEG, DM), F32),
            vm((3, S, 256), F32),
            vm((3, R16, 128, 128), U32),
            vm((3, S, 256), F32),
            pltpu.SMEM((4,), jnp.int32),
            pltpu.SemaphoreType.DMA((37,)),
        ],
        compiler_params=pltpu.CompilerParams(vmem_limit_bytes=110 * 2**20),
        name="rmt_gfnet",
    )(A_x.reshape(S, DM), A_mem0.reshape(M, DM),
      A_Wq.reshape(DM * H, DH), A_Wk.reshape(DM * H, DH), A_Wv.reshape(DM * H, DH),
      A_Wo.reshape(H * DH, DM), B_w_r.T, B_w_i.T, *consts)
    return out.reshape(1, S, DM)
```

```python
import functools
import math

import jax
import jax.numpy as jnp
import numpy as np
import jax.experimental.pallas as pl
import jax.experimental.pallas.tpu as pltpu

S, DM, H, DH, M, SEG = 2048, 640, 32, 128, 8, 32
L = M + SEG
DF = DM // 2 + 1
R16 = 16
NB = S // R16
F32, BF16, U32 = jnp.float32, jnp.bfloat16, jnp.uint32
_NN = (((1,), (0,)), ((), ()))
_NT = (((1,), (1,)), ((), ()))


def _dot(a, b, dims=_NN):
    return jax.lax.dot_general(a, b, dims, preferred_element_type=F32)


def _rnd(v):
    return v.astype(BF16).astype(F32)


def _constants():
    b = np.arange(128)[:, None].astype(np.float64)
    j = np.arange(128)
    fd = np.zeros((5 * 128, 256))
    th = 2 * np.pi * b * (5 * j[None, :65]) / DM
    fd[:128, :65] = np.cos(th)
    fd[:128, 128:128 + 65] = -np.sin(th)
    fd[:128, 128] = 0.0
    fd[:128, 128 + 64] = 0.0
    for r in (1, 2):
        fp = np.where(j < 64, r + 5 * j, (5 - r) + 5 * (j - 64))
        f = np.where(j < 64, fp, DM - fp)
        sg = np.where(j < 64, 1.0, -1.0)[None, :]
        th = 2 * np.pi * b * f[None, :] / DM
        o = 128 + (r - 1) * 256
        fd[o:o + 128, :128] = np.cos(th)
        fd[o:o + 128, 128:] = -sg * np.sin(th)
        fd[o + 128:o + 256, :128] = np.sin(th)
        fd[o + 128:o + 256, 128:] = sg * np.cos(th)
    fs = np.zeros((R16, 256, 256))
    g = np.arange(128)[:, None].astype(np.float64)
    bb = np.arange(128)[None, :].astype(np.float64)
    for r in range(R16):
        th = 2 * np.pi * ((r + R16 * g) * bb % S) / S
        c, s = np.cos(th), np.sin(th)
        fs[r] = np.block([[c, s], [-s, c]])
    bf = lambda a: np.asarray(a, dtype=BF16)

    il = np.arange(256) // 2 + 128 * (np.arange(256) % 2)

    def pk(a):
        w = np.ascontiguousarray(bf(a)).view(np.uint16).astype(np.uint32)
        return w[..., 0::2, :] | (w[..., 1::2, :] << 16)
    return (pk(fd), pk(fd.T), pk(fs[:, :, il]), pk(fs.transpose(0, 2, 1)[:, :, il]))


def _fft4(x, sgn):
    (ar, ai), (br, bi), (cr, ci), (dr, di) = x
    s0r, s0i, d0r, d0i = ar + cr, ai + ci, ar - cr, ai - ci
    s1r, s1i, d1r, d1i = br + dr, bi + di, br - dr, bi - di
    p = (d0r + d1i, d0i - d1r)
    q = (d0r - d1i, d0i + d1r)
    y1, y3 = (p, q) if sgn < 0 else (q, p)
    return [(s0r + s1r, s0i + s1i), y1, (s0r - s1r, s0i - s1i), y3]


def _twiddle(v, e, sgn):
    if e == 0:
        return v
    vr, vi = v
    if e == 4:
        return (-vi, vr) if sgn > 0 else (vi, -vr)
    c, s = math.cos(2 * math.pi * e / 16), sgn * math.sin(2 * math.pi * e / 16)
    if e in (2, 6):
        if c * s > 0:
            return ((vr - vi) * c, (vr + vi) * c)
        return ((vr + vi) * c, (vi - vr) * c)
    return (vr * c - vi * s, vr * s + vi * c)


def _fft16(x, sgn):
    t = [_fft4([x[n2 + 4 * n1] for n1 in range(4)], sgn) for n2 in range(4)]
    y = [None] * 16
    for k1 in range(4):
        o = _fft4([_twiddle(t[n2][k1], n2 * k1, sgn) for n2 in range(4)], sgn)
        for k2 in range(4):
            y[k1 + 4 * k2] = o[k2]
    return y


_C1, _C2 = math.cos(2 * math.pi / 5), math.cos(4 * math.pi / 5)
_S1, _S2 = math.sin(2 * math.pi / 5), math.sin(4 * math.pi / 5)


def _rfft5(u):
    x = [u[:, a * 128:(a + 1) * 128] for a in range(5)]
    s1, s2, d1, d2 = x[1] + x[4], x[2] + x[3], x[4] - x[1], x[3] - x[2]
    return jnp.concatenate([
        x[0] + s1 + s2,
        x[0] + _C1 * s1 + _C2 * s2, _S1 * d1 + _S2 * d2,
        x[0] + _C2 * s1 + _C1 * s2, _S2 * d1 - _S1 * d2], axis=1)


def _irfft5(q):
    q0, q1r, q1i, q2r, q2i = [q[:, a * 128:(a + 1) * 128] for a in range(5)]
    e1, e2 = q0 + _C1 * q1r + _C2 * q2r, q0 + _C2 * q1r + _C1 * q2r
    o1, o2 = _S1 * q1i + _S2 * q2i, _S2 * q1i - _S1 * q2i
    return jnp.concatenate([q0 + q1r + q2r, e1 - o1, e2 - o2, e2 + o2, e1 + o1], axis=1)


def _layernorm(x):
    mu = jnp.mean(x, axis=1, keepdims=True)
    d = x - mu
    var = jnp.mean(d * d, axis=1, keepdims=True)
    return _rnd(d * jax.lax.rsqrt(var + 1e-5))


NCH = 5
WROWS = DM * H // NCH


NWO = 16
WOROWS = H * DH // NWO
NSEG = S // SEG
LAG = (2, 3, 5)
UNROLL = 2
_KR = ((0, 128), (128, 384), (384, 640))


def _pack(v):
    return pltpu.bitcast(v.astype(BF16), U32)


def _pack_complex(re, im):
    return pltpu.bitcast(pltpu.pack_elementwise([re, im], packed_dtype=BF16), U32)


def _unpack(v):
    return pltpu.bitcast(v, BF16)


def _rows(i, n):
    return pl.ds(i * n, n) if isinstance(i, int) else pl.ds(pl.multiple_of(i * n, n), n)


def _kernel(x_hbm, mem_hbm, wq_hbm, wk_hbm, wv_hbm, wo_hbm, wr_hbm, wi_hbm,
            fd_hbm, fdt_hbm, fs_hbm, fst_hbm,
            o_hbm,
            xio, memb, stage, t32, wqkv, wostage, wo, wb, wt, wt2, wp,
            fd, fdt, fs, fst,
            xs, us, u_buf, t_buf, z_buf, zero, sems):
    cnt = [0]

    def copy(src, dst):
        c = pltpu.make_async_copy(src, dst, sems.at[cnt[0]])
        cnt[0] += 1
        c.start()
        return c

    head, rest = pl.ds(0, 128), pl.ds(128, S - 128)
    c_head = [copy(x_hbm.at[head], xio.at[head]), copy(mem_hbm, memb), copy(fd_hbm, fd),
              copy(wr_hbm.at[:, head], wb.at[0, :, head]), copy(wi_hbm.at[:, head], wb.at[1, :, head])]
    w_sem = cnt[0]
    for i, w in enumerate((wq_hbm, wk_hbm, wv_hbm)):
        for c in range(NCH):
            copy(w.at[pl.ds(c * WROWS, WROWS)], stage.at[i * NCH + c])
    wo_sem = cnt[0]
    for c in range(NWO):
        copy(wo_hbm.at[_rows(c, WOROWS)], wostage.at[_rows(c, WOROWS)])
    c_rest = [copy(x_hbm.at[rest], xio.at[rest]),
              copy(wr_hbm.at[:, rest], wb.at[0, :, rest]), copy(wi_hbm.at[:, rest], wb.at[1, :, rest])]
    c_b = [copy(fs_hbm, fs), copy(fst_hbm, fst), copy(fdt_hbm, fdt)]

    def set_input(i, x):
        x = x.astype(F32)
        xs[_rows(i, SEG), :] = x
        us[_rows(i, SEG), :] = _layernorm(x)

    for c in c_head:
        c.wait()
    set_input(0, xio[:SEG, :])

    for i in range(3):
        def w_chunk(c, _):
            n = i * NCH + c
            pltpu.make_async_copy(stage.at[n], stage.at[n], sems.at[w_sem + n]).wait()

            def widen(j, _):
                t32[_rows(j, 256), :] = pltpu.bitcast(stage[n, _rows(j, 512), :], U32)
            jax.lax.fori_loop(0, WROWS // 512, widen, None)

            def split(j, _):
                v = t32[pl.ds(j, 128, stride=H // 2), :]
                wqkv[2 * j, _rows(c, 64), i * 128:(i + 1) * 128] = _pack(pltpu.bitcast(v << 16, F32))
                wqkv[2 * j + 1, _rows(c, 64), i * 128:(i + 1) * 128] = _pack(
                    pltpu.bitcast(v & np.uint32(0xFFFF0000), F32))
            jax.lax.fori_loop(0, H // 2, split, None, unroll=2)
        jax.lax.fori_loop(0, NCH, w_chunk, None)

    def wo_chunk(c, _):
        blk = wostage.at[_rows(c, WOROWS)]
        pltpu.make_async_copy(blk, blk, sems.at[wo_sem + c]).wait()
        wo[_rows(c, WOROWS // 2), :] = pltpu.bitcast(wostage[_rows(c, WOROWS), :], U32)
    jax.lax.fori_loop(0, NWO, wo_chunk, None)

    def filter_prep(i):
        part, blk = i % 2, i // 2
        wt[:DF, :] = wb[part, :, _rows(blk, 128)].astype(F32)
        lane = jax.lax.broadcasted_iota(jnp.int32, (1, 128), 1)
        sub = jax.lax.broadcasted_iota(jnp.int32, (64, 128), 0)
        for r in range(3):
            lo = wt[pl.ds(r, 64, stride=5), :]
            if r == 0:
                hi = jnp.where(sub == 0, wt[DF - 1:DF, :], 0.0)
                c = jnp.where((lane == 0) | (lane == 64), 1.0 / (S * DM), 2.0 / (S * DM))
            else:
                hi = wt[pl.ds(5 - r, 64, stride=5), :]
                c = 2.0 / (S * DM)
            wt2[r] = jnp.concatenate([lo, hi], axis=0).T * c
            for k in range(R16):
                wp[part * 3 + r, k, _rows(blk, 8), :] = wt2[r, pl.ds(k, 8, stride=R16), :]

    def fwd_vpu(i, n=SEG):
        return _rfft5(_layernorm(xs[_rows(i, n), :]))

    def fwd_mxu(i, v, n=SEG):
        for r, (k0, k1) in enumerate(_KR):
            u_buf[r, _rows(i, n), :] = _dot(v[:, k0:k1], _unpack(fd[k0 // 2:k1 // 2, :]))

    def inv_mxu(i, n=SEG):
        return jnp.concatenate(
            [_dot(z_buf[r, _rows(i, n), :], _unpack(fdt[:, k0:k1])) for r, (k0, k1) in enumerate(_KR)],
            axis=1)

    def inv_vpu(i, q, n=SEG):
        return (xs[_rows(i, n), :] + _rnd(_irfft5(q))).astype(BF16)

    row = jax.lax.broadcasted_iota(jnp.int32, (L, L), 0)
    col = jax.lax.broadcasted_iota(jnp.int32, (L, L), 1)
    mask = (row >= SEG) | (col >= SEG) | (row >= col)
    scale = DH ** -0.5
    G = 4

    def a_step(s, mem, after_b, job):
        prv, nxt = jnp.maximum(s - 1, 0), jnp.minimum(s + 1, NSEG - 1)
        hh = jnp.concatenate([us[_rows(s, SEG), :], mem], axis=0)
        if after_b:
            q = inv_mxu(nxt)
        qkv, sc, pp, oo = {}, {}, {}, {}
        acc = None
        for t in range(H + H // G):
            if t < H:
                qkv[t] = _dot(hh, _unpack(wqkv[t]))
            else:
                g = t - H
                o = jnp.concatenate([oo[g * G + i] for i in range(G)], axis=1)
                o = jnp.concatenate([o[SEG:], o[:SEG]], axis=0)
                r = _dot(o, _unpack(wo[g * G * 64:(g + 1) * G * 64, :]))
                acc = r if acc is None else acc + r
            h = t - LAG[0]
            if 0 <= h < H:
                sc[h] = _dot(qkv[h][:, :128], qkv[h][:, 128:256].astype(BF16), _NT)
            h = t - LAG[1]
            if 0 <= h < H:
                z = jnp.where(mask, sc[h] * scale, -1e9)
                e = jnp.exp(z - jnp.max(z, axis=1, keepdims=True))
                pp[h] = e * (1.0 / jnp.sum(e, axis=1, keepdims=True))
            h = t - LAG[2]
            if 0 <= h < H:
                oo[h] = _dot(pp[h], qkv[h][:, 256:].astype(BF16))
            if t == 2:
                set_input(s + 1, inv_vpu(nxt, q) if after_b else xio[_rows(nxt, SEG), :])
            if t == 12 and job is not None:
                job()
            if t == H + 4:
                v = fwd_vpu(prv)
        fwd_mxu(prv, v)
        xs[_rows(s, SEG), :] = _rnd(xs[_rows(s, SEG), :] + _rnd(acc[M:]))
        return acc[:M]

    def radix_fwd(r, j):
        y = _fft16([(u_buf[r, _rows(a * 16 + j, 8), :128], u_buf[r, _rows(a * 16 + j, 8), 128:])
                    for a in range(R16)], -1)
        for k in range(R16):
            t_buf[r, k, _rows(j, 8), :] = _pack_complex(*y[k])

    def radix_inv(r, j):
        y = _fft16([(z_buf[r, _rows(k * 16 + j, 8), :128], z_buf[r, _rows(k * 16 + j, 8), 128:])
                    for k in range(R16)], +1)
        for a in range(R16):
            z_buf[r, _rows(a * 16 + j, 8), :128] = y[a][0]
            z_buf[r, _rows(a * 16 + j, 8), 128:] = y[a][1]

    def dft_fwd(r, k):
        return _dot(_unpack(fs[k]), _unpack(t_buf[r, k]))

    def filt(r, k, x):
        xr, xi = x[:NB], x[NB:]
        wr, wi = wp[r, k], wp[3 + r, k]
        return _unpack(_pack_complex(xr * wr - xi * wi, xr * wi + xi * wr))

    def dft_inv(r, k, y):
        z = _dot(_unpack(fst[k]), y)
        z_buf[r, _rows(k, NB), :128] = z[:NB]
        z_buf[r, _rows(k, NB), 128:] = z[NB:]

    def b_mid():
        z0, z1, z2, z3 = zero[0], zero[1], zero[2], zero[3]
        ys = {}
        for t in range(-8, 33):
            if 0 <= t < 24:
                r, j = divmod(t, 8)
                xf = [dft_fwd(r + z0, 2 * j + i) for i in range(2)]
            for i in range(2):
                if 0 <= t - 9 < 24:
                    r, j = divmod(2 * (t - 9) + i, 16)
                    radix_inv(r + z1, j)
            if 0 <= t - 1 < 24:
                r, j = divmod(t - 1, 8)
                for i in range(2):
                    dft_inv(r + z2, 2 * j + i, ys.pop((r, 2 * j + i)))
            if 0 <= t < 24:
                r, j = divmod(t, 8)
                for i in range(2):
                    ys[r, 2 * j + i] = filt(r, 2 * j + i, xf[i])
            for i in range(2):
                if 0 <= t + 8 < 24:
                    r, j = divmod(2 * (t + 8) + i, 16)
                    radix_fwd(r + z3, j)

    for i in range(4):
        zero[i] = 0
    mem0 = memb[...].astype(F32)

    def a_steps(i, mem, after_b):
        if not after_b:
            @pl.when(i == 1)
            def _():
                for c in c_rest:
                    c.wait()
        for u in range(UNROLL):
            job = functools.partial(filter_prep, i * (UNROLL // 2) + u // 2) if u % 2 == 0 and not after_b else None
            mem = a_step(i * UNROLL + u, mem, after_b, job)
        return mem
    a_first = functools.partial(a_steps, after_b=False)
    a_second = functools.partial(a_steps, after_b=True)
    jax.lax.fori_loop(0, NSEG // UNROLL, a_first, mem0)
    for c in c_b:
        c.wait()

    def layer(l, _):
        fwd_mxu(NSEG - 1, fwd_vpu(NSEG - 1))
        b_mid()

        @pl.when(l == 0)
        def _():
            set_input(0, inv_vpu(0, inv_mxu(0)))
            jax.lax.fori_loop(0, NSEG // UNROLL, a_second, mem0)
    jax.lax.fori_loop(0, 2, layer, None)

    c_out = []
    for i in range(S // 256):
        xio[_rows(i, 256), :] = inv_vpu(i, inv_mxu(i, 256), 256)
        c_out.append(copy(xio.at[_rows(i, 256)], o_hbm.at[_rows(i, 256)]))
    for c in c_out:
        c.wait()


@functools.partial(jax.jit, static_argnames=("A_seg_len",))
def pallas_interleave_layers__memory_aug_recurrent_mem_tr__spectral_gfnet__prompt_kernel(
    A_x, A_mem0, A_Wq, A_Wk, A_Wv, A_Wo, A_seg_len, B_x, B_w_r, B_w_i,
):
    del B_x
    assert A_x.shape == (1, S, DM) and A_Wq.shape == (DM, H, DH) and int(A_seg_len) == SEG
    consts = _constants()
    vm = pltpu.VMEM
    out = pl.pallas_call(
        _kernel,
        out_shape=jax.ShapeDtypeStruct((S, DM), BF16),
        in_specs=[pl.BlockSpec(memory_space=pltpu.HBM)] * 12,
        out_specs=pl.BlockSpec(memory_space=pltpu.HBM),
        scratch_shapes=[
            vm((S, DM), BF16),
            vm((M, DM), BF16),
            vm((3 * NCH, WROWS, DH), BF16),
            vm((WROWS // 2, DH), U32),
            vm((H, DM // 2, 3 * DH), U32),
            vm((H * DH, DM), BF16),
            vm((H * DH // 2, DM), U32),
            vm((2, DF, S), BF16),
            vm((328, 128), F32), vm((3, 128, 128), F32),
            vm((6, R16, NB, 128), F32),
            vm((DM // 2, 256), U32), vm((128, DM), U32),
            vm((R16, 128, 256), U32), vm((R16, 128, 256), U32),
            vm((S + SEG, DM), F32), vm((S + SEG, DM), F32),
            vm((3, S, 256), F32),
            vm((3, R16, 128, 128), U32),
            vm((3, S, 256), F32),
            pltpu.SMEM((4,), jnp.int32),
            pltpu.SemaphoreType.DMA((19 + 3 * NCH + NWO,)),
        ],
        compiler_params=pltpu.CompilerParams(vmem_limit_bytes=110 * 2**20),
        name="rmt_gfnet",
    )(A_x.reshape(S, DM), A_mem0.reshape(M, DM),
      A_Wq.reshape(DM * H, DH), A_Wk.reshape(DM * H, DH), A_Wv.reshape(DM * H, DH),
      A_Wo.reshape(H * DH, DM), B_w_r.T, B_w_i.T, *consts)
    return out.reshape(1, S, DM)
```

```python
import functools
import math

import jax
import jax.numpy as jnp
import numpy as np
import jax.experimental.pallas as pl
import jax.experimental.pallas.tpu as pltpu

S, DM, H, DH, M, SEG = 2048, 640, 32, 128, 8, 32
L = M + SEG
DF = DM // 2 + 1
R16 = 16
NB = S // R16
F32, BF16, U32 = jnp.float32, jnp.bfloat16, jnp.uint32
_NN = (((1,), (0,)), ((), ()))
_NT = (((1,), (1,)), ((), ()))


def _dot(a, b, dims=_NN):
    return jax.lax.dot_general(a, b, dims, preferred_element_type=F32)


def _rnd(v):
    return v.astype(BF16).astype(F32)


def _constants():
    b = np.arange(128)[:, None].astype(np.float64)
    j = np.arange(128)
    fd = np.zeros((5 * 128, 256))
    th = 2 * np.pi * b * (5 * j[None, :65]) / DM
    fd[:128, :65] = np.cos(th)
    fd[:128, 128:128 + 65] = -np.sin(th)
    fd[:128, 128] = 0.0
    fd[:128, 128 + 64] = 0.0
    for r in (1, 2):
        fp = np.where(j < 64, r + 5 * j, (5 - r) + 5 * (j - 64))
        f = np.where(j < 64, fp, DM - fp)
        sg = np.where(j < 64, 1.0, -1.0)[None, :]
        th = 2 * np.pi * b * f[None, :] / DM
        o = 128 + (r - 1) * 256
        fd[o:o + 128, :128] = np.cos(th)
        fd[o:o + 128, 128:] = -sg * np.sin(th)
        fd[o + 128:o + 256, :128] = np.sin(th)
        fd[o + 128:o + 256, 128:] = sg * np.cos(th)
    fs = np.zeros((R16, 256, 256))
    g = np.arange(128)[:, None].astype(np.float64)
    bb = np.arange(128)[None, :].astype(np.float64)
    for r in range(R16):
        th = 2 * np.pi * ((r + R16 * g) * bb % S) / S
        c, s = np.cos(th), np.sin(th)
        fs[r] = np.block([[c, s], [-s, c]])
    bf = lambda a: np.asarray(a, dtype=BF16)

    il = np.arange(256) // 2 + 128 * (np.arange(256) % 2)

    def pk(a):
        w = np.ascontiguousarray(bf(a)).view(np.uint16).astype(np.uint32)
        return w[..., 0::2, :] | (w[..., 1::2, :] << 16)
    return (pk(fd), pk(fd.T), pk(fs[:, :, il]), pk(fs.transpose(0, 2, 1)[:, :, il]))


def _fft4(x, sgn):
    (ar, ai), (br, bi), (cr, ci), (dr, di) = x
    s0r, s0i, d0r, d0i = ar + cr, ai + ci, ar - cr, ai - ci
    s1r, s1i, d1r, d1i = br + dr, bi + di, br - dr, bi - di
    p = (d0r + d1i, d0i - d1r)
    q = (d0r - d1i, d0i + d1r)
    y1, y3 = (p, q) if sgn < 0 else (q, p)
    return [(s0r + s1r, s0i + s1i), y1, (s0r - s1r, s0i - s1i), y3]


def _twiddle(v, e, sgn):
    if e == 0:
        return v
    vr, vi = v
    if e == 4:
        return (-vi, vr) if sgn > 0 else (vi, -vr)
    c, s = math.cos(2 * math.pi * e / 16), sgn * math.sin(2 * math.pi * e / 16)
    if e in (2, 6):
        if c * s > 0:
            return ((vr - vi) * c, (vr + vi) * c)
        return ((vr + vi) * c, (vi - vr) * c)
    return (vr * c - vi * s, vr * s + vi * c)


def _fft16(x, sgn):
    t = [_fft4([x[n2 + 4 * n1] for n1 in range(4)], sgn) for n2 in range(4)]
    y = [None] * 16
    for k1 in range(4):
        o = _fft4([_twiddle(t[n2][k1], n2 * k1, sgn) for n2 in range(4)], sgn)
        for k2 in range(4):
            y[k1 + 4 * k2] = o[k2]
    return y


_C1, _C2 = math.cos(2 * math.pi / 5), math.cos(4 * math.pi / 5)
_S1, _S2 = math.sin(2 * math.pi / 5), math.sin(4 * math.pi / 5)


def _rfft5(u):
    x = [u[:, a * 128:(a + 1) * 128] for a in range(5)]
    s1, s2, d1, d2 = x[1] + x[4], x[2] + x[3], x[4] - x[1], x[3] - x[2]
    return jnp.concatenate([
        x[0] + s1 + s2,
        x[0] + _C1 * s1 + _C2 * s2, _S1 * d1 + _S2 * d2,
        x[0] + _C2 * s1 + _C1 * s2, _S2 * d1 - _S1 * d2], axis=1)


def _irfft5(q):
    q0, q1r, q1i, q2r, q2i = [q[:, a * 128:(a + 1) * 128] for a in range(5)]
    e1, e2 = q0 + _C1 * q1r + _C2 * q2r, q0 + _C2 * q1r + _C1 * q2r
    o1, o2 = _S1 * q1i + _S2 * q2i, _S2 * q1i - _S1 * q2i
    return jnp.concatenate([q0 + q1r + q2r, e1 - o1, e2 - o2, e2 + o2, e1 + o1], axis=1)


def _layernorm(x):
    mu = jnp.mean(x, axis=1, keepdims=True)
    d = x - mu
    var = jnp.mean(d * d, axis=1, keepdims=True)
    return _rnd(d * jax.lax.rsqrt(var + 1e-5))


NCH = 5
WROWS = DM * H // NCH


NWO = 16
WOROWS = H * DH // NWO
NSEG = S // SEG
JT = (20, 10, 13)
LAG = (2, 3, 6)
PAIR = 2 * SEG
NPAIR = S // PAIR
_KR = ((0, 128), (128, 384), (384, 640))


def _pack(v):
    return pltpu.bitcast(v.astype(BF16), U32)


def _pack_complex(re, im):
    return pltpu.bitcast(pltpu.pack_elementwise([re, im], packed_dtype=BF16), U32)


def _unpack(v):
    return pltpu.bitcast(v, BF16)


def _rows(i, n):
    return pl.ds(i * n, n) if isinstance(i, int) else pl.ds(pl.multiple_of(i * n, n), n)


def _kernel(x_hbm, mem_hbm, wq_hbm, wk_hbm, wv_hbm, wo_hbm, wr_hbm, wi_hbm,
            fd_hbm, fdt_hbm, fs_hbm, fst_hbm,
            o_hbm,
            xio, memb, stage, t32, wqkv, wostage, wo, wb, wt, wt2, wp,
            fd, fdt, fs, fst,
            xs, us, u_buf, t_buf, z_buf, zero, sems):
    cnt = [0]

    def copy(src, dst):
        c = pltpu.make_async_copy(src, dst, sems.at[cnt[0]])
        cnt[0] += 1
        c.start()
        return c

    head, rest = pl.ds(0, 128), pl.ds(128, S - 128)
    c_head = [copy(x_hbm.at[head], xio.at[head]), copy(mem_hbm, memb), copy(fd_hbm, fd),
              copy(wr_hbm.at[:, head], wb.at[0, :, head]), copy(wi_hbm.at[:, head], wb.at[1, :, head])]
    w_sem = cnt[0]
    for i, w in enumerate((wq_hbm, wk_hbm, wv_hbm)):
        for c in range(NCH):
            copy(w.at[pl.ds(c * WROWS, WROWS)], stage.at[i * NCH + c])
    wo_sem = cnt[0]
    for c in range(NWO):
        copy(wo_hbm.at[_rows(c, WOROWS)], wostage.at[_rows(c, WOROWS)])
    c_rest = [copy(x_hbm.at[rest], xio.at[rest]),
              copy(wr_hbm.at[:, rest], wb.at[0, :, rest]), copy(wi_hbm.at[:, rest], wb.at[1, :, rest])]
    c_b = [copy(fs_hbm, fs), copy(fst_hbm, fst), copy(fdt_hbm, fdt)]

    def set_input(i, x):
        x = x.astype(F32)
        xs[_rows(i, PAIR), :] = x
        us[_rows(i, PAIR), :] = _layernorm(x)

    for c in c_head:
        c.wait()
    set_input(0, xio[:PAIR, :])

    for i in range(3):
        def w_chunk(c, _):
            n = i * NCH + c
            pltpu.make_async_copy(stage.at[n], stage.at[n], sems.at[w_sem + n]).wait()

            def widen(j, _):
                t32[_rows(j, 256), :] = pltpu.bitcast(stage[n, _rows(j, 512), :], U32)
            jax.lax.fori_loop(0, WROWS // 512, widen, None)

            def split(j, _):
                v = t32[pl.ds(j, 128, stride=H // 2), :]
                wqkv[2 * j, _rows(c, 64), i * 128:(i + 1) * 128] = _pack(pltpu.bitcast(v << 16, F32))
                wqkv[2 * j + 1, _rows(c, 64), i * 128:(i + 1) * 128] = _pack(
                    pltpu.bitcast(v & np.uint32(0xFFFF0000), F32))
            jax.lax.fori_loop(0, H // 2, split, None, unroll=2)
        jax.lax.fori_loop(0, NCH, w_chunk, None)

    def wo_chunk(c, _):
        blk = wostage.at[_rows(c, WOROWS)]
        pltpu.make_async_copy(blk, blk, sems.at[wo_sem + c]).wait()
        wo[_rows(c, WOROWS // 2), :] = pltpu.bitcast(wostage[_rows(c, WOROWS), :], U32)
    jax.lax.fori_loop(0, NWO, wo_chunk, None)

    def filter_prep(i):
        part, blk = i % 2, i // 2
        wt[:DF, :] = wb[part, :, _rows(blk, 128)].astype(F32)
        lane = jax.lax.broadcasted_iota(jnp.int32, (1, 128), 1)
        sub = jax.lax.broadcasted_iota(jnp.int32, (64, 128), 0)
        for r in range(3):
            lo = wt[pl.ds(r, 64, stride=5), :]
            if r == 0:
                hi = jnp.where(sub == 0, wt[DF - 1:DF, :], 0.0)
                c = jnp.where((lane == 0) | (lane == 64), 1.0 / (S * DM), 2.0 / (S * DM))
            else:
                hi = wt[pl.ds(5 - r, 64, stride=5), :]
                c = 2.0 / (S * DM)
            wt2[r] = jnp.concatenate([lo, hi], axis=0).T * c
            for k in range(R16):
                wp[part * 3 + r, k, _rows(blk, 8), :] = wt2[r, pl.ds(k, 8, stride=R16), :]

    def fwd_vpu(i, n=PAIR):
        return _rfft5(_layernorm(xs[_rows(i, n), :]))

    def fwd_mxu(i, v, n=PAIR):
        for r, (k0, k1) in enumerate(_KR):
            u_buf[r, _rows(i, n), :] = _dot(v[:, k0:k1], _unpack(fd[k0 // 2:k1 // 2, :]))

    def inv_mxu(i, n=PAIR):
        return jnp.concatenate(
            [_dot(z_buf[r, _rows(i, n), :], _unpack(fdt[:, k0:k1])) for r, (k0, k1) in enumerate(_KR)],
            axis=1)

    def inv_vpu(i, q, n=PAIR):
        return (xs[_rows(i, n), :] + _rnd(_irfft5(q))).astype(BF16)

    row = jax.lax.broadcasted_iota(jnp.int32, (L, L), 0)
    col = jax.lax.broadcasted_iota(jnp.int32, (L, L), 1)
    mask = (row >= SEG) | (col >= SEG) | (row >= col)
    scale = DH ** -0.5
    G = 4

    def a_step(s, mem, jobs):
        hh = jnp.concatenate([us[_rows(s, SEG), :], mem], axis=0)
        qkv, sc, pp, oo = {}, {}, {}, {}
        acc = None
        for t in range(H + H // G):
            if t < H:
                qkv[t] = _dot(hh, _unpack(wqkv[t]))
            else:
                g = t - H
                o = jnp.concatenate([oo[g * G + i] for i in range(G)], axis=1)
                o = jnp.concatenate([o[SEG:], o[:SEG]], axis=0)
                r = _dot(o, _unpack(wo[g * G * 64:(g + 1) * G * 64, :]))
                acc = r if acc is None else acc + r
            h = t - LAG[0]
            if 0 <= h < H:
                sc[h] = _dot(qkv[h][:, :128], qkv[h][:, 128:256].astype(BF16), _NT)
            h = t - LAG[1]
            if 0 <= h < H:
                z = jnp.where(mask, sc[h] * scale, -1e9)
                e = jnp.exp(z - jnp.max(z, axis=1, keepdims=True))
                pp[h] = e * (1.0 / jnp.sum(e, axis=1, keepdims=True))
            h = t - LAG[2]
            if 0 <= h < H:
                oo[h] = _dot(pp[h], qkv[h][:, 256:].astype(BF16))
            if t in jobs:
                jobs[t]()
        xs[_rows(s, SEG), :] = _rnd(xs[_rows(s, SEG), :] + _rnd(acc[M:]))
        return acc[:M]

    def radix_fwd(r, j):
        y = _fft16([(u_buf[r, _rows(a * 16 + j, 8), :128], u_buf[r, _rows(a * 16 + j, 8), 128:])
                    for a in range(R16)], -1)
        for k in range(R16):
            t_buf[r, k, _rows(j, 8), :] = _pack_complex(*y[k])

    def radix_inv(r, j):
        y = _fft16([(z_buf[r, _rows(k * 16 + j, 8), :128], z_buf[r, _rows(k * 16 + j, 8), 128:])
                    for k in range(R16)], +1)
        for a in range(R16):
            z_buf[r, _rows(a * 16 + j, 8), :128] = y[a][0]
            z_buf[r, _rows(a * 16 + j, 8), 128:] = y[a][1]

    def dft_fwd(r, k):
        return _dot(_unpack(fs[k]), _unpack(t_buf[r, k]))

    def filt(r, k, x):
        xr, xi = x[:NB], x[NB:]
        wr, wi = wp[r, k], wp[3 + r, k]
        return _unpack(_pack_complex(xr * wr - xi * wi, xr * wi + xi * wr))

    def dft_inv(r, k, y):
        z = _dot(_unpack(fst[k]), y)
        z_buf[r, _rows(k, NB), :128] = z[:NB]
        z_buf[r, _rows(k, NB), 128:] = z[NB:]

    def b_mid():
        z0, z1, z2, z3 = zero[0], zero[1], zero[2], zero[3]
        ys = {}
        for t in range(-8, 33):
            if 0 <= t < 24:
                r, j = divmod(t, 8)
                xf = [dft_fwd(r + z0, 2 * j + i) for i in range(2)]
            for i in range(2):
                if 0 <= t - 9 < 24:
                    r, j = divmod(2 * (t - 9) + i, 16)
                    radix_inv(r + z1, j)
            if 0 <= t - 1 < 24:
                r, j = divmod(t - 1, 8)
                for i in range(2):
                    dft_inv(r + z2, 2 * j + i, ys.pop((r, 2 * j + i)))
            if 0 <= t < 24:
                r, j = divmod(t, 8)
                for i in range(2):
                    ys[r, 2 * j + i] = filt(r, 2 * j + i, xf[i])
            for i in range(2):
                if 0 <= t + 8 < 24:
                    r, j = divmod(2 * (t + 8) + i, 16)
                    radix_fwd(r + z3, j)

    for i in range(4):
        zero[i] = 0
    mem0 = memb[...].astype(F32)

    def a_steps(i, mem, after_b):
        if not after_b:
            @pl.when(i == 1)
            def _():
                for c in c_rest:
                    c.wait()
        prv, nxt = jnp.maximum(i - 1, 0), jnp.minimum(i + 1, NPAIR - 1)
        st = {}
        first = {JT[0]: lambda: st.update(v=fwd_vpu(prv)), H + H // G - 1: lambda: fwd_mxu(prv, st["v"])}
        if after_b:
            second = {JT[1]: lambda: st.update(q=inv_mxu(nxt)), JT[2]: lambda: set_input(i + 1, inv_vpu(nxt, st["q"]))}
        else:
            second = {JT[1]: lambda: set_input(i + 1, xio[_rows(nxt, PAIR), :]), 12: lambda: filter_prep(i)}
        return a_step(2 * i + 1, a_step(2 * i, mem, first), second)
    a_first = functools.partial(a_steps, after_b=False)
    a_second = functools.partial(a_steps, after_b=True)
    jax.lax.fori_loop(0, NPAIR, a_first, mem0)
    for c in c_b:
        c.wait()

    def layer(l, _):
        fwd_mxu(NPAIR - 1, fwd_vpu(NPAIR - 1))
        b_mid()

        @pl.when(l == 0)
        def _():
            set_input(0, inv_vpu(0, inv_mxu(0)))
            jax.lax.fori_loop(0, NPAIR, a_second, mem0)
    jax.lax.fori_loop(0, 2, layer, None)

    c_out = []
    for i in range(S // 256):
        xio[_rows(i, 256), :] = inv_vpu(i, inv_mxu(i, 256), 256)
        c_out.append(copy(xio.at[_rows(i, 256)], o_hbm.at[_rows(i, 256)]))
    for c in c_out:
        c.wait()


@functools.partial(jax.jit, static_argnames=("A_seg_len",))
def pallas_interleave_layers__memory_aug_recurrent_mem_tr__spectral_gfnet__prompt_kernel(
    A_x, A_mem0, A_Wq, A_Wk, A_Wv, A_Wo, A_seg_len, B_x, B_w_r, B_w_i,
):
    del B_x
    assert A_x.shape == (1, S, DM) and A_Wq.shape == (DM, H, DH) and int(A_seg_len) == SEG
    consts = _constants()
    vm = pltpu.VMEM
    out = pl.pallas_call(
        _kernel,
        out_shape=jax.ShapeDtypeStruct((S, DM), BF16),
        in_specs=[pl.BlockSpec(memory_space=pltpu.HBM)] * 12,
        out_specs=pl.BlockSpec(memory_space=pltpu.HBM),
        scratch_shapes=[
            vm((S, DM), BF16),
            vm((M, DM), BF16),
            vm((3 * NCH, WROWS, DH), BF16),
            vm((WROWS // 2, DH), U32),
            vm((H, DM // 2, 3 * DH), U32),
            vm((H * DH, DM), BF16),
            vm((H * DH // 2, DM), U32),
            vm((2, DF, S), BF16),
            vm((328, 128), F32), vm((3, 128, 128), F32),
            vm((6, R16, NB, 128), F32),
            vm((DM // 2, 256), U32), vm((128, DM), U32),
            vm((R16, 128, 256), U32), vm((R16, 128, 256), U32),
            vm((S + PAIR, DM), F32), vm((S + PAIR, DM), F32),
            vm((3, S, 256), F32),
            vm((3, R16, 128, 128), U32),
            vm((3, S, 256), F32),
            pltpu.SMEM((4,), jnp.int32),
            pltpu.SemaphoreType.DMA((19 + 3 * NCH + NWO,)),
        ],
        compiler_params=pltpu.CompilerParams(vmem_limit_bytes=110 * 2**20),
        name="rmt_gfnet",
    )(A_x.reshape(S, DM), A_mem0.reshape(M, DM),
      A_Wq.reshape(DM * H, DH), A_Wk.reshape(DM * H, DH), A_Wv.reshape(DM * H, DH),
      A_Wo.reshape(H * DH, DM), B_w_r.T, B_w_i.T, *consts)
    return out.reshape(1, S, DM)
```

```python
import functools
import math

import jax
import jax.numpy as jnp
import numpy as np
import jax.experimental.pallas as pl
import jax.experimental.pallas.tpu as pltpu

S, DM, H, DH, M, SEG = 2048, 640, 32, 128, 8, 32
L = M + SEG
DF = DM // 2 + 1
RS = 32
NB = S // RS
F32, BF16, U32 = jnp.float32, jnp.bfloat16, jnp.uint32
_NN = (((1,), (0,)), ((), ()))
_NT = (((1,), (1,)), ((), ()))


def _dot(a, b, dims=_NN):
    return jax.lax.dot_general(a, b, dims, preferred_element_type=F32)


def _rnd(v):
    return v.astype(BF16).astype(F32)


def _constants():
    b = np.arange(128)[:, None].astype(np.float64)
    j = np.arange(128)
    fd = np.zeros((5 * 128, 256))
    th = 2 * np.pi * b * (5 * j[None, :65]) / DM
    fd[:128, :65] = np.cos(th)
    fd[:128, 128:128 + 65] = -np.sin(th)
    fd[:128, 128] = 0.0
    fd[:128, 128 + 64] = 0.0
    for r in (1, 2):
        fp = np.where(j < 64, r + 5 * j, (5 - r) + 5 * (j - 64))
        f = np.where(j < 64, fp, DM - fp)
        sg = np.where(j < 64, 1.0, -1.0)[None, :]
        th = 2 * np.pi * b * f[None, :] / DM
        o = 128 + (r - 1) * 256
        fd[o:o + 128, :128] = np.cos(th)
        fd[o:o + 128, 128:] = -sg * np.sin(th)
        fd[o + 128:o + 256, :128] = np.sin(th)
        fd[o + 128:o + 256, 128:] = sg * np.cos(th)
    fs = np.zeros((RS, 2 * NB, 2 * NB))
    g = np.arange(NB)[:, None].astype(np.float64)
    bb = np.arange(NB)[None, :].astype(np.float64)
    for r in range(RS):
        th = 2 * np.pi * ((r + RS * g) * bb % S) / S
        c, s = np.cos(th), np.sin(th)
        fs[r] = np.block([[c, s], [-s, c]])
    bf = lambda a: np.asarray(a, dtype=BF16)

    il = np.arange(2 * NB) // 2 + NB * (np.arange(2 * NB) % 2)

    def pk(a):
        w = np.ascontiguousarray(bf(a)).view(np.uint16).astype(np.uint32)
        return w[..., 0::2, :] | (w[..., 1::2, :] << 16)
    return (pk(fd), pk(fd.T), pk(fs[:, :, il]), pk(fs.transpose(0, 2, 1)[:, :, il]))


def _fft4(x, sgn):
    (ar, ai), (br, bi), (cr, ci), (dr, di) = x
    s0r, s0i, d0r, d0i = ar + cr, ai + ci, ar - cr, ai - ci
    s1r, s1i, d1r, d1i = br + dr, bi + di, br - dr, bi - di
    p = (d0r + d1i, d0i - d1r)
    q = (d0r - d1i, d0i + d1r)
    y1, y3 = (p, q) if sgn < 0 else (q, p)
    return [(s0r + s1r, s0i + s1i), y1, (s0r - s1r, s0i - s1i), y3]


def _twiddle(v, e, n, sgn):
    if e == 0:
        return v
    vr, vi = v
    if 4 * e == n:
        return (-vi, vr) if sgn > 0 else (vi, -vr)
    c, s = math.cos(2 * math.pi * e / n), sgn * math.sin(2 * math.pi * e / n)
    if (8 * e) % (2 * n) == n:
        if c * s > 0:
            return ((vr - vi) * c, (vr + vi) * c)
        return ((vr + vi) * c, (vi - vr) * c)
    return (vr * c - vi * s, vr * s + vi * c)


def _fft8(x, sgn):
    ev, od = _fft4(x[0::2], sgn), _fft4(x[1::2], sgn)
    y = [None] * 8
    for k in range(4):
        (er, ei) = ev[k]
        if k == 2:
            p, q = (er + od[k][1], ei - od[k][0]), (er - od[k][1], ei + od[k][0])
            y[k], y[k + 4] = (p, q) if sgn < 0 else (q, p)
        else:
            tr, ti = _twiddle(od[k], k, 8, sgn)
            y[k], y[k + 4] = (er + tr, ei + ti), (er - tr, ei - ti)
    return y


def _fft32(load, store, sgn):
    t = []
    for n2 in range(8):
        o = _fft4([load(n2 + 8 * n1) for n1 in range(4)], sgn)
        t.append([_twiddle(o[k1], n2 * k1, 32, sgn) for k1 in range(4)])
    for k1 in range(4):
        o = _fft8([t[n2][k1] for n2 in range(8)], sgn)
        for k2 in range(8):
            store(k1 + 4 * k2, o[k2])


_C1, _C2 = math.cos(2 * math.pi / 5), math.cos(4 * math.pi / 5)
_S1, _S2 = math.sin(2 * math.pi / 5), math.sin(4 * math.pi / 5)


def _rfft5(u):
    x = [u[:, a * 128:(a + 1) * 128] for a in range(5)]
    s1, s2, d1, d2 = x[1] + x[4], x[2] + x[3], x[4] - x[1], x[3] - x[2]
    return jnp.concatenate([
        x[0] + s1 + s2,
        x[0] + _C1 * s1 + _C2 * s2, _S1 * d1 + _S2 * d2,
        x[0] + _C2 * s1 + _C1 * s2, _S2 * d1 - _S1 * d2], axis=1)


def _irfft5(q):
    q0, q1r, q1i, q2r, q2i = [q[:, a * 128:(a + 1) * 128] for a in range(5)]
    e1, e2 = q0 + _C1 * q1r + _C2 * q2r, q0 + _C2 * q1r + _C1 * q2r
    o1, o2 = _S1 * q1i + _S2 * q2i, _S2 * q1i - _S1 * q2i
    return jnp.concatenate([q0 + q1r + q2r, e1 - o1, e2 - o2, e2 + o2, e1 + o1], axis=1)


def _layernorm(x):
    mu = jnp.mean(x, axis=1, keepdims=True)
    d = x - mu
    var = jnp.mean(d * d, axis=1, keepdims=True)
    return _rnd(d * jax.lax.rsqrt(var + 1e-5))


NCH = 5
WROWS = DM * H // NCH


NWO = 16
WOROWS = H * DH // NWO
NSEG = S // SEG
JT = (20, 10, 13)
BSCHED = (('d', 0), ('s', 9), ('i', 1), ('f', 0), ('r', -8))
LAG = (2, 3, 6)
PAIR = 2 * SEG
NPAIR = S // PAIR
_KR = ((0, 128), (128, 384), (384, 640))


def _pack(v):
    return pltpu.bitcast(v.astype(BF16), U32)


def _pack_complex(re, im):
    return pltpu.bitcast(pltpu.pack_elementwise([re, im], packed_dtype=BF16), U32)


def _unpack(v):
    return pltpu.bitcast(v, BF16)


def _rows(i, n):
    return pl.ds(i * n, n) if isinstance(i, int) else pl.ds(pl.multiple_of(i * n, n), n)


def _kernel(x_hbm, mem_hbm, wq_hbm, wk_hbm, wv_hbm, wo_hbm, wr_hbm, wi_hbm,
            fd_hbm, fdt_hbm, fs_hbm, fst_hbm,
            o_hbm,
            xio, memb, stage, t32, wqkv, wostage, wo, wb, wt, wp,
            fd, fdt, fs, fst,
            xs, us, u_buf, t_buf, z_buf, zero, sems):
    cnt = [0]

    def copy(src, dst):
        c = pltpu.make_async_copy(src, dst, sems.at[cnt[0]])
        cnt[0] += 1
        c.start()
        return c

    head, rest = pl.ds(0, 128), pl.ds(128, S - 128)
    c_head = [copy(x_hbm.at[head], xio.at[head]), copy(mem_hbm, memb), copy(fd_hbm, fd),
              copy(wr_hbm.at[:, head], wb.at[0, :, head]), copy(wi_hbm.at[:, head], wb.at[1, :, head])]
    w_sem = cnt[0]
    for i, w in enumerate((wq_hbm, wk_hbm, wv_hbm)):
        for c in range(NCH):
            copy(w.at[pl.ds(c * WROWS, WROWS)], stage.at[i * NCH + c])
    wo_sem = cnt[0]
    for c in range(NWO):
        copy(wo_hbm.at[_rows(c, WOROWS)], wostage.at[_rows(c, WOROWS)])
    c_rest = [copy(x_hbm.at[rest], xio.at[rest]),
              copy(wr_hbm.at[:, rest], wb.at[0, :, rest]), copy(wi_hbm.at[:, rest], wb.at[1, :, rest])]
    c_b = [copy(fs_hbm, fs), copy(fst_hbm, fst), copy(fdt_hbm, fdt)]

    def set_input(i, x):
        x = x.astype(F32)
        xs[_rows(i, PAIR), :] = x
        us[_rows(i, PAIR), :] = _layernorm(x)

    for c in c_head:
        c.wait()
    set_input(0, xio[:PAIR, :])

    for i in range(3):
        def w_chunk(c, _):
            n = i * NCH + c
            pltpu.make_async_copy(stage.at[n], stage.at[n], sems.at[w_sem + n]).wait()

            def widen(j, _):
                t32[_rows(j, 256), :] = pltpu.bitcast(stage[n, _rows(j, 512), :], U32)
            jax.lax.fori_loop(0, WROWS // 512, widen, None)

            def split(j, _):
                v = t32[pl.ds(j, 128, stride=H // 2), :]
                wqkv[2 * j, _rows(c, 64), i * 128:(i + 1) * 128] = _pack(pltpu.bitcast(v << 16, F32))
                wqkv[2 * j + 1, _rows(c, 64), i * 128:(i + 1) * 128] = _pack(
                    pltpu.bitcast(v & np.uint32(0xFFFF0000), F32))
            jax.lax.fori_loop(0, H // 2, split, None, unroll=2)
        jax.lax.fori_loop(0, NCH, w_chunk, None)

    def wo_chunk(c, _):
        blk = wostage.at[_rows(c, WOROWS)]
        pltpu.make_async_copy(blk, blk, sems.at[wo_sem + c]).wait()
        wo[_rows(c, WOROWS // 2), :] = pltpu.bitcast(wostage[_rows(c, WOROWS), :], U32)
    jax.lax.fori_loop(0, NWO, wo_chunk, None)

    def filter_prep(i):
        part, blk = i % 2, i // 2
        wt[:DF, :] = wb[part, :, _rows(blk, 128)].astype(F32)
        lane = jax.lax.broadcasted_iota(jnp.int32, (1, 128), 1)
        sub = jax.lax.broadcasted_iota(jnp.int32, (64, 128), 0)
        for r in range(3):
            lo = wt[pl.ds(r, 64, stride=5), :]
            if r == 0:
                hi = jnp.where(sub == 0, wt[DF - 1:DF, :], 0.0)
                c = jnp.where((lane == 0) | (lane == 64), 1.0 / (S * DM), 2.0 / (S * DM))
            else:
                hi = wt[pl.ds(5 - r, 64, stride=5), :]
                c = 2.0 / (S * DM)
            w = jnp.concatenate([lo, hi], axis=0).T * c
            for g in range(128 // RS):
                wp[part * 3 + r, pl.ds(blk * (128 // RS) + g, RS, stride=NB + 1), :] = w[g * RS:(g + 1) * RS]

    def fwd_vpu(i, n=PAIR):
        return _rfft5(_layernorm(xs[_rows(i, n), :]))

    def fwd_mxu(i, v, n=PAIR):
        for r, (k0, k1) in enumerate(_KR):
            u_buf[r, _rows(i, n), :] = _dot(v[:, k0:k1], _unpack(fd[k0 // 2:k1 // 2, :]))

    def inv_mxu(i, n=PAIR):
        return jnp.concatenate(
            [_dot(z_buf[r, _rows(i, n), :], _unpack(fdt[:, k0:k1])) for r, (k0, k1) in enumerate(_KR)],
            axis=1)

    def inv_vpu(i, q, n=PAIR):
        return (xs[_rows(i, n), :] + _rnd(_irfft5(q))).astype(BF16)

    row = jax.lax.broadcasted_iota(jnp.int32, (L, L), 0)
    col = jax.lax.broadcasted_iota(jnp.int32, (L, L), 1)
    mask = (row >= SEG) | (col >= SEG) | (row >= col)
    scale = DH ** -0.5
    G = 4

    def a_step(s, mem, jobs):
        hh = jnp.concatenate([us[_rows(s, SEG), :], mem], axis=0)
        qkv, sc, pp, oo = {}, {}, {}, {}
        acc = None
        for t in range(H + H // G):
            if t < H:
                qkv[t] = _dot(hh, _unpack(wqkv[t]))
            else:
                g = t - H
                o = jnp.concatenate([oo[g * G + i] for i in range(G)], axis=1)
                o = jnp.concatenate([o[SEG:], o[:SEG]], axis=0)
                r = _dot(o, _unpack(wo[g * G * 64:(g + 1) * G * 64, :]))
                acc = r if acc is None else acc + r
            h = t - LAG[0]
            if 0 <= h < H:
                sc[h] = _dot(qkv[h][:, :128], qkv[h][:, 128:256].astype(BF16), _NT)
            h = t - LAG[1]
            if 0 <= h < H:
                z = jnp.where(mask, sc[h] * scale, -1e9)
                e = jnp.exp(z - jnp.max(z, axis=1, keepdims=True))
                pp[h] = e * (1.0 / jnp.sum(e, axis=1, keepdims=True))
            h = t - LAG[2]
            if 0 <= h < H:
                oo[h] = _dot(pp[h], qkv[h][:, 256:].astype(BF16))
            if t in jobs:
                jobs[t]()
        xs[_rows(s, SEG), :] = _rnd(xs[_rows(s, SEG), :] + _rnd(acc[M:]))
        return acc[:M]

    def radix_fwd(r, j):
        def store(k, v):
            t_buf[r, k, _rows(j, 8), :] = _pack_complex(*v)
        _fft32(lambda a: (u_buf[r, _rows(a * 8 + j, 8), :128], u_buf[r, _rows(a * 8 + j, 8), 128:]), store, -1)

    def radix_inv(r, j):
        def store(a, v):
            z_buf[r, _rows(a * 8 + j, 8), :128] = v[0]
            z_buf[r, _rows(a * 8 + j, 8), 128:] = v[1]
        _fft32(lambda k: (z_buf[r, _rows(k * 8 + j, 8), :128], z_buf[r, _rows(k * 8 + j, 8), 128:]), store, +1)

    def dft_fwd(r, k):
        return _dot(_unpack(fs[k]), _unpack(t_buf[r, k]))

    def filt(r, k, x):
        xr, xi = x[:NB], x[NB:]
        wr, wi = wp[r, pl.ds(k * (NB + 1), NB), :], wp[3 + r, pl.ds(k * (NB + 1), NB), :]
        return _unpack(_pack_complex(xr * wr - xi * wi, xr * wi + xi * wr))

    def dft_inv(r, k, y):
        z = _dot(_unpack(fst[k]), y)
        z_buf[r, _rows(k, NB), :128] = z[:NB]
        z_buf[r, _rows(k, NB), 128:] = z[NB:]

    def b_mid():
        z0, z1, z2, z3 = zero[0], zero[1], zero[2], zero[3]
        ys = {}
        def f_dft(r, j):
            for k in range(4 * j, 4 * j + 4):
                ys[r, k] = dft_fwd(r + z0, k)

        def f_filt(r, j):
            for k in range(4 * j, 4 * j + 4):
                ys[r, k] = filt(r, k, ys[r, k])

        def f_idft(r, j):
            for k in range(4 * j, 4 * j + 4):
                dft_inv(r + z2, k, ys.pop((r, k)))
        stages = dict(d=f_dft, f=f_filt, i=f_idft,
                      r=lambda r, j: radix_fwd(r + z3, j), s=lambda r, j: radix_inv(r + z1, j))
        for t in range(-12, 40):
            for name, lag in BSCHED:
                if 0 <= t - lag < 24:
                    stages[name](*divmod(t - lag, 8))

    for i in range(4):
        zero[i] = 0
    mem0 = memb[...].astype(F32)

    def a_steps(i, mem, after_b):
        if not after_b:
            @pl.when(i == 1)
            def _():
                for c in c_rest:
                    c.wait()
        prv, nxt = jnp.maximum(i - 1, 0), jnp.minimum(i + 1, NPAIR - 1)
        st = {}
        first = {JT[0]: lambda: st.update(v=fwd_vpu(prv)), H + H // G - 1: lambda: fwd_mxu(prv, st["v"])}
        if after_b:
            second = {JT[1]: lambda: st.update(q=inv_mxu(nxt)), JT[2]: lambda: set_input(i + 1, inv_vpu(nxt, st["q"]))}
        else:
            second = {JT[1]: lambda: set_input(i + 1, xio[_rows(nxt, PAIR), :]), 12: lambda: filter_prep(i)}
        return a_step(2 * i + 1, a_step(2 * i, mem, first), second)
    a_first = functools.partial(a_steps, after_b=False)
    a_second = functools.partial(a_steps, after_b=True)
    jax.lax.fori_loop(0, NPAIR, a_first, mem0)
    for c in c_b:
        c.wait()

    def layer(l, _):
        fwd_mxu(NPAIR - 1, fwd_vpu(NPAIR - 1))
        b_mid()

        @pl.when(l == 0)
        def _():
            set_input(0, inv_vpu(0, inv_mxu(0)))
            jax.lax.fori_loop(0, NPAIR, a_second, mem0)
    jax.lax.fori_loop(0, 2, layer, None)

    c_out = []
    for i in range(S // 256):
        xio[_rows(i, 256), :] = inv_vpu(i, inv_mxu(i, 256), 256)
        c_out.append(copy(xio.at[_rows(i, 256)], o_hbm.at[_rows(i, 256)]))
    for c in c_out:
        c.wait()


@functools.partial(jax.jit, static_argnames=("A_seg_len",))
def pallas_interleave_layers__memory_aug_recurrent_mem_tr__spectral_gfnet__prompt_kernel(
    A_x, A_mem0, A_Wq, A_Wk, A_Wv, A_Wo, A_seg_len, B_x, B_w_r, B_w_i,
):
    del B_x
    assert A_x.shape == (1, S, DM) and A_Wq.shape == (DM, H, DH) and int(A_seg_len) == SEG
    consts = _constants()
    vm = pltpu.VMEM
    out = pl.pallas_call(
        _kernel,
        out_shape=jax.ShapeDtypeStruct((S, DM), BF16),
        in_specs=[pl.BlockSpec(memory_space=pltpu.HBM)] * 12,
        out_specs=pl.BlockSpec(memory_space=pltpu.HBM),
        scratch_shapes=[
            vm((S, DM), BF16),
            vm((M, DM), BF16),
            vm((3 * NCH, WROWS, DH), BF16),
            vm((WROWS // 2, DH), U32),
            vm((H, DM // 2, 3 * DH), U32),
            vm((H * DH, DM), BF16),
            vm((H * DH // 2, DM), U32),
            vm((2, DF, S), BF16),
            vm((328, 128), F32),
            vm((6, S + RS, 128), F32),
            vm((DM // 2, 256), U32), vm((128, DM), U32),
            vm((RS, NB, 128), U32), vm((RS, NB, 128), U32),
            vm((S + PAIR, DM), F32), vm((S + PAIR, DM), F32),
            vm((3, S, 256), F32),
            vm((3, RS, NB, 128), U32),
            vm((3, S, 256), F32),
            pltpu.SMEM((4,), jnp.int32),
            pltpu.SemaphoreType.DMA((19 + 3 * NCH + NWO,)),
        ],
        compiler_params=pltpu.CompilerParams(vmem_limit_bytes=110 * 2**20),
        name="rmt_gfnet",
    )(A_x.reshape(S, DM), A_mem0.reshape(M, DM),
      A_Wq.reshape(DM * H, DH), A_Wk.reshape(DM * H, DH), A_Wv.reshape(DM * H, DH),
      A_Wo.reshape(H * DH, DM), B_w_r.T, B_w_i.T, *consts)
    return out.reshape(1, S, DM)
```

```python
import functools
import math

import jax
import jax.numpy as jnp
import numpy as np
import jax.experimental.pallas as pl
import jax.experimental.pallas.tpu as pltpu

S, DM, H, DH, M, SEG = 2048, 640, 32, 128, 8, 32
L = M + SEG
DF = DM // 2 + 1
RS = 32
NB = S // RS
F32, BF16, U32 = jnp.float32, jnp.bfloat16, jnp.uint32
_NN = (((1,), (0,)), ((), ()))
_NT = (((1,), (1,)), ((), ()))


def _dot(a, b, dims=_NN):
    return jax.lax.dot_general(a, b, dims, preferred_element_type=F32)


def _rnd(v):
    return v.astype(BF16).astype(F32)


def _constants():
    b = np.arange(128)[:, None].astype(np.float64)
    j = np.arange(128)
    fd = np.zeros((5 * 128, 256))
    th = 2 * np.pi * b * (5 * j[None, :65]) / DM
    fd[:128, :65] = np.cos(th)
    fd[:128, 128:128 + 65] = -np.sin(th)
    fd[:128, 128] = 0.0
    fd[:128, 128 + 64] = 0.0
    for r in (1, 2):
        fp = np.where(j < 64, r + 5 * j, (5 - r) + 5 * (j - 64))
        f = np.where(j < 64, fp, DM - fp)
        sg = np.where(j < 64, 1.0, -1.0)[None, :]
        th = 2 * np.pi * b * f[None, :] / DM
        o = 128 + (r - 1) * 256
        fd[o:o + 128, :128] = np.cos(th)
        fd[o:o + 128, 128:] = -sg * np.sin(th)
        fd[o + 128:o + 256, :128] = np.sin(th)
        fd[o + 128:o + 256, 128:] = sg * np.cos(th)
    fs = np.zeros((RS, 2 * NB, 2 * NB))
    g = np.arange(NB)[:, None].astype(np.float64)
    bb = np.arange(NB)[None, :].astype(np.float64)
    for r in range(RS):
        th = 2 * np.pi * ((r + RS * g) * bb % S) / S
        c, s = np.cos(th), np.sin(th)
        fs[r] = np.block([[c, s], [-s, c]])
    bf = lambda a: np.asarray(a, dtype=BF16)

    il = np.arange(2 * NB) // 2 + NB * (np.arange(2 * NB) % 2)

    def pk(a):
        w = np.ascontiguousarray(bf(a)).view(np.uint16).astype(np.uint32)
        return w[..., 0::2, :] | (w[..., 1::2, :] << 16)
    return (pk(fd), pk(fd.T), pk(fs[:, :, il]), pk(fs.transpose(0, 2, 1)[:, :, il]))


def _fft4(x, sgn):
    (ar, ai), (br, bi), (cr, ci), (dr, di) = x
    s0r, s0i, d0r, d0i = ar + cr, ai + ci, ar - cr, ai - ci
    s1r, s1i, d1r, d1i = br + dr, bi + di, br - dr, bi - di
    p = (d0r + d1i, d0i - d1r)
    q = (d0r - d1i, d0i + d1r)
    y1, y3 = (p, q) if sgn < 0 else (q, p)
    return [(s0r + s1r, s0i + s1i), y1, (s0r - s1r, s0i - s1i), y3]


def _twiddle(v, e, n, sgn):
    if e == 0:
        return v
    vr, vi = v
    if 4 * e == n:
        return (-vi, vr) if sgn > 0 else (vi, -vr)
    c, s = math.cos(2 * math.pi * e / n), sgn * math.sin(2 * math.pi * e / n)
    if (8 * e) % (2 * n) == n:
        if c * s > 0:
            return ((vr - vi) * c, (vr + vi) * c)
        return ((vr + vi) * c, (vi - vr) * c)
    return (vr * c - vi * s, vr * s + vi * c)


def _fft8(x, sgn):
    ev, od = _fft4(x[0::2], sgn), _fft4(x[1::2], sgn)
    y = [None] * 8
    for k in range(4):
        (er, ei) = ev[k]
        if k == 2:
            p, q = (er + od[k][1], ei - od[k][0]), (er - od[k][1], ei + od[k][0])
            y[k], y[k + 4] = (p, q) if sgn < 0 else (q, p)
        else:
            tr, ti = _twiddle(od[k], k, 8, sgn)
            y[k], y[k + 4] = (er + tr, ei + ti), (er - tr, ei - ti)
    return y


def _fft32(load, store, sgn):
    t = []
    for n2 in range(8):
        o = _fft4([load(n2 + 8 * n1) for n1 in range(4)], sgn)
        t.append([_twiddle(o[k1], n2 * k1, 32, sgn) for k1 in range(4)])
    for k1 in range(4):
        o = _fft8([t[n2][k1] for n2 in range(8)], sgn)
        for k2 in range(8):
            store(k1 + 4 * k2, o[k2])


_C1, _C2 = math.cos(2 * math.pi / 5), math.cos(4 * math.pi / 5)
_S1, _S2 = math.sin(2 * math.pi / 5), math.sin(4 * math.pi / 5)


def _rfft5(u):
    x = [u[:, a * 128:(a + 1) * 128] for a in range(5)]
    s1, s2, d1, d2 = x[1] + x[4], x[2] + x[3], x[4] - x[1], x[3] - x[2]
    return jnp.concatenate([
        x[0] + s1 + s2,
        x[0] + _C1 * s1 + _C2 * s2, _S1 * d1 + _S2 * d2,
        x[0] + _C2 * s1 + _C1 * s2, _S2 * d1 - _S1 * d2], axis=1)


def _irfft5(q):
    q0, q1r, q1i, q2r, q2i = [q[:, a * 128:(a + 1) * 128] for a in range(5)]
    e1, e2 = q0 + _C1 * q1r + _C2 * q2r, q0 + _C2 * q1r + _C1 * q2r
    o1, o2 = _S1 * q1i + _S2 * q2i, _S2 * q1i - _S1 * q2i
    return jnp.concatenate([q0 + q1r + q2r, e1 - o1, e2 - o2, e2 + o2, e1 + o1], axis=1)


def _layernorm(x):
    mu = jnp.mean(x, axis=1, keepdims=True)
    d = x - mu
    var = jnp.mean(d * d, axis=1, keepdims=True)
    return _rnd(d * jax.lax.rsqrt(var + 1e-5))


NCH = 5
WROWS = DM * H // NCH


NWO = 16
WOROWS = H * DH // NWO
NSEG = S // SEG
JT = (20, 10, 13)
BSCHED = (('d', 0), ('s', 9), ('i', 1), ('f', 0), ('r', -8))
LAG = (2, 3, 6)
PAIR = 2 * SEG
NPAIR = S // PAIR
_KR = ((0, 128), (128, 384), (384, 640))


def _pack(v):
    return pltpu.bitcast(v.astype(BF16), U32)


def _pack_complex(re, im):
    return pltpu.bitcast(pltpu.pack_elementwise([re, im], packed_dtype=BF16), U32)


def _unpack(v):
    return pltpu.bitcast(v, BF16)


def _rows(i, n):
    return pl.ds(i * n, n) if isinstance(i, int) else pl.ds(pl.multiple_of(i * n, n), n)


def _kernel(x_hbm, mem_hbm, wq_hbm, wk_hbm, wv_hbm, wo_hbm, wr_hbm, wi_hbm,
            fd_hbm, fdt_hbm, fs_hbm, fst_hbm,
            o_hbm,
            xio, memb, stage, t32, wqkv, wostage, wo, wb, wt, wp,
            fd, fdt, fs, fst,
            xs, us, u_buf, t_buf, z_buf, zero, sems):
    cnt = [0]

    def copy(src, dst):
        c = pltpu.make_async_copy(src, dst, sems.at[cnt[0]])
        cnt[0] += 1
        c.start()
        return c

    head, rest = pl.ds(0, 128), pl.ds(128, S - 128)
    c_head = [copy(x_hbm.at[head], xio.at[head]), copy(mem_hbm, memb), copy(fd_hbm, fd),
              copy(wr_hbm.at[:, head], wb.at[0, :, head]), copy(wi_hbm.at[:, head], wb.at[1, :, head])]
    w_sem = cnt[0]
    for i, w in enumerate((wq_hbm, wk_hbm, wv_hbm)):
        for c in range(NCH):
            copy(w.at[pl.ds(c * WROWS, WROWS)], stage.at[i * NCH + c])
    wo_sem = cnt[0]
    for c in range(NWO):
        copy(wo_hbm.at[_rows(c, WOROWS)], wostage.at[_rows(c, WOROWS)])
    c_rest = [copy(x_hbm.at[rest], xio.at[rest]),
              copy(wr_hbm.at[:, rest], wb.at[0, :, rest]), copy(wi_hbm.at[:, rest], wb.at[1, :, rest])]
    c_b = [copy(fs_hbm, fs), copy(fst_hbm, fst), copy(fdt_hbm, fdt)]

    def set_input(i, x):
        x = x.astype(F32)
        xs[_rows(i, PAIR), :] = x
        us[_rows(i, PAIR), :] = _layernorm(x)

    for c in c_head:
        c.wait()
    set_input(0, xio[:PAIR, :])

    for i in range(3):
        def w_chunk(c, _):
            n = i * NCH + c
            pltpu.make_async_copy(stage.at[n], stage.at[n], sems.at[w_sem + n]).wait()

            def widen(j, _):
                t32[_rows(j, 256), :] = pltpu.bitcast(stage[n, _rows(j, 512), :], U32)
            jax.lax.fori_loop(0, WROWS // 512, widen, None)

            def split(j, _):
                v = t32[pl.ds(j, 128, stride=H // 2), :]
                wqkv[2 * j, _rows(c, 64), i * 128:(i + 1) * 128] = _pack(pltpu.bitcast(v << 16, F32))
                wqkv[2 * j + 1, _rows(c, 64), i * 128:(i + 1) * 128] = _pack(
                    pltpu.bitcast(v & np.uint32(0xFFFF0000), F32))
            jax.lax.fori_loop(0, H // 2, split, None, unroll=2)
        jax.lax.fori_loop(0, NCH, w_chunk, None)

    def wo_chunk(c, _):
        blk = wostage.at[_rows(c, WOROWS)]
        pltpu.make_async_copy(blk, blk, sems.at[wo_sem + c]).wait()
        wo[_rows(c, WOROWS // 2), :] = pltpu.bitcast(wostage[_rows(c, WOROWS), :], U32)
    jax.lax.fori_loop(0, NWO, wo_chunk, None)

    def filter_prep(i):
        part, blk = i % 2, i // 2
        wt[:DF, :] = wb[part, :, _rows(blk, 128)].astype(F32)
        lane = jax.lax.broadcasted_iota(jnp.int32, (1, 128), 1)
        sub = jax.lax.broadcasted_iota(jnp.int32, (64, 128), 0)
        for r in range(3):
            lo = wt[pl.ds(r, 64, stride=5), :]
            if r == 0:
                hi = jnp.where(sub == 0, wt[DF - 1:DF, :], 0.0)
                c = jnp.where((lane == 0) | (lane == 64), 1.0 / (S * DM), 2.0 / (S * DM))
            else:
                hi = wt[pl.ds(5 - r, 64, stride=5), :]
                c = 2.0 / (S * DM)
            w = jnp.concatenate([lo, hi], axis=0).T * c
            for g in range(128 // RS):
                wp[part * 3 + r, pl.ds(blk * (128 // RS) + g, RS, stride=NB + 1), :] = w[g * RS:(g + 1) * RS]

    def fwd_vpu(i, n=PAIR):
        return _rfft5(_layernorm(xs[_rows(i, n), :]))

    def fwd_mxu(i, v, n=PAIR):
        for r, (k0, k1) in enumerate(_KR):
            u_buf[r, _rows(i, n), :] = _dot(v[:, k0:k1], _unpack(fd[k0 // 2:k1 // 2, :]))

    def inv_mxu(i, n=PAIR):
        return jnp.concatenate(
            [_dot(z_buf[r, _rows(i, n), :], _unpack(fdt[:, k0:k1])) for r, (k0, k1) in enumerate(_KR)],
            axis=1)

    def inv_vpu(i, q, n=PAIR):
        return (xs[_rows(i, n), :] + _rnd(_irfft5(q))).astype(BF16)

    row = jax.lax.broadcasted_iota(jnp.int32, (L, L), 0)
    col = jax.lax.broadcasted_iota(jnp.int32, (L, L), 1)
    mask = (row >= SEG) | (col >= SEG) | (row >= col)
    scale = DH ** -0.5
    G = 4

    def a_step(s, mem, jobs):
        hh = jnp.concatenate([us[_rows(s, SEG), :], mem], axis=0)
        qkv, sc, pp, oo = {}, {}, {}, {}
        acc = None
        for t in range(H + H // G):
            if t < H:
                qkv[t] = _dot(hh, _unpack(wqkv[t]))
            else:
                g = t - H
                o = jnp.concatenate([oo[g * G + i] for i in range(G)], axis=1)
                o = jnp.concatenate([o[SEG:], o[:SEG]], axis=0)
                r = _dot(o, _unpack(wo[g * G * 64:(g + 1) * G * 64, :]))
                acc = r if acc is None else acc + r
            h = t - LAG[0]
            if 0 <= h < H:
                sc[h] = _dot(qkv[h][:, :128], qkv[h][:, 128:256].astype(BF16), _NT)
            h = t - LAG[1]
            if 0 <= h < H:
                z = jnp.where(mask, sc[h] * scale, -1e9)
                e = jnp.exp(z - jnp.max(z, axis=1, keepdims=True))
                pp[h] = e * (1.0 / jnp.sum(e, axis=1, keepdims=True))
            h = t - LAG[2]
            if 0 <= h < H:
                oo[h] = _dot(pp[h], qkv[h][:, 256:].astype(BF16))
            if t in jobs:
                jobs[t]()
        xs[_rows(s, SEG), :] = _rnd(xs[_rows(s, SEG), :] + _rnd(acc[M:]))
        return acc[:M]

    def radix_fwd(r, j):
        def store(k, v):
            t_buf[r, k, _rows(j, 8), :] = _pack_complex(*v)
        _fft32(lambda a: (u_buf[r, _rows(a * 8 + j, 8), :128], u_buf[r, _rows(a * 8 + j, 8), 128:]), store, -1)

    def radix_inv(r, j):
        def store(a, v):
            z_buf[r, _rows(a * 8 + j, 8), :128] = v[0]
            z_buf[r, _rows(a * 8 + j, 8), 128:] = v[1]
        _fft32(lambda k: (z_buf[r, _rows(k * 8 + j, 8), :128], z_buf[r, _rows(k * 8 + j, 8), 128:]), store, +1)

    def dft_fwd(r, k):
        return _dot(_unpack(fs[k]), _unpack(t_buf[r, k]))

    def filt(r, k, x):
        xr, xi = x[:NB], x[NB:]
        wr, wi = wp[r, pl.ds(k * (NB + 1), NB), :], wp[3 + r, pl.ds(k * (NB + 1), NB), :]
        return _unpack(_pack_complex(xr * wr - xi * wi, xr * wi + xi * wr))

    def dft_inv(r, k, y):
        z = _dot(_unpack(fst[k]), y)
        z_buf[r, _rows(k, NB), :128] = z[:NB]
        z_buf[r, _rows(k, NB), 128:] = z[NB:]

    def b_mid():
        z0, z1 = zero[0], zero[1]
        ys = {}
        def f_dft(r, j):
            for k in range(4 * j, 4 * j + 4):
                ys[r, k] = dft_fwd(r + z0, k)

        def f_filt(r, j):
            for k in range(4 * j, 4 * j + 4):
                ys[r, k] = filt(r, k, ys[r, k])

        def f_idft(r, j):
            for k in range(4 * j, 4 * j + 4):
                dft_inv(r, k, ys.pop((r, k)))
        stages = dict(d=f_dft, f=f_filt, i=f_idft,
                      r=lambda r, j: radix_fwd(r + z1, j), s=radix_inv)
        for t in range(-12, 40):
            for name, lag in BSCHED:
                if 0 <= t - lag < 24:
                    stages[name](*divmod(t - lag, 8))

    for i in range(2):
        zero[i] = 0
    mem0 = memb[...].astype(F32)

    def a_steps(i, mem, after_b):
        if not after_b:
            @pl.when(i == 1)
            def _():
                for c in c_rest:
                    c.wait()
        prv, nxt = jnp.maximum(i - 1, 0), jnp.minimum(i + 1, NPAIR - 1)
        st = {}
        first = {JT[0]: lambda: st.update(v=fwd_vpu(prv)), H + H // G - 1: lambda: fwd_mxu(prv, st["v"])}
        if after_b:
            second = {JT[1]: lambda: st.update(q=inv_mxu(nxt)), JT[2]: lambda: set_input(i + 1, inv_vpu(nxt, st["q"]))}
        else:
            second = {JT[1]: lambda: set_input(i + 1, xio[_rows(nxt, PAIR), :]), 12: lambda: filter_prep(i)}
        return a_step(2 * i + 1, a_step(2 * i, mem, first), second)
    a_first = functools.partial(a_steps, after_b=False)
    a_second = functools.partial(a_steps, after_b=True)
    jax.lax.fori_loop(0, NPAIR, a_first, mem0)
    for c in c_b:
        c.wait()

    def layer(l, _):
        fwd_mxu(NPAIR - 1, fwd_vpu(NPAIR - 1))
        b_mid()

        @pl.when(l == 0)
        def _():
            set_input(0, inv_vpu(0, inv_mxu(0)))
            jax.lax.fori_loop(0, NPAIR, a_second, mem0)
    jax.lax.fori_loop(0, 2, layer, None)

    c_out = []
    for i in range(S // 256):
        xio[_rows(i, 256), :] = inv_vpu(i, inv_mxu(i, 256), 256)
        c_out.append(copy(xio.at[_rows(i, 256)], o_hbm.at[_rows(i, 256)]))
    for c in c_out:
        c.wait()


@functools.partial(jax.jit, static_argnames=("A_seg_len",))
def pallas_interleave_layers__memory_aug_recurrent_mem_tr__spectral_gfnet__prompt_kernel(
    A_x, A_mem0, A_Wq, A_Wk, A_Wv, A_Wo, A_seg_len, B_x, B_w_r, B_w_i,
):
    del B_x
    assert A_x.shape == (1, S, DM) and A_Wq.shape == (DM, H, DH) and int(A_seg_len) == SEG
    consts = _constants()
    vm = pltpu.VMEM
    out = pl.pallas_call(
        _kernel,
        out_shape=jax.ShapeDtypeStruct((S, DM), BF16),
        in_specs=[pl.BlockSpec(memory_space=pltpu.HBM)] * 12,
        out_specs=pl.BlockSpec(memory_space=pltpu.HBM),
        scratch_shapes=[
            vm((S, DM), BF16),
            vm((M, DM), BF16),
            vm((3 * NCH, WROWS, DH), BF16),
            vm((WROWS // 2 + H, DH), U32),
            vm((H, DM // 2, 3 * DH), U32),
            vm((H * DH, DM), BF16),
            vm((H * DH // 2, DM), U32),
            vm((2, DF, S), BF16),
            vm((328, 128), F32),
            vm((6, S + RS + NB, 128), F32),
            vm((DM // 2, 256), U32), vm((128, DM), U32),
            vm((RS, NB, 128), U32), vm((RS, NB, 128), U32),
            vm((S + PAIR, DM), F32), vm((S + PAIR, DM), F32),
            vm((3, S, 256), F32),
            vm((3, RS, NB, 128), U32),
            vm((3, S, 256), F32),
            pltpu.SMEM((2,), jnp.int32),
            pltpu.SemaphoreType.DMA((19 + 3 * NCH + NWO,)),
        ],
        compiler_params=pltpu.CompilerParams(vmem_limit_bytes=110 * 2**20),
        name="rmt_gfnet",
    )(A_x.reshape(S, DM), A_mem0.reshape(M, DM),
      A_Wq.reshape(DM * H, DH), A_Wk.reshape(DM * H, DH), A_Wv.reshape(DM * H, DH),
      A_Wo.reshape(H * DH, DM), B_w_r.T, B_w_i.T, *consts)
    return out.reshape(1, S, DM)
```

```python
import functools
import math

import jax
import jax.numpy as jnp
import numpy as np
import jax.experimental.pallas as pl
import jax.experimental.pallas.tpu as pltpu

S, DM, H, DH, M, SEG = 2048, 640, 32, 128, 8, 32
L = M + SEG
DF = DM // 2 + 1
RS = 32
NB = S // RS
F32, BF16, U32 = jnp.float32, jnp.bfloat16, jnp.uint32
_NN = (((1,), (0,)), ((), ()))
_NT = (((1,), (1,)), ((), ()))


def _dot(a, b, dims=_NN):
    return jax.lax.dot_general(a, b, dims, preferred_element_type=F32)


def _rnd(v):
    return v.astype(BF16).astype(F32)


def _constants():
    b = np.arange(128)[:, None].astype(np.float64)
    j = np.arange(128)
    fd = np.zeros((5 * 128, 256))
    th = 2 * np.pi * b * (5 * j[None, :65]) / DM
    fd[:128, :65] = np.cos(th)
    fd[:128, 128:128 + 65] = -np.sin(th)
    fd[:128, 128] = 0.0
    fd[:128, 128 + 64] = 0.0
    for r in (1, 2):
        fp = np.where(j < 64, r + 5 * j, (5 - r) + 5 * (j - 64))
        f = np.where(j < 64, fp, DM - fp)
        sg = np.where(j < 64, 1.0, -1.0)[None, :]
        th = 2 * np.pi * b * f[None, :] / DM
        o = 128 + (r - 1) * 256
        fd[o:o + 128, :128] = np.cos(th)
        fd[o:o + 128, 128:] = -sg * np.sin(th)
        fd[o + 128:o + 256, :128] = np.sin(th)
        fd[o + 128:o + 256, 128:] = sg * np.cos(th)
    fs = np.zeros((RS, 2 * NB, 2 * NB))
    g = np.arange(NB)[:, None].astype(np.float64)
    bb = np.arange(NB)[None, :].astype(np.float64)
    for r in range(RS):
        th = 2 * np.pi * ((r + RS * g) * bb % S) / S
        c, s = np.cos(th), np.sin(th)
        fs[r] = np.block([[c, s], [-s, c]])
    i = np.arange(2 * NB)
    il = i % 8 + 8 * (i // 16) + NB * (i // 8 % 2)
    fs = fs[:, il][:, :, il]
    bf = lambda a: np.asarray(a, dtype=BF16)


    def pk(a):
        w = np.ascontiguousarray(bf(a)).view(np.uint16).astype(np.uint32)
        return w[..., 0::2, :] | (w[..., 1::2, :] << 16)
    return (pk(fd), pk(fd.T), pk(fs), pk(fs.transpose(0, 2, 1)))


def _fft4(x, sgn):
    (ar, ai), (br, bi), (cr, ci), (dr, di) = x
    s0r, s0i, d0r, d0i = ar + cr, ai + ci, ar - cr, ai - ci
    s1r, s1i, d1r, d1i = br + dr, bi + di, br - dr, bi - di
    p = (d0r + d1i, d0i - d1r)
    q = (d0r - d1i, d0i + d1r)
    y1, y3 = (p, q) if sgn < 0 else (q, p)
    return [(s0r + s1r, s0i + s1i), y1, (s0r - s1r, s0i - s1i), y3]


def _twiddle(v, e, n, sgn):
    if e == 0:
        return v
    vr, vi = v
    if 4 * e == n:
        return (-vi, vr) if sgn > 0 else (vi, -vr)
    c, s = math.cos(2 * math.pi * e / n), sgn * math.sin(2 * math.pi * e / n)
    if (8 * e) % (2 * n) == n:
        if c * s > 0:
            return ((vr - vi) * c, (vr + vi) * c)
        return ((vr + vi) * c, (vi - vr) * c)
    return (vr * c - vi * s, vr * s + vi * c)


def _fft8(x, sgn):
    ev, od = _fft4(x[0::2], sgn), _fft4(x[1::2], sgn)
    y = [None] * 8
    for k in range(4):
        (er, ei) = ev[k]
        if k == 2:
            p, q = (er + od[k][1], ei - od[k][0]), (er - od[k][1], ei + od[k][0])
            y[k], y[k + 4] = (p, q) if sgn < 0 else (q, p)
        else:
            tr, ti = _twiddle(od[k], k, 8, sgn)
            y[k], y[k + 4] = (er + tr, ei + ti), (er - tr, ei - ti)
    return y


_C1, _C2 = math.cos(2 * math.pi / 5), math.cos(4 * math.pi / 5)
_S1, _S2 = math.sin(2 * math.pi / 5), math.sin(4 * math.pi / 5)


def _rfft5(u):
    x = [u[:, a * 128:(a + 1) * 128] for a in range(5)]
    s1, s2, d1, d2 = x[1] + x[4], x[2] + x[3], x[4] - x[1], x[3] - x[2]
    return jnp.concatenate([
        x[0] + s1 + s2,
        x[0] + _C1 * s1 + _C2 * s2, _S1 * d1 + _S2 * d2,
        x[0] + _C2 * s1 + _C1 * s2, _S2 * d1 - _S1 * d2], axis=1)


def _irfft5(q):
    q0, q1r, q1i, q2r, q2i = [q[:, a * 128:(a + 1) * 128] for a in range(5)]
    e1, e2 = q0 + _C1 * q1r + _C2 * q2r, q0 + _C2 * q1r + _C1 * q2r
    o1, o2 = _S1 * q1i + _S2 * q2i, _S2 * q1i - _S1 * q2i
    return jnp.concatenate([q0 + q1r + q2r, e1 - o1, e2 - o2, e2 + o2, e1 + o1], axis=1)


def _layernorm(x):
    mu = jnp.mean(x, axis=1, keepdims=True)
    d = x - mu
    var = jnp.mean(d * d, axis=1, keepdims=True)
    return _rnd(d * jax.lax.rsqrt(var + 1e-5))


NCH = 5
WROWS = DM * H // NCH


NWO = 16
WOROWS = H * DH // NWO
NSEG = S // SEG
JT = (20, 10, 13)
BSCHED = (('d', 0), ('s', 9), ('i', 1), ('f', 0), ('r', -8))
LAG = (2, 3, 6)
PAIR = 2 * SEG
NPAIR = S // PAIR
_KR = ((0, 128), (128, 384), (384, 640))


def _pack(v):
    return pltpu.bitcast(v.astype(BF16), U32)


def _unpack(v):
    return pltpu.bitcast(v, BF16)


def _rows(i, n):
    return pl.ds(i * n, n) if isinstance(i, int) else pl.ds(pl.multiple_of(i * n, n), n)


def _kernel(x_hbm, mem_hbm, wq_hbm, wk_hbm, wv_hbm, wo_hbm, wr_hbm, wi_hbm,
            fd_hbm, fdt_hbm, fs_hbm, fst_hbm,
            o_hbm,
            xio, memb, stage, t32, wqkv, wostage, wo, wb, wt, wp,
            fd, fdt, fs, fst,
            xs, us, u_buf, z_buf, zero, sems):
    cnt = [0]

    def copy(src, dst):
        c = pltpu.make_async_copy(src, dst, sems.at[cnt[0]])
        cnt[0] += 1
        c.start()
        return c

    head, rest = pl.ds(0, 128), pl.ds(128, S - 128)
    c_head = [copy(x_hbm.at[head], xio.at[head]), copy(mem_hbm, memb), copy(fd_hbm, fd),
              copy(wr_hbm.at[:, head], wb.at[0, :, head]), copy(wi_hbm.at[:, head], wb.at[1, :, head])]
    w_sem = cnt[0]
    for i, w in enumerate((wq_hbm, wk_hbm, wv_hbm)):
        for c in range(NCH):
            copy(w.at[pl.ds(c * WROWS, WROWS)], stage.at[i * NCH + c])
    wo_sem = cnt[0]
    for c in range(NWO):
        copy(wo_hbm.at[_rows(c, WOROWS)], wostage.at[_rows(c, WOROWS)])
    c_rest = [copy(x_hbm.at[rest], xio.at[rest]),
              copy(wr_hbm.at[:, rest], wb.at[0, :, rest]), copy(wi_hbm.at[:, rest], wb.at[1, :, rest])]
    c_b = [copy(fs_hbm, fs), copy(fst_hbm, fst), copy(fdt_hbm, fdt)]

    def set_input(i, x):
        x = x.astype(F32)
        xs[_rows(i, PAIR), :] = x
        us[_rows(i, PAIR), :] = _layernorm(x)

    for c in c_head:
        c.wait()
    set_input(0, xio[:PAIR, :])

    for i in range(3):
        def w_chunk(c, _):
            n = i * NCH + c
            pltpu.make_async_copy(stage.at[n], stage.at[n], sems.at[w_sem + n]).wait()

            def widen(j, _):
                t32[_rows(j, 256), :] = pltpu.bitcast(stage[n, _rows(j, 512), :], U32)
            jax.lax.fori_loop(0, WROWS // 512, widen, None)

            def split(j, _):
                v = t32[pl.ds(j, 128, stride=H // 2), :]
                wqkv[2 * j, _rows(c, 64), i * 128:(i + 1) * 128] = _pack(pltpu.bitcast(v << 16, F32))
                wqkv[2 * j + 1, _rows(c, 64), i * 128:(i + 1) * 128] = _pack(
                    pltpu.bitcast(v & np.uint32(0xFFFF0000), F32))
            jax.lax.fori_loop(0, H // 2, split, None, unroll=2)
        jax.lax.fori_loop(0, NCH, w_chunk, None)

    def wo_chunk(c, _):
        blk = wostage.at[_rows(c, WOROWS)]
        pltpu.make_async_copy(blk, blk, sems.at[wo_sem + c]).wait()
        wo[_rows(c, WOROWS // 2), :] = pltpu.bitcast(wostage[_rows(c, WOROWS), :], U32)
    jax.lax.fori_loop(0, NWO, wo_chunk, None)

    def filter_prep(i):
        part, blk = i % 2, i // 2
        wt[:DF, :] = wb[part, :, _rows(blk, 128)].astype(F32)
        lane = jax.lax.broadcasted_iota(jnp.int32, (1, 128), 1)
        sub = jax.lax.broadcasted_iota(jnp.int32, (64, 128), 0)
        for r in range(3):
            lo = wt[pl.ds(r, 64, stride=5), :]
            if r == 0:
                hi = jnp.where(sub == 0, wt[DF - 1:DF, :], 0.0)
                c = jnp.where((lane == 0) | (lane == 64), 1.0 / (S * DM), 2.0 / (S * DM))
            else:
                hi = wt[pl.ds(5 - r, 64, stride=5), :]
                c = 2.0 / (S * DM)
            w = jnp.concatenate([lo, hi], axis=0).T * c
            for g in range(128 // RS):
                wp[part * 3 + r, pl.ds(blk * (128 // RS) + g, RS, stride=NB + 1), :] = w[g * RS:(g + 1) * RS]

    def fwd_vpu(i, n=PAIR):
        return _rfft5(_layernorm(xs[_rows(i, n), :]))

    def fwd_mxu(i, v, n=PAIR):
        for r, (k0, k1) in enumerate(_KR):
            u_buf[r, _rows(i, n), :] = _dot(v[:, k0:k1], _unpack(fd[k0 // 2:k1 // 2, :]))

    def inv_mxu(i, n=PAIR):
        return jnp.concatenate(
            [_dot(z_buf[r, _rows(i, n), :], _unpack(fdt[:, k0:k1])) for r, (k0, k1) in enumerate(_KR)],
            axis=1)

    def inv_vpu(i, q, n=PAIR):
        return (xs[_rows(i, n), :] + _rnd(_irfft5(q))).astype(BF16)

    row = jax.lax.broadcasted_iota(jnp.int32, (L, L), 0)
    col = jax.lax.broadcasted_iota(jnp.int32, (L, L), 1)
    mask = (row >= SEG) | (col >= SEG) | (row >= col)
    scale = DH ** -0.5
    G = 4

    def a_step(s, mem, jobs):
        hh = jnp.concatenate([us[_rows(s, SEG), :], mem], axis=0)
        qkv, sc, pp, oo = {}, {}, {}, {}
        acc = None
        for t in range(H + H // G):
            if t < H:
                qkv[t] = _dot(hh, _unpack(wqkv[t]))
            else:
                g = t - H
                o = jnp.concatenate([oo[g * G + i] for i in range(G)], axis=1)
                o = jnp.concatenate([o[SEG:], o[:SEG]], axis=0)
                r = _dot(o, _unpack(wo[g * G * 64:(g + 1) * G * 64, :]))
                acc = r if acc is None else acc + r
            h = t - LAG[0]
            if 0 <= h < H:
                sc[h] = _dot(qkv[h][:, :128], qkv[h][:, 128:256].astype(BF16), _NT)
            h = t - LAG[1]
            if 0 <= h < H:
                z = jnp.where(mask, sc[h] * scale, -1e9)
                e = jnp.exp(z - jnp.max(z, axis=1, keepdims=True))
                pp[h] = e * (1.0 / jnp.sum(e, axis=1, keepdims=True))
            h = t - LAG[2]
            if 0 <= h < H:
                oo[h] = _dot(pp[h], qkv[h][:, 256:].astype(BF16))
            if t in jobs:
                jobs[t]()
        xs[_rows(s, SEG), :] = _rnd(xs[_rows(s, SEG), :] + _rnd(acc[M:]))
        return acc[:M]

    def radix8(buf, sgn, r, j):
        for n1 in range(4):
            rows = [_rows((n1 + 4 * m) * 8 + j, 8) for m in range(8)]
            y = _fft8([(buf[r, q, :128], buf[r, q, 128:]) for q in rows], sgn)
            for q, (re, im) in zip(rows, y):
                buf[r, q, :128] = re
                buf[r, q, 128:] = im

    def parts(x, j):
        return x[16 * j:16 * j + 8], x[16 * j + 8:16 * j + 16]

    def dft_fwd(r, k2):
        t = []
        for j in range(8):
            rows = [_rows((n1 + 4 * k2) * 8 + j, 8) for n1 in range(4)]
            t.append(_fft4([_twiddle((u_buf[r, q, :128], u_buf[r, q, 128:]), n1 * k2, RS, -1)
                            for n1, q in enumerate(rows)], -1))
        return [_dot(_unpack(fs[k2 + 8 * k1]), jnp.concatenate([v for j in range(8) for v in t[j][k1]], axis=0).astype(BF16))
                for k1 in range(4)]

    def filt(r, k2, xf):
        out = []
        for k1, x in enumerate(xf):
            y = []
            for j in range(8):
                q = pl.ds((k2 + 8 * k1) * (NB + 1) + 8 * j, 8)
                (xr, xi), wr, wi = parts(x, j), wp[r, q, :], wp[3 + r, q, :]
                y += [xr * wr - xi * wi, xr * wi + xi * wr]
            out.append(jnp.concatenate(y, axis=0).astype(BF16))
        return out

    def dft_inv(r, k2, ys):
        z = [_dot(_unpack(fst[k2 + 8 * k1]), y) for k1, y in enumerate(ys)]
        for j in range(8):
            for n1, v in enumerate(_fft4([parts(x, j) for x in z], +1)):
                q = _rows((n1 + 4 * k2) * 8 + j, 8)
                z_buf[r, q, :128], z_buf[r, q, 128:] = _twiddle(v, n1 * k2, RS, +1)

    def b_mid():
        z0, z1 = zero[0], zero[1]
        st = {}
        stages = dict(d=lambda r, j: st.update({(r, j): dft_fwd(r + z0, j)}),
                      f=lambda r, j: st.update({(r, j): filt(r, j, st[r, j])}),
                      i=lambda r, j: dft_inv(r, j, st.pop((r, j))),
                      r=lambda r, j: radix8(u_buf, -1, r + z1, j),
                      s=lambda r, j: radix8(z_buf, +1, r, j))
        for t in range(-12, 40):
            for name, lag in BSCHED:
                if 0 <= t - lag < 24:
                    stages[name](*divmod(t - lag, 8))

    for i in range(2):
        zero[i] = 0
    mem0 = memb[...].astype(F32)

    def a_steps(i, mem, after_b):
        if not after_b:
            @pl.when(i == 1)
            def _():
                for c in c_rest:
                    c.wait()
        prv, nxt = jnp.maximum(i - 1, 0), jnp.minimum(i + 1, NPAIR - 1)
        st = {}
        first = {JT[0]: lambda: st.update(v=fwd_vpu(prv)), H + H // G - 1: lambda: fwd_mxu(prv, st["v"])}
        if after_b:
            second = {JT[1]: lambda: st.update(q=inv_mxu(nxt)), JT[2]: lambda: set_input(i + 1, inv_vpu(nxt, st["q"]))}
        else:
            second = {JT[1]: lambda: set_input(i + 1, xio[_rows(nxt, PAIR), :]), 12: lambda: filter_prep(i)}
        return a_step(2 * i + 1, a_step(2 * i, mem, first), second)
    a_first = functools.partial(a_steps, after_b=False)
    a_second = functools.partial(a_steps, after_b=True)
    jax.lax.fori_loop(0, NPAIR, a_first, mem0)
    for c in c_b:
        c.wait()

    def layer(l, _):
        fwd_mxu(NPAIR - 1, fwd_vpu(NPAIR - 1))
        b_mid()

        @pl.when(l == 0)
        def _():
            set_input(0, inv_vpu(0, inv_mxu(0)))
            jax.lax.fori_loop(0, NPAIR, a_second, mem0)
    jax.lax.fori_loop(0, 2, layer, None)

    c_out = []
    for i in range(S // 256):
        xio[_rows(i, 256), :] = inv_vpu(i, inv_mxu(i, 256), 256)
        c_out.append(copy(xio.at[_rows(i, 256)], o_hbm.at[_rows(i, 256)]))
    for c in c_out:
        c.wait()


@functools.partial(jax.jit, static_argnames=("A_seg_len",))
def pallas_interleave_layers__memory_aug_recurrent_mem_tr__spectral_gfnet__prompt_kernel(
    A_x, A_mem0, A_Wq, A_Wk, A_Wv, A_Wo, A_seg_len, B_x, B_w_r, B_w_i,
):
    del B_x
    assert A_x.shape == (1, S, DM) and A_Wq.shape == (DM, H, DH) and int(A_seg_len) == SEG
    consts = _constants()
    vm = pltpu.VMEM
    out = pl.pallas_call(
        _kernel,
        out_shape=jax.ShapeDtypeStruct((S, DM), BF16),
        in_specs=[pl.BlockSpec(memory_space=pltpu.HBM)] * 12,
        out_specs=pl.BlockSpec(memory_space=pltpu.HBM),
        scratch_shapes=[
            vm((S, DM), BF16),
            vm((M, DM), BF16),
            vm((3 * NCH, WROWS, DH), BF16),
            vm((WROWS // 2 + H, DH), U32),
            vm((H, DM // 2, 3 * DH), U32),
            vm((H * DH, DM), BF16),
            vm((H * DH // 2, DM), U32),
            vm((2, DF, S), BF16),
            vm((328, 128), F32),
            vm((6, S + RS + NB, 128), F32),
            vm((DM // 2, 256), U32), vm((128, DM), U32),
            vm((RS, NB, 128), U32), vm((RS, NB, 128), U32),
            vm((S + PAIR, DM), F32), vm((S + PAIR, DM), F32),
            vm((3, S, 256), F32),
            vm((3, S, 256), F32),
            pltpu.SMEM((2,), jnp.int32),
            pltpu.SemaphoreType.DMA((19 + 3 * NCH + NWO,)),
        ],
        compiler_params=pltpu.CompilerParams(vmem_limit_bytes=110 * 2**20),
        name="rmt_gfnet",
    )(A_x.reshape(S, DM), A_mem0.reshape(M, DM),
      A_Wq.reshape(DM * H, DH), A_Wk.reshape(DM * H, DH), A_Wv.reshape(DM * H, DH),
      A_Wo.reshape(H * DH, DM), B_w_r.T, B_w_i.T, *consts)
    return out.reshape(1, S, DM)
```

```python
import functools
import math

import jax
import jax.numpy as jnp
import numpy as np
import jax.experimental.pallas as pl
import jax.experimental.pallas.tpu as pltpu

S, DM, H, DH, M, SEG = 2048, 640, 32, 128, 8, 32
L = M + SEG
DF = DM // 2 + 1
RS = 32
NB = S // RS
F32, BF16, U32 = jnp.float32, jnp.bfloat16, jnp.uint32
_NN = (((1,), (0,)), ((), ()))
_NT = (((1,), (1,)), ((), ()))


def _dot(a, b, dims=_NN):
    return jax.lax.dot_general(a, b, dims, preferred_element_type=F32)


def _rnd(v):
    return v.astype(BF16).astype(F32)


def _constants():
    b = np.arange(128)[:, None].astype(np.float64)
    j = np.arange(128)
    fd = np.zeros((5 * 128, 256))
    th = 2 * np.pi * b * (5 * j[None, :65]) / DM
    fd[:128, :65] = np.cos(th)
    fd[:128, 128:128 + 65] = -np.sin(th)
    fd[:128, 128] = 0.0
    fd[:128, 128 + 64] = 0.0
    for r in (1, 2):
        fp = np.where(j < 64, r + 5 * j, (5 - r) + 5 * (j - 64))
        f = np.where(j < 64, fp, DM - fp)
        sg = np.where(j < 64, 1.0, -1.0)[None, :]
        th = 2 * np.pi * b * f[None, :] / DM
        o = 128 + (r - 1) * 256
        fd[o:o + 128, :128] = np.cos(th)
        fd[o:o + 128, 128:] = -sg * np.sin(th)
        fd[o + 128:o + 256, :128] = np.sin(th)
        fd[o + 128:o + 256, 128:] = sg * np.cos(th)
    fs = np.zeros((RS, 2 * NB, 2 * NB))
    g = np.arange(NB)[:, None].astype(np.float64)
    bb = np.arange(NB)[None, :].astype(np.float64)
    for r in range(RS):
        th = 2 * np.pi * ((r + RS * g) * bb % S) / S
        c, s = np.cos(th), np.sin(th)
        fs[r] = np.block([[c, s], [-s, c]])
    i = np.arange(2 * NB)
    il = i % 8 + 8 * (i // 16) + NB * (i // 8 % 2)
    fs = fs[:, il][:, :, il]
    bf = lambda a: np.asarray(a, dtype=BF16)


    def pk(a):
        w = np.ascontiguousarray(bf(a)).view(np.uint16).astype(np.uint32)
        return w[..., 0::2, :] | (w[..., 1::2, :] << 16)
    return (pk(fd), pk(fd.T), pk(fs), pk(fs.transpose(0, 2, 1)))


def _fft4(x, sgn):
    (ar, ai), (br, bi), (cr, ci), (dr, di) = x
    s0r, s0i, d0r, d0i = ar + cr, ai + ci, ar - cr, ai - ci
    s1r, s1i, d1r, d1i = br + dr, bi + di, br - dr, bi - di
    p = (d0r + d1i, d0i - d1r)
    q = (d0r - d1i, d0i + d1r)
    y1, y3 = (p, q) if sgn < 0 else (q, p)
    return [(s0r + s1r, s0i + s1i), y1, (s0r - s1r, s0i - s1i), y3]


def _twiddle(v, e, n, sgn):
    if e == 0:
        return v
    vr, vi = v
    if 4 * e == n:
        return (-vi, vr) if sgn > 0 else (vi, -vr)
    c, s = math.cos(2 * math.pi * e / n), sgn * math.sin(2 * math.pi * e / n)
    if (8 * e) % (2 * n) == n:
        if c * s > 0:
            return ((vr - vi) * c, (vr + vi) * c)
        return ((vr + vi) * c, (vi - vr) * c)
    return (vr * c - vi * s, vr * s + vi * c)


def _fft8(x, sgn):
    ev, od = _fft4(x[0::2], sgn), _fft4(x[1::2], sgn)
    y = [None] * 8
    for k in range(4):
        (er, ei) = ev[k]
        if k == 2:
            p, q = (er + od[k][1], ei - od[k][0]), (er - od[k][1], ei + od[k][0])
            y[k], y[k + 4] = (p, q) if sgn < 0 else (q, p)
        else:
            tr, ti = _twiddle(od[k], k, 8, sgn)
            y[k], y[k + 4] = (er + tr, ei + ti), (er - tr, ei - ti)
    return y


_C1, _C2 = math.cos(2 * math.pi / 5), math.cos(4 * math.pi / 5)
_S1, _S2 = math.sin(2 * math.pi / 5), math.sin(4 * math.pi / 5)


def _rfft5(u):
    x = [u[:, a * 128:(a + 1) * 128] for a in range(5)]
    s1, s2, d1, d2 = x[1] + x[4], x[2] + x[3], x[4] - x[1], x[3] - x[2]
    return jnp.concatenate([
        x[0] + s1 + s2,
        x[0] + _C1 * s1 + _C2 * s2, _S1 * d1 + _S2 * d2,
        x[0] + _C2 * s1 + _C1 * s2, _S2 * d1 - _S1 * d2], axis=1)


def _irfft5(q):
    q0, q1r, q1i, q2r, q2i = [q[:, a * 128:(a + 1) * 128] for a in range(5)]
    e1, e2 = q0 + _C1 * q1r + _C2 * q2r, q0 + _C2 * q1r + _C1 * q2r
    o1, o2 = _S1 * q1i + _S2 * q2i, _S2 * q1i - _S1 * q2i
    return jnp.concatenate([q0 + q1r + q2r, e1 - o1, e2 - o2, e2 + o2, e1 + o1], axis=1)


def _layernorm(x):
    mu = jnp.mean(x, axis=1, keepdims=True)
    d = x - mu
    var = jnp.mean(d * d, axis=1, keepdims=True)
    return _rnd(d * jax.lax.rsqrt(var + 1e-5))


NCH = 5
WROWS = DM * H // NCH


NWO = 16
WOROWS = H * DH // NWO
NSEG = S // SEG
BSCHED = (('d', 0), ('s', 9), ('i', 1), ('f', 0), ('r', -8))
LAG = (2, 3, 6)
_KR = ((0, 128), (128, 384), (384, 640))


def _pack(v):
    return pltpu.bitcast(v.astype(BF16), U32)


def _unpack(v):
    return pltpu.bitcast(v, BF16)


def _rows(i, n):
    return pl.ds(i * n, n) if isinstance(i, int) else pl.ds(pl.multiple_of(i * n, n), n)


def _segs(s, n):
    return pl.ds(s * SEG, n * SEG) if isinstance(s, int) else pl.ds(pl.multiple_of(s * SEG, SEG), n * SEG)


def _kernel(x_hbm, mem_hbm, wq_hbm, wk_hbm, wv_hbm, wo_hbm, wr_hbm, wi_hbm,
            fd_hbm, fdt_hbm, fs_hbm, fst_hbm,
            o_hbm,
            xio, memb, stage, t32, wqkv, wostage, wo, wb, wt, wp,
            fd, fdt, fs, fst,
            xs, us, u_buf, z_buf, zero, sems):
    cnt = [0]

    def copy(src, dst):
        c = pltpu.make_async_copy(src, dst, sems.at[cnt[0]])
        cnt[0] += 1
        c.start()
        return c

    head, rest = pl.ds(0, 256), pl.ds(256, S - 256)
    c_head = [copy(x_hbm.at[head], xio.at[head]), copy(mem_hbm, memb)]
    w_sem = cnt[0]
    for i, w in enumerate((wq_hbm, wk_hbm, wv_hbm)):
        for c in range(NCH):
            copy(w.at[pl.ds(c * WROWS, WROWS)], stage.at[i * NCH + c])
    wo_sem = cnt[0]
    for c in range(NWO):
        copy(wo_hbm.at[_rows(c, WOROWS)], wostage.at[_rows(c, WOROWS)])
    c_next = [copy(fd_hbm, fd),
              copy(wr_hbm.at[:, head], wb.at[0, :, head]), copy(wi_hbm.at[:, head], wb.at[1, :, head])]
    c_rest = [copy(x_hbm.at[rest], xio.at[rest]),
              copy(wr_hbm.at[:, rest], wb.at[0, :, rest]), copy(wi_hbm.at[:, rest], wb.at[1, :, rest])]
    c_b = [copy(fs_hbm, fs), copy(fst_hbm, fst), copy(fdt_hbm, fdt)]

    def set_input(s, x):
        x = x.astype(F32)
        xs[_segs(s, x.shape[0] // SEG), :] = x
        us[_segs(s, x.shape[0] // SEG), :] = _layernorm(x)

    for c in c_head:
        c.wait()
    set_input(0, xio[:4 * SEG, :])

    for i in range(3):
        def w_chunk(c, _):
            n = i * NCH + c
            pltpu.make_async_copy(stage.at[n], stage.at[n], sems.at[w_sem + n]).wait()

            def widen(j, _):
                t32[_rows(j, 256), :] = pltpu.bitcast(stage[n, _rows(j, 512), :], U32)
            jax.lax.fori_loop(0, WROWS // 512, widen, None)

            def split(j, _):
                v = t32[pl.ds(j, 128, stride=H // 2), :]
                wqkv[2 * j, _rows(c, 64), i * 128:(i + 1) * 128] = _pack(pltpu.bitcast(v << 16, F32))
                wqkv[2 * j + 1, _rows(c, 64), i * 128:(i + 1) * 128] = _pack(
                    pltpu.bitcast(v & np.uint32(0xFFFF0000), F32))
            jax.lax.fori_loop(0, H // 2, split, None, unroll=2)
        jax.lax.fori_loop(0, NCH, w_chunk, None)

    def wo_chunk(c, _):
        blk = wostage.at[_rows(c, WOROWS)]
        pltpu.make_async_copy(blk, blk, sems.at[wo_sem + c]).wait()
        wo[_rows(c, WOROWS // 2), :] = pltpu.bitcast(wostage[_rows(c, WOROWS), :], U32)

    def filter_prep(part, blk):
        wt[:DF, :] = wb[part, :, _rows(blk, 128)].astype(F32)
        lane = jax.lax.broadcasted_iota(jnp.int32, (1, 128), 1)
        sub = jax.lax.broadcasted_iota(jnp.int32, (64, 128), 0)
        for r in range(3):
            lo = wt[pl.ds(r, 64, stride=5), :]
            if r == 0:
                hi = jnp.where(sub == 0, wt[DF - 1:DF, :], 0.0)
                c = jnp.where((lane == 0) | (lane == 64), 1.0 / (S * DM), 2.0 / (S * DM))
            else:
                hi = wt[pl.ds(5 - r, 64, stride=5), :]
                c = 2.0 / (S * DM)
            w = jnp.concatenate([lo, hi], axis=0).T * c
            for g in range(128 // RS):
                wp[part * 3 + r, pl.ds(blk * (128 // RS) + g, RS, stride=NB + 1), :] = w[g * RS:(g + 1) * RS]

    def fwd_vpu(i, n):
        return _rfft5(_layernorm(xs[_segs(i, n), :]))

    def fwd_mxu(i, v, n):
        for r, (k0, k1) in enumerate(_KR):
            u_buf[r, _segs(i, n), :] = _dot(v[:, k0:k1], _unpack(fd[k0 // 2:k1 // 2, :]))

    def inv_mxu(i, n):
        return jnp.concatenate(
            [_dot(z_buf[r, _segs(i, n), :], _unpack(fdt[:, k0:k1])) for r, (k0, k1) in enumerate(_KR)],
            axis=1)

    def inv_vpu(i, q, n):
        return (xs[_segs(i, n), :] + _rnd(_irfft5(q))).astype(BF16)

    row = jax.lax.broadcasted_iota(jnp.int32, (L, L), 0)
    col = jax.lax.broadcasted_iota(jnp.int32, (L, L), 1)
    mask = (row >= SEG) | (col >= SEG) | (row >= col)
    scale = DH ** -0.5
    G = 4

    def a_step(s, mem, jobs):
        hh = jnp.concatenate([us[_rows(s, SEG), :], mem], axis=0)
        qkv, sc, pp, oo = {}, {}, {}, {}
        acc = None
        for t in range(H + H // G):
            if t < H:
                qkv[t] = _dot(hh, _unpack(wqkv[t]))
            else:
                g = t - H
                o = jnp.concatenate([oo[g * G + i] for i in range(G)], axis=1)
                o = jnp.concatenate([o[SEG:], o[:SEG]], axis=0)
                r = _dot(o, _unpack(wo[g * G * 64:(g + 1) * G * 64, :]))
                acc = r if acc is None else acc + r
            h = t - LAG[0]
            if 0 <= h < H:
                sc[h] = _dot(qkv[h][:, :128], qkv[h][:, 128:256].astype(BF16), _NT)
            h = t - LAG[1]
            if 0 <= h < H:
                z = jnp.where(mask, sc[h] * scale, -1e9)
                e = jnp.exp(z - jnp.max(z, axis=1, keepdims=True))
                pp[h] = e * (1.0 / jnp.sum(e, axis=1, keepdims=True))
            h = t - LAG[2]
            if 0 <= h < H:
                oo[h] = _dot(pp[h], qkv[h][:, 256:].astype(BF16))
            if t in jobs:
                jobs[t]()
        xs[_rows(s, SEG), :] = _rnd(xs[_rows(s, SEG), :] + _rnd(acc[M:]))
        return acc[:M]

    def radix8(buf, sgn, r, j):
        for n1 in range(4):
            rows = [_rows((n1 + 4 * m) * 8 + j, 8) for m in range(8)]
            y = _fft8([(buf[r, q, :128], buf[r, q, 128:]) for q in rows], sgn)
            for q, (re, im) in zip(rows, y):
                buf[r, q, :128] = re
                buf[r, q, 128:] = im

    def parts(x, j):
        return x[16 * j:16 * j + 8], x[16 * j + 8:16 * j + 16]

    def dft_fwd(r, k2):
        t = []
        for j in range(8):
            rows = [_rows((n1 + 4 * k2) * 8 + j, 8) for n1 in range(4)]
            t.append(_fft4([_twiddle((u_buf[r, q, :128], u_buf[r, q, 128:]), n1 * k2, RS, -1)
                            for n1, q in enumerate(rows)], -1))
        return [_dot(_unpack(fs[k2 + 8 * k1]), jnp.concatenate([v for j in range(8) for v in t[j][k1]], axis=0).astype(BF16))
                for k1 in range(4)]

    def filt(r, k2, xf):
        out = []
        for k1, x in enumerate(xf):
            y = []
            for j in range(8):
                q = pl.ds((k2 + 8 * k1) * (NB + 1) + 8 * j, 8)
                (xr, xi), wr, wi = parts(x, j), wp[r, q, :], wp[3 + r, q, :]
                y += [xr * wr - xi * wi, xr * wi + xi * wr]
            out.append(jnp.concatenate(y, axis=0).astype(BF16))
        return out

    def dft_inv(r, k2, ys):
        z = [_dot(_unpack(fst[k2 + 8 * k1]), y) for k1, y in enumerate(ys)]
        for j in range(8):
            for n1, v in enumerate(_fft4([parts(x, j) for x in z], +1)):
                q = _rows((n1 + 4 * k2) * 8 + j, 8)
                z_buf[r, q, :128], z_buf[r, q, 128:] = _twiddle(v, n1 * k2, RS, +1)

    def b_mid():
        z0, z1 = zero[0], zero[1]
        st = {}
        stages = dict(d=lambda r, j: st.update({(r, j): dft_fwd(r + z0, j)}),
                      f=lambda r, j: st.update({(r, j): filt(r, j, st[r, j])}),
                      i=lambda r, j: dft_inv(r, j, st.pop((r, j))),
                      r=lambda r, j: radix8(u_buf, -1, r + z1, j),
                      s=lambda r, j: radix8(z_buf, +1, r, j))
        for t in range(-12, 40):
            for name, lag in BSCHED:
                if 0 <= t - lag < 24:
                    stages[name](*divmod(t - lag, 8))

    for i in range(2):
        zero[i] = 0
    mem0 = memb[...].astype(F32)

    last = H + H // G - 1

    def a_first(i, mem):
        @pl.when(i == 1)
        def _():
            for c in c_rest:
                c.wait()
        s = 3 * i + 1
        prv, nxt, blk = jnp.maximum(s - 2, 0), jnp.minimum(s + 3, NSEG - 3), jnp.minimum(i, S // 128 - 1)
        st = {}
        mem = a_step(s, mem, {10: lambda: filter_prep(0, blk), 20: lambda: st.update(v=fwd_vpu(prv, 2)),
                              last: lambda: fwd_mxu(prv, st["v"], 2)})
        mem = a_step(s + 1, mem, {10: lambda: filter_prep(1, blk), 20: lambda: st.update(v=fwd_vpu(s, 1)),
                                  last: lambda: fwd_mxu(s, st["v"], 1)})
        return a_step(s + 2, mem, {10: lambda: set_input(s + 3, xio[_segs(nxt, 3), :])})

    def a_second(i, mem):
        s = 2 * i
        prv, nxt = jnp.maximum(s - 2, 0), jnp.minimum(s + 2, NSEG - 2)
        st = {}
        mem = a_step(s, mem, {20: lambda: st.update(v=fwd_vpu(prv, 2)), last: lambda: fwd_mxu(prv, st["v"], 2)})
        return a_step(s + 1, mem, {10: lambda: st.update(q=inv_mxu(nxt, 2)),
                                   13: lambda: set_input(s + 2, inv_vpu(nxt, st["q"], 2))})

    per = NWO * G // H
    mem1 = a_step(0, mem0, {H - 1 + g: functools.partial(jax.lax.fori_loop, g * per, (g + 1) * per, wo_chunk, None)
                            for g in range(H // G)})
    for c in c_next:
        c.wait()
    jax.lax.fori_loop(0, (NSEG - 1) // 3, a_first, mem1)
    for c in c_b:
        c.wait()

    def layer(l, _):
        fwd_mxu(NSEG - 2, fwd_vpu(NSEG - 2, 2), 2)
        b_mid()

        @pl.when(l == 0)
        def _():
            set_input(0, inv_vpu(0, inv_mxu(0, 2), 2))
            jax.lax.fori_loop(0, NSEG // 2, a_second, mem0)
    jax.lax.fori_loop(0, 2, layer, None)

    c_out = []
    for s in range(0, NSEG, 8):
        xio[_segs(s, 8), :] = inv_vpu(s, inv_mxu(s, 8), 8)
        c_out.append(copy(xio.at[_segs(s, 8)], o_hbm.at[_segs(s, 8)]))
    for c in c_out:
        c.wait()


@functools.partial(jax.jit, static_argnames=("A_seg_len",))
def pallas_interleave_layers__memory_aug_recurrent_mem_tr__spectral_gfnet__prompt_kernel(
    A_x, A_mem0, A_Wq, A_Wk, A_Wv, A_Wo, A_seg_len, B_x, B_w_r, B_w_i,
):
    del B_x
    assert A_x.shape == (1, S, DM) and A_Wq.shape == (DM, H, DH) and int(A_seg_len) == SEG
    consts = _constants()
    vm = pltpu.VMEM
    out = pl.pallas_call(
        _kernel,
        out_shape=jax.ShapeDtypeStruct((S, DM), BF16),
        in_specs=[pl.BlockSpec(memory_space=pltpu.HBM)] * 12,
        out_specs=pl.BlockSpec(memory_space=pltpu.HBM),
        scratch_shapes=[
            vm((S, DM), BF16),
            vm((M, DM), BF16),
            vm((3 * NCH, WROWS, DH), BF16),
            vm((WROWS // 2 + H, DH), U32),
            vm((H, DM // 2, 3 * DH), U32),
            vm((H * DH, DM), BF16),
            vm((H * DH // 2, DM), U32),
            vm((2, DF, S), BF16),
            vm((328, 128), F32),
            vm((6, S + RS + NB, 128), F32),
            vm((DM // 2, 256), U32), vm((128, DM), U32),
            vm((RS, NB, 128), U32), vm((RS, NB, 128), U32),
            vm((S + 3 * SEG, DM), F32), vm((S + 3 * SEG, DM), F32),
            vm((3, S, 256), F32),
            vm((3, S, 256), F32),
            pltpu.SMEM((2,), jnp.int32),
            pltpu.SemaphoreType.DMA((19 + 3 * NCH + NWO,)),
        ],
        compiler_params=pltpu.CompilerParams(vmem_limit_bytes=110 * 2**20),
        name="rmt_gfnet",
    )(A_x.reshape(S, DM), A_mem0.reshape(M, DM),
      A_Wq.reshape(DM * H, DH), A_Wk.reshape(DM * H, DH), A_Wv.reshape(DM * H, DH),
      A_Wo.reshape(H * DH, DM), B_w_r.T, B_w_i.T, *consts)
    return out.reshape(1, S, DM)
```

```python
import functools
import math

import jax
import jax.numpy as jnp
import numpy as np
import jax.experimental.pallas as pl
import jax.experimental.pallas.tpu as pltpu

S, DM, H, DH, M, SEG = 2048, 640, 32, 128, 8, 32
L = M + SEG
DF = DM // 2 + 1
RS = 32
NB = S // RS
F32, BF16, U32 = jnp.float32, jnp.bfloat16, jnp.uint32
_NN = (((1,), (0,)), ((), ()))
_NT = (((1,), (1,)), ((), ()))


def _dot(a, b, dims=_NN):
    return jax.lax.dot_general(a, b, dims, preferred_element_type=F32)


def _rnd(v):
    return v.astype(BF16).astype(F32)


def _constants():
    b = np.arange(128)[:, None].astype(np.float64)
    j = np.arange(128)
    fd = np.zeros((5 * 128, 256))
    th = 2 * np.pi * b * (5 * j[None, :65]) / DM
    fd[:128, :65] = np.cos(th)
    fd[:128, 128:128 + 65] = -np.sin(th)
    fd[:128, 128] = 0.0
    fd[:128, 128 + 64] = 0.0
    for r in (1, 2):
        fp = np.where(j < 64, r + 5 * j, (5 - r) + 5 * (j - 64))
        f = np.where(j < 64, fp, DM - fp)
        sg = np.where(j < 64, 1.0, -1.0)[None, :]
        th = 2 * np.pi * b * f[None, :] / DM
        o = 128 + (r - 1) * 256
        fd[o:o + 128, :128] = np.cos(th)
        fd[o:o + 128, 128:] = -sg * np.sin(th)
        fd[o + 128:o + 256, :128] = np.sin(th)
        fd[o + 128:o + 256, 128:] = sg * np.cos(th)
    fs = np.zeros((RS, 2 * NB, 2 * NB))
    g = np.arange(NB)[:, None].astype(np.float64)
    bb = np.arange(NB)[None, :].astype(np.float64)
    for r in range(RS):
        th = 2 * np.pi * ((r + RS * g) * bb % S) / S
        c, s = np.cos(th), np.sin(th)
        fs[r] = np.block([[c, s], [-s, c]])
    i = np.arange(2 * NB)
    il = i % 8 + 8 * (i // 16) + NB * (i // 8 % 2)
    fs = fs[:, il][:, :, il]
    bf = lambda a: np.asarray(a, dtype=BF16)


    def pk(a):
        w = np.ascontiguousarray(bf(a)).view(np.uint16).astype(np.uint32)
        return w[..., 0::2, :] | (w[..., 1::2, :] << 16)
    return (pk(fd), pk(fd.T), pk(fs), pk(fs.transpose(0, 2, 1)))


def _fft4(x, sgn):
    (ar, ai), (br, bi), (cr, ci), (dr, di) = x
    s0r, s0i, d0r, d0i = ar + cr, ai + ci, ar - cr, ai - ci
    s1r, s1i, d1r, d1i = br + dr, bi + di, br - dr, bi - di
    p = (d0r + d1i, d0i - d1r)
    q = (d0r - d1i, d0i + d1r)
    y1, y3 = (p, q) if sgn < 0 else (q, p)
    return [(s0r + s1r, s0i + s1i), y1, (s0r - s1r, s0i - s1i), y3]


def _twiddle(v, e, n, sgn):
    if e == 0:
        return v
    vr, vi = v
    if 4 * e == n:
        return (-vi, vr) if sgn > 0 else (vi, -vr)
    c, s = math.cos(2 * math.pi * e / n), sgn * math.sin(2 * math.pi * e / n)
    if (8 * e) % (2 * n) == n:
        if c * s > 0:
            return ((vr - vi) * c, (vr + vi) * c)
        return ((vr + vi) * c, (vi - vr) * c)
    return (vr * c - vi * s, vr * s + vi * c)


def _fft8(x, sgn):
    ev, od = _fft4(x[0::2], sgn), _fft4(x[1::2], sgn)
    y = [None] * 8
    for k in range(4):
        (er, ei) = ev[k]
        if k == 2:
            p, q = (er + od[k][1], ei - od[k][0]), (er - od[k][1], ei + od[k][0])
            y[k], y[k + 4] = (p, q) if sgn < 0 else (q, p)
        else:
            tr, ti = _twiddle(od[k], k, 8, sgn)
            y[k], y[k + 4] = (er + tr, ei + ti), (er - tr, ei - ti)
    return y


_C1, _C2 = math.cos(2 * math.pi / 5), math.cos(4 * math.pi / 5)
_S1, _S2 = math.sin(2 * math.pi / 5), math.sin(4 * math.pi / 5)


def _rfft5(u):
    x = [u[:, a * 128:(a + 1) * 128] for a in range(5)]
    s1, s2, d1, d2 = x[1] + x[4], x[2] + x[3], x[4] - x[1], x[3] - x[2]
    return jnp.concatenate([
        x[0] + s1 + s2,
        x[0] + _C1 * s1 + _C2 * s2, _S1 * d1 + _S2 * d2,
        x[0] + _C2 * s1 + _C1 * s2, _S2 * d1 - _S1 * d2], axis=1)


def _irfft5(q):
    q0, q1r, q1i, q2r, q2i = [q[:, a * 128:(a + 1) * 128] for a in range(5)]
    e1, e2 = q0 + _C1 * q1r + _C2 * q2r, q0 + _C2 * q1r + _C1 * q2r
    o1, o2 = _S1 * q1i + _S2 * q2i, _S2 * q1i - _S1 * q2i
    return jnp.concatenate([q0 + q1r + q2r, e1 - o1, e2 - o2, e2 + o2, e1 + o1], axis=1)


def _layernorm(x):
    mu = jnp.mean(x, axis=1, keepdims=True)
    d = x - mu
    var = jnp.mean(d * d, axis=1, keepdims=True)
    return _rnd(d * jax.lax.rsqrt(var + 1e-5))


NCH = 5
WROWS = DM * H // NCH
NWO = 16
WOROWS = H * DH // NWO
NSEG = S // SEG
OUT_SEGS = (8,) * 8
LAG = (2, 3, 6)
BSCHED = (("d", 0), ("s", 9), ("i", 1), ("f", 0), ("r", -8))
_KR = ((0, 128), (128, 384), (384, 640))


def _pack(v):
    return pltpu.bitcast(v.astype(BF16), U32)


def _unpack(v):
    return pltpu.bitcast(v, BF16)


def _rows(i, n):
    return pl.ds(i * n, n) if isinstance(i, int) else pl.ds(pl.multiple_of(i * n, n), n)


def _segs(s, n):
    return pl.ds(s * SEG, n * SEG) if isinstance(s, int) else pl.ds(pl.multiple_of(s * SEG, SEG), n * SEG)


def _kernel(x_hbm, mem_hbm, wq_hbm, wk_hbm, wv_hbm, wo_hbm, wr_hbm, wi_hbm,
            fd_hbm, fdt_hbm, fs_hbm, fst_hbm,
            o_hbm,
            xio, memb, stage, t32, wqkv, wostage, wo, wb, wt, wp,
            fd, fdt, fs, fst,
            xs, us, u_buf, z_buf, zero, sems):
    cnt = [0]

    def copy(src, dst):
        c = pltpu.make_async_copy(src, dst, sems.at[cnt[0]])
        cnt[0] += 1
        c.start()
        return c

    head, rest = _segs(0, 7), _segs(7, NSEG - 7)
    whead, wrest = pl.ds(0, 128), pl.ds(128, S - 128)
    c_head = [copy(x_hbm.at[head], xio.at[head]), copy(mem_hbm, memb)]
    w_sem = cnt[0]
    for i, w in enumerate((wq_hbm, wk_hbm, wv_hbm)):
        for c in range(NCH):
            copy(w.at[pl.ds(c * WROWS, WROWS)], stage.at[i * NCH + c])
    wo_sem = cnt[0]
    for c in range(NWO):
        copy(wo_hbm.at[_rows(c, WOROWS)], wostage.at[_rows(c, WOROWS)])
    c_next = [copy(fd_hbm, fd),
              copy(wr_hbm.at[:, whead], wb.at[0, :, whead]), copy(wi_hbm.at[:, whead], wb.at[1, :, whead])]
    c_rest = [copy(x_hbm.at[rest], xio.at[rest]),
              copy(wr_hbm.at[:, wrest], wb.at[0, :, wrest]), copy(wi_hbm.at[:, wrest], wb.at[1, :, wrest])]
    c_b = [copy(fs_hbm, fs), copy(fst_hbm, fst), copy(fdt_hbm, fdt)]

    def set_input(s, x):
        x = x.astype(F32)
        xs[_segs(s, x.shape[0] // SEG), :] = x
        us[_segs(s, x.shape[0] // SEG), :] = _layernorm(x)

    for c in c_head:
        c.wait()
    set_input(0, xio[:4 * SEG, :])

    for i in range(3):
        def w_chunk(c, _):
            n = i * NCH + c
            pltpu.make_async_copy(stage.at[n], stage.at[n], sems.at[w_sem + n]).wait()

            def widen(j, _):
                t32[_rows(j, 256), :] = pltpu.bitcast(stage[n, _rows(j, 512), :], U32)
            jax.lax.fori_loop(0, WROWS // 512, widen, None)

            def split(j, _):
                v = t32[pl.ds(j, 128, stride=H // 2), :]
                wqkv[2 * j, _rows(c, 64), i * 128:(i + 1) * 128] = _pack(pltpu.bitcast(v << 16, F32))
                wqkv[2 * j + 1, _rows(c, 64), i * 128:(i + 1) * 128] = _pack(
                    pltpu.bitcast(v & np.uint32(0xFFFF0000), F32))
            jax.lax.fori_loop(0, H // 2, split, None, unroll=2)
        jax.lax.fori_loop(0, NCH, w_chunk, None)

    def wo_chunk(c, _):
        blk = wostage.at[_rows(c, WOROWS)]
        pltpu.make_async_copy(blk, blk, sems.at[wo_sem + c]).wait()
        wo[_rows(c, WOROWS // 2), :] = pltpu.bitcast(wostage[_rows(c, WOROWS), :], U32)

    def filter_prep(part, blk):
        wt[:DF, :] = wb[part, :, _rows(blk, 128)].astype(F32)
        lane = jax.lax.broadcasted_iota(jnp.int32, (1, 128), 1)
        sub = jax.lax.broadcasted_iota(jnp.int32, (64, 128), 0)
        for r in range(3):
            lo = wt[pl.ds(r, 64, stride=5), :]
            if r == 0:
                hi = jnp.where(sub == 0, wt[DF - 1:DF, :], 0.0)
                c = jnp.where((lane == 0) | (lane == 64), 1.0 / (S * DM), 2.0 / (S * DM))
            else:
                hi = wt[pl.ds(5 - r, 64, stride=5), :]
                c = 2.0 / (S * DM)
            w = jnp.concatenate([lo, hi], axis=0).T * c
            for g in range(128 // RS):
                wp[part * 3 + r, pl.ds(blk * (128 // RS) + g, RS, stride=NB + 1), :] = w[g * RS:(g + 1) * RS]

    def fwd_vpu(i, n):
        return _rfft5(_layernorm(xs[_segs(i, n), :]))

    def fwd_mxu(i, v, n):
        for r, (k0, k1) in enumerate(_KR):
            u_buf[r, _segs(i, n), :] = _dot(v[:, k0:k1], _unpack(fd[k0 // 2:k1 // 2, :]))

    def inv_mxu(i, n):
        return jnp.concatenate(
            [_dot(z_buf[r, _segs(i, n), :], _unpack(fdt[:, k0:k1])) for r, (k0, k1) in enumerate(_KR)],
            axis=1)

    def inv_vpu(i, q, n):
        return (xs[_segs(i, n), :] + _rnd(_irfft5(q))).astype(BF16)

    row = jax.lax.broadcasted_iota(jnp.int32, (L, L), 0)
    col = jax.lax.broadcasted_iota(jnp.int32, (L, L), 1)
    mask = (row >= SEG) | (col >= SEG) | (row >= col)
    scale = DH ** -0.5
    G = 4

    def a_step(s, mem, jobs):
        hh = jnp.concatenate([us[_rows(s, SEG), :], mem], axis=0)
        qkv, sc, pp, oo = {}, {}, {}, {}
        acc = None
        for t in range(H + H // G):
            if t < H:
                qkv[t] = _dot(hh, _unpack(wqkv[t]))
            else:
                g = t - H
                o = jnp.concatenate([oo[g * G + i] for i in range(G)], axis=1)
                o = jnp.concatenate([o[SEG:], o[:SEG]], axis=0)
                r = _dot(o, _unpack(wo[g * G * 64:(g + 1) * G * 64, :]))
                acc = r if acc is None else acc + r
            h = t - LAG[0]
            if 0 <= h < H:
                sc[h] = _dot(qkv[h][:, :128], qkv[h][:, 128:256].astype(BF16), _NT)
            h = t - LAG[1]
            if 0 <= h < H:
                z = jnp.where(mask, sc[h] * scale, -1e9)
                e = jnp.exp(z - jnp.max(z, axis=1, keepdims=True))
                pp[h] = e * (1.0 / jnp.sum(e, axis=1, keepdims=True))
            h = t - LAG[2]
            if 0 <= h < H:
                oo[h] = _dot(pp[h], qkv[h][:, 256:].astype(BF16))
            if t in jobs:
                jobs[t]()
        xs[_rows(s, SEG), :] = _rnd(xs[_rows(s, SEG), :] + _rnd(acc[M:]))
        return acc[:M]

    def radix8(buf, sgn, r, j):
        for n1 in range(4):
            rows = [_rows((n1 + 4 * m) * 8 + j, 8) for m in range(8)]
            y = _fft8([(buf[r, q, :128], buf[r, q, 128:]) for q in rows], sgn)
            for q, (re, im) in zip(rows, y):
                buf[r, q, :128] = re
                buf[r, q, 128:] = im

    def parts(x, j):
        return x[16 * j:16 * j + 8], x[16 * j + 8:16 * j + 16]

    def dft_fwd(r, k2):
        t = []
        for j in range(8):
            rows = [_rows((n1 + 4 * k2) * 8 + j, 8) for n1 in range(4)]
            t.append(_fft4([_twiddle((u_buf[r, q, :128], u_buf[r, q, 128:]), n1 * k2, RS, -1)
                            for n1, q in enumerate(rows)], -1))
        return [_dot(_unpack(fs[k2 + 8 * k1]),
                     jnp.concatenate([v for j in range(8) for v in t[j][k1]], axis=0).astype(BF16))
                for k1 in range(4)]

    def filt(r, k2, xf):
        out = []
        for k1, x in enumerate(xf):
            y = []
            for j in range(8):
                q = pl.ds((k2 + 8 * k1) * (NB + 1) + 8 * j, 8)
                (xr, xi), wr, wi = parts(x, j), wp[r, q, :], wp[3 + r, q, :]
                y += [xr * wr - xi * wi, xr * wi + xi * wr]
            out.append(jnp.concatenate(y, axis=0).astype(BF16))
        return out

    def dft_inv(r, k2, ys):
        z = [_dot(_unpack(fst[k2 + 8 * k1]), y) for k1, y in enumerate(ys)]
        for j in range(8):
            for n1, v in enumerate(_fft4([parts(x, j) for x in z], +1)):
                q = _rows((n1 + 4 * k2) * 8 + j, 8)
                z_buf[r, q, :128], z_buf[r, q, 128:] = _twiddle(v, n1 * k2, RS, +1)

    def b_mid():
        z0, z1 = zero[0], zero[1]
        st = {}
        stages = dict(d=lambda r, j: st.update({(r, j): dft_fwd(r + z0, j)}),
                      f=lambda r, j: st.update({(r, j): filt(r, j, st[r, j])}),
                      i=lambda r, j: dft_inv(r, j, st.pop((r, j))),
                      r=lambda r, j: radix8(u_buf, -1, r + z1, j),
                      s=lambda r, j: radix8(z_buf, +1, r, j))
        for t in range(-12, 40):
            for name, lag in BSCHED:
                if 0 <= t - lag < 24:
                    stages[name](*divmod(t - lag, 8))

    for i in range(2):
        zero[i] = 0
    mem0 = memb[...].astype(F32)

    last = H + H // G - 1

    def a_first(i, mem):
        @pl.when(i == 1)
        def _():
            for c in c_rest:
                c.wait()
        s = 3 * i + 1
        prv, nxt, blk = jnp.maximum(s - 2, 0), jnp.minimum(s + 3, NSEG - 3), jnp.minimum(i, S // 128 - 1)
        st = {}
        mem = a_step(s, mem, {10: lambda: filter_prep(0, blk), 20: lambda: st.update(v=fwd_vpu(prv, 2)),
                              last: lambda: fwd_mxu(prv, st["v"], 2)})
        mem = a_step(s + 1, mem, {10: lambda: filter_prep(1, blk), 20: lambda: st.update(v=fwd_vpu(s, 1)),
                                  last: lambda: fwd_mxu(s, st["v"], 1)})
        return a_step(s + 2, mem, {10: lambda: set_input(s + 3, xio[_segs(nxt, 3), :])})

    def a_second(i, mem):
        s = 2 * i
        prv, nxt = jnp.maximum(s - 2, 0), jnp.minimum(s + 2, NSEG - 2)
        st = {}
        mem = a_step(s, mem, {20: lambda: st.update(v=fwd_vpu(prv, 2)), last: lambda: fwd_mxu(prv, st["v"], 2)})
        return a_step(s + 1, mem, {10: lambda: st.update(q=inv_mxu(nxt, 2)),
                                   13: lambda: set_input(s + 2, inv_vpu(nxt, st["q"], 2))})

    per = NWO * G // H
    mem1 = a_step(0, mem0, {H - 1 + g: functools.partial(jax.lax.fori_loop, g * per, (g + 1) * per, wo_chunk, None)
                            for g in range(H // G)})
    for c in c_next:
        c.wait()
    jax.lax.fori_loop(0, (NSEG - 1) // 3, a_first, mem1)
    for c in c_b:
        c.wait()

    def layer(l, _):
        fwd_mxu(NSEG - 2, fwd_vpu(NSEG - 2, 2), 2)
        b_mid()

        @pl.when(l == 0)
        def _():
            set_input(0, inv_vpu(0, inv_mxu(0, 2), 2))
            jax.lax.fori_loop(0, NSEG // 2, a_second, mem0)
    jax.lax.fori_loop(0, 2, layer, None)

    c_out, s = [], 0
    for n in OUT_SEGS:
        xio[_segs(s, n), :] = inv_vpu(s, inv_mxu(s, n), n)
        c_out.append(copy(xio.at[_segs(s, n)], o_hbm.at[_segs(s, n)]))
        s += n
    for c in c_out:
        c.wait()


@functools.partial(jax.jit, static_argnames=("A_seg_len",))
def pallas_interleave_layers__memory_aug_recurrent_mem_tr__spectral_gfnet__prompt_kernel(
    A_x, A_mem0, A_Wq, A_Wk, A_Wv, A_Wo, A_seg_len, B_x, B_w_r, B_w_i,
):
    del B_x
    assert A_x.shape == (1, S, DM) and A_Wq.shape == (DM, H, DH) and int(A_seg_len) == SEG
    consts = _constants()
    vm = pltpu.VMEM
    out = pl.pallas_call(
        _kernel,
        out_shape=jax.ShapeDtypeStruct((S, DM), BF16),
        in_specs=[pl.BlockSpec(memory_space=pltpu.HBM)] * 12,
        out_specs=pl.BlockSpec(memory_space=pltpu.HBM),
        scratch_shapes=[
            vm((S, DM), BF16),
            vm((M, DM), BF16),
            vm((3 * NCH, WROWS, DH), BF16),
            vm((WROWS // 2 + H, DH), U32),
            vm((H, DM // 2, 3 * DH), U32),
            vm((H * DH, DM), BF16),
            vm((H * DH // 2, DM), U32),
            vm((2, DF, S), BF16),
            vm((328, 128), F32),
            vm((6, S + RS + NB, 128), F32),
            vm((DM // 2, 256), U32), vm((128, DM), U32),
            vm((RS, NB, 128), U32), vm((RS, NB, 128), U32),
            vm((S + 3 * SEG, DM), F32), vm((S + 3 * SEG, DM), F32),
            vm((3, S, 256), F32),
            vm((3, S, 256), F32),
            pltpu.SMEM((2,), jnp.int32),
            pltpu.SemaphoreType.DMA((11 + 3 * NCH + NWO + len(OUT_SEGS),)),
        ],
        compiler_params=pltpu.CompilerParams(vmem_limit_bytes=110 * 2**20),
        name="rmt_gfnet",
    )(A_x.reshape(S, DM), A_mem0.reshape(M, DM),
      A_Wq.reshape(DM * H, DH), A_Wk.reshape(DM * H, DH), A_Wv.reshape(DM * H, DH),
      A_Wo.reshape(H * DH, DM), B_w_r.T, B_w_i.T, *consts)
    return out.reshape(1, S, DM)
```
